```python
import jax
import jax.numpy as jnp

def _softmax(x, axis=-1):
    return jax.nn.softmax(x, axis=axis)
def _gelu(x):
    return jax.nn.gelu(x, approximate=True)
def _silu(x):
    return jax.nn.silu(x)
def _sigmoid(x):
    return jax.nn.sigmoid(x)
def _layernorm(x, axis=-1, eps=1e-5):
    m = jnp.mean(x, axis=axis, keepdims=True)
    v = jnp.var(x, axis=axis, keepdims=True)
    return (x - m) / jnp.sqrt(v + eps)
def _scatter_add(tgt, idx, src, axis=0):
    return tgt.at[idx].add(src)
def _segment_sum(src, seg, n):
    return jax.ops.segment_sum(src, seg, n)
class _Rng:
    def __init__(self, key):
        self._k = key
    def _next(self):
        self._k, sub = jax.random.split(self._k)
        return sub
    def normal(self, shape):
        return jax.random.normal(self._next(), shape, dtype=jnp.bfloat16)
    def randint(self, lo, hi, shape):
        return jax.random.randint(self._next(), shape, lo, hi, dtype=jnp.int32)
    def uniform(self, shape, lo=0.0, hi=1.0):
        return jax.random.uniform(self._next(), shape, jnp.bfloat16, lo, hi)
    def permutation(self, n):
        return jax.random.permutation(self._next(), n)


kernel_name = 'concat_heads__sliding_local_dilated__ssm_conv_s5__prompt'

def setup_inputs():
    _rng = _Rng(jax.random.key(int.from_bytes(__import__("os").urandom(4), "little")))
    _w = (lambda a: (lambda t: t.astype(jnp.bfloat16) if jnp.issubdtype(t.dtype, jnp.floating) else t)(jnp.asarray(a)))
    def _A_setup():
        B, S, D = 1, 2048, 448
        return {
            "x": _w((lambda *s: _rng.normal(s) * 0.05)(B, S, D)),
            "wqkv": _w((lambda *s: _rng.normal(s) * 0.05)(D, 3 * D)),
            "wo": _w((lambda *s: _rng.normal(s) * 0.05)(D, D)),
        }
    _A_in = _A_setup()

    def _B_setup():
        B, S, D = 1, 2048, 448
        P = D
        Lambda_re = -0.5 * jnp.exp((lambda *s: _rng.normal(s) * 0.05)(P))
        Lambda_im = (lambda *s: _rng.normal(s) * 0.05)(P) * 1.0
        B_re = (lambda *s: _rng.normal(s) * 0.05)(P, D) * (D ** -0.5)
        B_im = (lambda *s: _rng.normal(s) * 0.05)(P, D) * (D ** -0.5)
        C_re = (lambda *s: _rng.normal(s) * 0.05)(D, P) * (P ** -0.5)
        C_im = (lambda *s: _rng.normal(s) * 0.05)(D, P) * (P ** -0.5)
        log_dt = (lambda *s: _rng.normal(s) * 0.05)(P) * 0.3 - 2.0
        Dskip = (lambda *s: _rng.normal(s) * 0.05)(D)
        return {
            "x": _w((lambda *s: _rng.normal(s) * 0.05)(B, S, D)),
            "Lambda_re": _w(Lambda_re),
            "Lambda_im": _w(Lambda_im),
            "B_re": _w(B_re),
            "B_im": _w(B_im),
            "C_re": _w(C_re),
            "C_im": _w(C_im),
            "log_dt": _w(log_dt),
            "Dskip": _w(Dskip),
        }
    _B_in = _B_setup()

    return {
        "A_x": _A_in["x"],
        "A_wqkv": _A_in["wqkv"],
        "A_wo": _A_in["wo"],
        "B_x": _B_in["x"],
        "B_Lambda_re": _B_in["Lambda_re"],
        "B_Lambda_im": _B_in["Lambda_im"],
        "B_B_re": _B_in["B_re"],
        "B_B_im": _B_in["B_im"],
        "B_C_re": _B_in["C_re"],
        "B_C_im": _B_in["C_im"],
        "B_log_dt": _B_in["log_dt"],
        "B_Dskip": _B_in["Dskip"],
    }

def reference(A_x, A_wqkv, A_wo, B_x, B_Lambda_re, B_Lambda_im, B_B_re, B_B_im, B_C_re, B_C_im, B_log_dt, B_Dskip):
    def _A_ref(x, wqkv, wo):
        B, S, D = x.shape
        H = 16; Dh = D // H
        W, dil = 8, 2
        qkv = (lambda x, *d: x.transpose(*d))((x @ wqkv).reshape(B, S, 3, H, Dh), 2, 0, 3, 1, 4)
        q, k, v = qkv[0], qkv[1], qkv[2]
        scale = Dh ** -0.5
        pos = jnp.arange(S)
        off = jnp.arange(W) * dil
        idx = pos[:, None] - off[None, :]
        mask = idx >= 0
        idx_c = jnp.where(mask, idx, 0).reshape(-1)
        kg = k[:, :, idx_c, :].reshape(B, H, S, W, Dh)
        vg = v[:, :, idx_c, :].reshape(B, H, S, W, Dh)
        logits = jnp.einsum("bhsd,bhswd->bhsw", q, kg) * scale
        logits = jnp.where(mask[None, None, :, :], logits, -1e9)
        attn = _softmax(logits, axis=-1)
        o = jnp.einsum("bhsw,bhswd->bhsd", attn, vg)
        return (lambda x, *d: x.transpose(*d))(o, 0, 2, 1, 3).reshape(B, S, D) @ wo

    def _B_ref(x, Lambda_re, Lambda_im, B_re, B_im, C_re, C_im, log_dt, Dskip):
        Bsz, L, H = x.shape
        Lam = Lambda_re + 1j * Lambda_im
        Bmat = B_re + 1j * B_im
        Cmat = C_re + 1j * C_im
        dt = jnp.exp(log_dt)
        Lam_bar = jnp.exp(dt * Lam)
        B_bar = ((Lam_bar - 1.0) / Lam)[:, None] * Bmat
        Bu = jnp.einsum("bld,pd->blp", x + 0j, B_bar)
        h = jnp.zeros_like(Bu[:, 0, :])
        hs = []
        for t in range(L):
            h = Lam_bar[None, :] * h + Bu[:, t, :]
            hs.append(h)
        hseq = jnp.stack(hs, 1)
        y = 2.0 * jnp.einsum("blp,dp->bld", hseq, Cmat).real + x * Dskip[None, None, :]
        return y

    a = _A_ref(A_x, A_wqkv, A_wo)
    b = _B_ref(B_x, B_Lambda_re, B_Lambda_im, B_B_re, B_B_im, B_C_re, B_C_im, B_log_dt, B_Dskip)
    return jnp.concatenate([a, b], axis=-1)
```

```python
import jax
import jax.numpy as jnp
from jax import lax
import jax.experimental.pallas as pl
import jax.experimental.pallas.tpu as pltpu

S, D, H, DH, W = 2048, 448, 16, 28, 8
NJ = 16
T = 256
NC = S // T
SEG = T // 8
NPRE = 3
F32, BF16 = jnp.float32, jnp.bfloat16
NT = (((1,), (1,)), ((), ()))


def _cmul(ar, ai, br, bi):
    return ar * br - ai * bi, ar * bi + ai * br


def _kernel(ax_h, wqkv_h, wo_h, bx_h, lre_h, lim_h, bre_h, bim_h, cre_h, cim_h, ldt_h, dsk_h,
            out_h,
            axv, wv, wov, bxv, bv, cv, pv0, pv1, pv2, pv3, prm, bcat, ccat, xb32, ubuf, hbuf,
            wt32, wtp, wo32, wop, xa32, xp, kext, vext, obuf, isem, osem):
    def cp(i, src, dst):
        return pltpu.make_async_copy(src, dst, isem.at[i])
    c_par = [cp(0, lre_h, pv0), cp(1, lim_h, pv1), cp(2, ldt_h, pv2), cp(3, dsk_h, pv3)]
    c_b = [cp(4, bre_h, bv.at[0]), cp(5, bim_h, bv.at[1])]
    c_c = [cp(6, cre_h, cv.at[0]), cp(7, cim_h, cv.at[1])]
    c_bx = [cp(8 + c, bx_h.at[:, pl.ds(c * T, T)], bxv.at[c]) for c in range(NC)]
    c_w, c_ax, c_wo = cp(8 + NC, wqkv_h, wv), cp(9 + NC, ax_h, axv), cp(10 + NC, wo_h, wov)
    for c in c_par + c_b + c_bx[:1] + c_c + c_bx[1:NPRE] + [c_w, c_ax, c_wo] + c_bx[NPRE:]:
        c.start()

    for c in c_par:
        c.wait()
    prm[...] = jnp.zeros(prm.shape, F32)
    for i in range(4):
        prm[i:i + 1, 0:D] = (pv0, pv1, pv2, pv3)[i][...].astype(F32).reshape(1, D)
    lane5 = lax.broadcasted_iota(jnp.int32, (8, 512), 1)
    lre = jnp.where(lane5 < D, jnp.broadcast_to(prm[0:1, :], (8, 512)), -1.0)
    lim = jnp.broadcast_to(prm[1:2, :], (8, 512))
    dt = jnp.exp(jnp.broadcast_to(prm[2:3, :], (8, 512))).astype(BF16).astype(F32)
    zr, zi = dt * lre, dt * lim
    mag = jnp.exp(zr)
    lr, li = mag * jnp.cos(zi), mag * jnp.sin(zi)
    den = lre * lre + lim * lim
    nr, ni = lr - 1.0, li
    cr = (nr * lre + ni * lim) / den
    ci = (ni * lre - nr * lim) / den
    lane1 = lax.broadcasted_iota(jnp.int32, (8, 128), 1)
    lo = lane1 < 64

    def tiles(r, i):
        r3, i3 = r[:, 384:], i[:, 384:]
        rr = jnp.where(lo, r3, pltpu.roll(r3, 64, 1))
        ii = jnp.where(lo, -i3, pltpu.roll(i3, 64, 1))
        return ([r[:, 128 * k:128 * k + 128] for k in range(3)] + [rr],
                [i[:, 128 * k:128 * k + 128] for k in range(3)] + [ii])
    lam = tiles(lr, li)
    pr, pi_ = lr, li
    for _ in range(5):
        pr, pi_ = _cmul(pr, pi_, pr, pi_)
    pw = []
    for _ in range(3):
        pw.append(tiles(pr, pi_))
        pr, pi_ = _cmul(pr, pi_, pr, pi_)
    dsk = pltpu.roll(jnp.broadcast_to(prm[3:4, :], (8, 512)), 64, 1)

    def cstep(m, k, a, b):
        if k < 3:
            return m[0][k] * a - m[1][k] * b, m[0][k] * b + m[1][k] * a
        return m[0][k] * a + m[1][k] * b, m[0][k] * b - m[1][k] * a

    for c in c_b:
        c.wait()
    zb = jnp.zeros((D, 64), BF16)
    b_re = jnp.concatenate([zb, bv[0]], axis=1)
    b_im = jnp.concatenate([zb, bv[1]], axis=1)
    bcat[0:384, :] = b_re[0:384]
    bcat[384:768, :] = b_im[0:384]
    bcat[768:832, :] = b_re[384:448]
    bcat[832:896, :] = b_im[384:448]

    def prep_c():
        for c in c_c:
            c.wait()
        c_re = cv[0].astype(F32)
        c_im = cv[1].astype(F32)
        c2r = (2.0 * (c_re * cr[0:1, :D] - c_im * ci[0:1, :D])).astype(BF16)
        c2i = (-2.0 * (c_re * ci[0:1, :D] + c_im * cr[0:1, :D])).astype(BF16)
        ccat[0:64, :] = jnp.zeros((64, 896), BF16)
        ccat[64:512, 0:384] = c2r[:, 0:384]
        ccat[64:512, 384:768] = c2i[:, 0:384]
        ccat[64:512, 768:896] = jnp.concatenate([c2r[:, 384:448], c2i[:, 384:448]], axis=1)

    sub = lax.broadcasted_iota(jnp.int32, (8, 128), 0)

    def ssm_in(c):
        c_bx[c].wait()
        s = c % 2
        xt = bxv[c].astype(F32)
        xb32[s, 0] = jnp.concatenate([jnp.zeros((64, T), F32), xt[0:64]], axis=0).T
        for k in range(1, 4):
            xb32[s, k] = xt[128 * k - 64:128 * k + 64].T
        rows = []
        for j in range(SEG):
            rows.append(jnp.concatenate(
                [xb32[s, k, pl.ds(j, 8, stride=SEG), :] for k in range(4)], axis=1))
        xl = jnp.concatenate(rows, axis=0).astype(BF16)
        ubuf[s] = lax.dot_general(xl, bcat[...], NT, preferred_element_type=F32)

    def ssm_scan(c, carry):
        s = c % 2

        def u(j, k):
            if k < 3:
                return (ubuf[s, 8 * j:8 * j + 8, 128 * k:128 * k + 128],
                        ubuf[s, 8 * j:8 * j + 8, 384 + 128 * k:512 + 128 * k])
            m = ubuf[s, 8 * j:8 * j + 8, 768:896]
            return m, pltpu.roll(m, 64, 1)
        h = [u(0, k) for k in range(4)]
        for j in range(1, SEG):
            for k in range(4):
                a, b = cstep(lam, k, *h[k])
                ua, ub = u(j, k)
                h[k] = (a + ua, b + ub)
        for k in range(4):
            z = [jnp.where(sub == 0, carry[k][i], pltpu.roll(h[k][i], 1, 0)) for i in range(2)]
            for n in range(3):
                sh = 1 << n
                a, b = cstep(pw[n], k, *[jnp.where(sub >= sh, pltpu.roll(v, sh, 0), 0.0) for v in z])
                z = [z[0] + a, z[1] + b]
            h[k] = tuple(z)
        for j2 in range(SEG // 2):
            keep = []
            for j in (2 * j2, 2 * j2 + 1):
                for k in range(4):
                    a, b = cstep(lam, k, *h[k])
                    ua, ub = u(j, k)
                    h[k] = (a + ua, b + ub)
                keep.append(jnp.concatenate([h[0][0], h[1][0], h[2][0], h[0][1], h[1][1], h[2][1], h[3][0]], axis=1))
            hbuf[s, 16 * j2:16 * j2 + 16, :] = jnp.concatenate(keep, axis=0).astype(BF16)
        return [tuple(jnp.broadcast_to(v[7:8], (8, 128)) for v in h[k]) for k in range(4)]

    def ssm_out(c):
        s = c % 2
        y = lax.dot_general(hbuf[s], ccat[...], NT, preferred_element_type=F32)
        for j in range(SEG):
            for k in range(4):
                v = y[8 * j:8 * j + 8, 128 * k:128 * k + 128] + \
                    xb32[s, k, pl.ds(j, 8, stride=SEG), :] * dsk[:, 128 * k:128 * k + 128]
                if k == 0:
                    if c >= NPRE:
                        v = jnp.where(lo, obuf[3, pl.ds(c * T + j, 8, stride=SEG), :], v)
                    obuf[3, pl.ds(c * T + j, 8, stride=SEG), :] = v
                else:
                    obuf[3 + k, pl.ds(c * T + j, 8, stride=SEG), :] = v

    def out_b(c):
        return [pltpu.make_async_copy(obuf.at[k, pl.ds(c * T, T)],
                                      out_h.at[pl.ds(c * T, T), pl.ds(128 * k, 128)],
                                      osem.at[3 + 4 * c + k - 3]) for k in range(3, 7)]

    def att_prep():
        c_w.wait()
        for k in range(4):
            n = min(128, D - 128 * k)
            blk = wv[128 * k:128 * k + n, :].astype(F32)
            if n < 128:
                blk = jnp.concatenate([blk, jnp.zeros((128 - n, 3 * D), F32)], axis=0)
            wt32[k] = blk.T
        for g in range(3):
            for d in range(DH):
                v = [jnp.concatenate([wt32[k, pl.ds(g * D + hh * 224 + d, 8, stride=DH), :]
                                      for k in range(4)], axis=1) for hh in range(2)]
                wtp[g * D + 16 * d:g * D + 16 * d + 16, :] = jnp.concatenate(v, axis=0).astype(BF16)
        c_ax.wait()
        for k in range(4):
            n = min(128, D - 128 * k)
            blk = axv[128 * k:128 * k + n, :].astype(F32)
            if n < 128:
                blk = jnp.concatenate([blk, jnp.zeros((128 - n, S), F32)], axis=0)
            xa32[k] = blk.T
        c_wo.wait()
        wo = jnp.concatenate([wov[...].astype(F32), jnp.zeros((D, 64), F32)], axis=1)
        for k in range(4):
            wo32[k] = wo[:, 128 * k:128 * k + 128]
        for d in range(DH):
            v = [jnp.concatenate([wo32[k, pl.ds(hh * 224 + d, 8, stride=DH), :]
                                  for k in range(4)], axis=1) for hh in range(2)]
            wop[16 * d:16 * d + 16, :] = jnp.concatenate(v, axis=0).astype(BF16)

    def att_kv(j):
        xj = jnp.concatenate([xa32[k, pl.ds(j, 128, stride=NJ), :] for k in range(4)], axis=1).astype(BF16)
        xp[j] = xj
        kv = lax.dot_general(wtp[D:3 * D, :], xj, NT, preferred_element_type=F32)
        kext[j + 14] = kv[:D]
        vext[j + 14] = kv[D:]
        if j >= 2:
            kext[j - 2] = pltpu.roll(kv[:D], 1, 1)
            vext[j - 2] = pltpu.roll(kv[D:], 1, 1)

    lane16 = lax.broadcasted_iota(jnp.int32, (16, 128), 1)
    scale = DH ** -0.5

    def att(j):
        q = lax.dot_general(wtp[0:D, :], xp[j], NT, preferred_element_type=F32)
        lg = [None] * W
        for d in range(DH):
            qd = q[16 * d:16 * d + 16]
            for w in range(W):
                t = qd * kext[j + 14 - 2 * w, 16 * d:16 * d + 16, :]
                lg[w] = t if d == 0 else lg[w] + t
        for w in range(W):
            lg[w] = lg[w] * scale
            if j < 2 * w:
                lg[w] = jnp.where(lane16 == 0, -1e9, lg[w])
        m = lg[0]
        for w in range(1, W):
            m = jnp.maximum(m, lg[w])
        e = [jnp.exp(l - m) for l in lg]
        ssum = e[0]
        for w in range(1, W):
            ssum = ssum + e[w]
        inv = 1.0 / ssum
        p = [x * inv for x in e]
        os_ = []
        for d in range(DH):
            acc = None
            for w in range(W):
                t = p[w] * vext[j + 14 - 2 * w, 16 * d:16 * d + 16, :]
                acc = t if acc is None else acc + t
            os_.append(acc)
        o = jnp.concatenate(os_, axis=0).T.astype(BF16)
        res = jnp.dot(o, wop[...], preferred_element_type=F32)
        for k in range(4):
            v = res[:, 128 * k:128 * k + 128]
            if k == 3:
                n = NPRE * T // NJ
                old = obuf[3, pl.ds(j, n, stride=NJ), :]
                v = jnp.concatenate([jnp.where(lo[0:1], v[:n], old), v[n:]], axis=0)
            obuf[k, pl.ds(j, 128, stride=NJ), :] = v

    z = jnp.zeros((8, 128), F32)
    carry = [(z, z)] * 4
    ssm_in(0)
    prep_c()
    for c in range(NPRE):
        if c + 1 < NPRE:
            ssm_in(c + 1)
        carry = ssm_scan(c, carry)
        ssm_out(c)
    att_prep()
    for j in range(NJ):
        att_kv(j)
    for j in range(NJ):
        att(j)
    ssm_in(NPRE)
    oa = [pltpu.make_async_copy(obuf.at[k], out_h.at[:, pl.ds(128 * k, 128)], osem.at[k]) for k in range(3)]
    for c in oa:
        c.start()
    for c in range(NPRE):
        for x in out_b(c):
            x.start()
    for c in range(NPRE, NC):
        if c + 1 < NC:
            ssm_in(c + 1)
        carry = ssm_scan(c, carry)
        ssm_out(c)
        for x in out_b(c):
            x.start()
    for c in oa:
        c.wait()
    for c in range(NC):
        for x in out_b(c):
            x.wait()


@jax.jit
def pallas_concat_heads__sliding_local_dilated__ssm_conv_s5__prompt_kernel(
    A_x, A_wqkv, A_wo, B_x, B_Lambda_re, B_Lambda_im, B_B_re, B_B_im, B_C_re, B_C_im,
    B_log_dt, B_Dskip,
):
    hbm = pl.BlockSpec(memory_space=pltpu.HBM)
    out = pl.pallas_call(
        _kernel,
        out_shape=jax.ShapeDtypeStruct((S, 2 * D), F32),
        in_specs=[hbm] * 12,
        out_specs=hbm,
        scratch_shapes=[
            pltpu.VMEM((D, S), BF16),
            pltpu.VMEM((D, 3 * D), BF16),
            pltpu.VMEM((D, D), BF16),
            pltpu.VMEM((NC, D, T), BF16),
            pltpu.VMEM((2, D, D), BF16),
            pltpu.VMEM((2, D, D), BF16),
            *[pltpu.VMEM((D,), BF16)] * 4,
            pltpu.VMEM((8, 512), F32),
            pltpu.VMEM((896, 512), BF16),
            pltpu.VMEM((512, 896), BF16),
            pltpu.VMEM((2, 4, T, 128), F32),
            pltpu.VMEM((2, T, 896), F32),
            pltpu.VMEM((2, T, 896), BF16),
            pltpu.VMEM((4, 3 * D, 128), F32),
            pltpu.VMEM((3 * D, 512), BF16),
            pltpu.VMEM((4, D, 128), F32),
            pltpu.VMEM((D, 512), BF16),
            pltpu.VMEM((4, S, 128), F32),
            pltpu.VMEM((NJ, 128, 512), BF16),
            pltpu.VMEM((30, D, 128), F32),
            pltpu.VMEM((30, D, 128), F32),
            pltpu.VMEM((7, S, 128), F32),
            pltpu.SemaphoreType.DMA((11 + NC,)),
            pltpu.SemaphoreType.DMA((3 + 4 * NC,)),
        ],
        compiler_params=pltpu.CompilerParams(vmem_limit_bytes=100 * 1024 * 1024),
    )(A_x[0].T, A_wqkv, A_wo, B_x[0].T, B_Lambda_re, B_Lambda_im,
      B_B_re, B_B_im, B_C_re, B_C_im, B_log_dt, B_Dskip)
    return out.reshape(1, S, 2 * D)
```

```python
import jax
import jax.numpy as jnp
from jax import lax
import jax.experimental.pallas as pl
import jax.experimental.pallas.tpu as pltpu

S, D, H, DH, W = 2048, 448, 16, 28, 8
NJ = 16
T = 256
NC = S // T
SEGS = (36, 28)
XP = 20


def _row0(c):
    return 512 * (c // 2) + 8 * SEGS[0] * (c % 2)
NPRE = 3
F32, BF16 = jnp.float32, jnp.bfloat16
NT = (((1,), (1,)), ((), ()))


def _cmul(ar, ai, br, bi):
    return ar * br - ai * bi, ar * bi + ai * br


def _pk(x):
    return x.astype(BF16)


def _up(x):
    return x


def _seq(*gens):
    for g in gens:
        yield from g


def _take(g, n):
    for _ in range(n):
        next(g)
        yield


def _mix(*streams):
    pos = [0.0] * len(streams)
    live = set(range(len(streams)))
    while live:
        i = min(live, key=lambda a: (pos[a], a))
        try:
            next(streams[i][0])
            pos[i] += 1.0 / streams[i][1]
        except StopIteration:
            live.remove(i)


def _kernel(ax_h, wqkv_h, wo_h, bx_h, lre_h, lim_h, bre_h, bim_h, cre_h, cim_h, ldt_h, dsk_h,
            out_h,
            axv, wv, wov, bxv, bv, cv, pv0, pv1, pv2, pv3, prm, bcat, ccat, xb0, xb1, xb2, xb3, xl0, xl1, ub0, ub1, hb0, hb1,
            wt32, wtp, wo32, wop, xa32, xp, kext, vext, qb0, qb1, ob0, ob1, obuf, a3, oa24, isem, osem):
    xb32, xl, ubuf, hbuf = (xb0, xb1, xb2, xb3), (xl0, xl1), (ub0, ub1), (hb0, hb1)
    qbuf, ob = (qb0, qb1), (ob0, ob1)
    def cp(i, src, dst):
        return pltpu.make_async_copy(src, dst, isem.at[i])
    c_par = [cp(0, lre_h, pv0), cp(1, lim_h, pv1), cp(2, ldt_h, pv2), cp(3, dsk_h, pv3)]
    c_b = [cp(4, bre_h, bv.at[0]), cp(5, bim_h, bv.at[1])]
    c_c = [cp(6, cre_h, cv.at[0]), cp(7, cim_h, cv.at[1])]
    c_bx = [cp(8 + c, bx_h.at[:, pl.ds(c * T, T)], bxv.at[c]) for c in range(NC)]
    c_w, c_ax, c_wo = cp(8 + NC, wqkv_h, wv), cp(9 + NC, ax_h, axv), cp(10 + NC, wo_h, wov)
    for c in c_par + c_b + c_bx[:1] + c_c + c_bx[1:NPRE] + [c_w, c_ax, c_wo] + c_bx[NPRE:]:
        c.start()

    for c in c_par:
        c.wait()
    prm[...] = jnp.zeros(prm.shape, F32)
    for i in range(4):
        prm[i:i + 1, 0:D] = (pv0, pv1, pv2, pv3)[i][...].astype(F32).reshape(1, D)
    lane5 = lax.broadcasted_iota(jnp.int32, (8, 512), 1)
    lre = jnp.where(lane5 < D, jnp.broadcast_to(prm[0:1, :], (8, 512)), -1.0)
    lim = jnp.broadcast_to(prm[1:2, :], (8, 512))
    dt = jnp.exp(jnp.broadcast_to(prm[2:3, :], (8, 512))).astype(BF16).astype(F32)
    zr, zi = dt * lre, dt * lim
    mag = jnp.exp(zr)
    lr, li = mag * jnp.cos(zi), mag * jnp.sin(zi)
    den = lre * lre + lim * lim
    nr, ni = lr - 1.0, li
    cr = (nr * lre + ni * lim) / den
    ci = (ni * lre - nr * lim) / den
    lane1 = lax.broadcasted_iota(jnp.int32, (8, 128), 1)
    lo = lane1 < 64

    def tiles(r, i):
        r3, i3 = r[:, 384:], i[:, 384:]
        rr = jnp.where(lo, r3, pltpu.roll(r3, 64, 1))
        ii = jnp.where(lo, -i3, pltpu.roll(i3, 64, 1))
        return ([r[:, 128 * k:128 * k + 128] for k in range(3)] + [rr],
                [i[:, 128 * k:128 * k + 128] for k in range(3)] + [ii])
    lam = tiles(lr, li)
    sq = [(lr, li)]
    for _ in range(5):
        sq.append(_cmul(*sq[-1], *sq[-1]))
    pws = []
    for base in (_cmul(*sq[5], *sq[2]), _cmul(*_cmul(*sq[4], *sq[3]), *sq[2])):
        pw = []
        for _ in range(3):
            pw.append(tiles(*base))
            base = _cmul(*base, *base)
        pws.append(pw)
    dsk = pltpu.roll(jnp.broadcast_to(prm[3:4, :], (8, 512)), 64, 1)

    def cstep(m, k, a, b):
        if k < 3:
            return m[0][k] * a - m[1][k] * b, m[0][k] * b + m[1][k] * a
        return m[0][k] * a + m[1][k] * b, m[0][k] * b - m[1][k] * a

    for c in c_b:
        c.wait()
    zb = jnp.zeros((D, 64), BF16)
    b_re = jnp.concatenate([zb, bv[0]], axis=1)
    b_im = jnp.concatenate([zb, bv[1]], axis=1)
    bcat[0:384, :] = b_re[0:384]
    bcat[384:768, :] = b_im[0:384]
    bcat[768:832, :] = b_re[384:448]
    bcat[832:896, :] = b_im[384:448]

    def prep_c():
        for c in c_c:
            c.wait()
        c_re = cv[0].astype(F32)
        c_im = cv[1].astype(F32)
        c2r = (2.0 * (c_re * cr[0:1, :D] - c_im * ci[0:1, :D]))
        c2i = (-2.0 * (c_re * ci[0:1, :D] + c_im * cr[0:1, :D]))
        ccat[0:64, :] = jnp.zeros((64, 896), BF16)
        ccat[64:512, 0:384] = _pk(c2r[:, 0:384])
        ccat[64:512, 384:768] = _pk(c2i[:, 0:384])
        ccat[64:512, 768:896] = _pk(jnp.concatenate([c2r[:, 384:448], c2i[:, 384:448]], axis=1))

    sub = lax.broadcasted_iota(jnp.int32, (8, 128), 0)

    def ssm_t(c):
        if c < NPRE + 1:
            c_bx[c].wait()
        for k in range(4):
            if k == 0:
                xt = jnp.concatenate([jnp.zeros((64, T), F32), bxv[c, 0:64, :].astype(F32)], axis=0)
            else:
                xt = bxv[c, 128 * k - 64:128 * k + 64, :].astype(F32)
            xb32[c // 2][k, T * (c % 2):T * (c % 2) + T, :] = xt.T
            yield

    def xs(c, k, j):
        return xb32[c // 2][k, pl.ds(_row0(c) % 512 + j, 8, stride=SEGS[c % 2]), :]

    def ssm_x(c):
        for j2 in range(SEGS[c % 2] // 2):
            v = [jnp.concatenate([xs(c, k, j) for k in range(4)], axis=1) for j in (2 * j2, 2 * j2 + 1)]
            xl[c % 2][16 * j2:16 * j2 + 16, :] = _pk(jnp.concatenate(v, axis=0))
            if j2 % 4 == 3:
                yield

    def ssm_in(c):
        s = c % 2
        for n in range(7):
            ubuf[s][:, 128 * n:128 * n + 128] = lax.dot_general(
                _up(xl[s][...]), _up(bcat[128 * n:128 * n + 128, :]), NT, preferred_element_type=F32)
            yield

    def ssm_scan(c, carry):
        s = c % 2
        SEG, pw = SEGS[s], pws[s]

        def u(j, k):
            if k < 3:
                return (ubuf[s][8 * j:8 * j + 8, 128 * k:128 * k + 128],
                        ubuf[s][8 * j:8 * j + 8, 384 + 128 * k:512 + 128 * k])
            m = ubuf[s][8 * j:8 * j + 8, 768:896]
            return m, pltpu.roll(m, 64, 1)
        h = [u(0, k) for k in range(4)]
        for j in range(1, SEG):
            for k in range(4):
                a, b = cstep(lam, k, *h[k])
                ua, ub = u(j, k)
                h[k] = (a + ua, b + ub)
            if j % 2:
                yield
        for k in range(4):
            z = [jnp.where(sub == 0, carry[k][i], pltpu.roll(h[k][i], 1, 0)) for i in range(2)]
            for n in range(3):
                sh = 1 << n
                a, b = cstep(pw[n], k, *[jnp.where(sub >= sh, pltpu.roll(v, sh, 0), 0.0) for v in z])
                z = [z[0] + a, z[1] + b]
            h[k] = tuple(z)
        yield
        for j2 in range(SEG // 2):
            keep = []
            for j in (2 * j2, 2 * j2 + 1):
                for k in range(4):
                    a, b = cstep(lam, k, *h[k])
                    ua, ub = u(j, k)
                    h[k] = (a + ua, b + ub)
                keep.append(jnp.concatenate([h[0][0], h[1][0], h[2][0], h[0][1], h[1][1], h[2][1], h[3][0]], axis=1))
            hbuf[s][16 * j2:16 * j2 + 16, :] = _pk(jnp.concatenate(keep, axis=0))
            yield
        carry[:] = [tuple(jnp.broadcast_to(v[7:8], (8, 128)) for v in h[k]) for k in range(4)]

    def ssm_out(c):
        s = c % 2
        for k in range(4):
            y = lax.dot_general(_up(hbuf[s][...]), _up(ccat[128 * k:128 * k + 128, :]), NT,
                                preferred_element_type=F32)
            for j in range(SEGS[s]):
                rows = pl.ds(_row0(c) + j, 8, stride=SEGS[s])
                v = y[8 * j:8 * j + 8] + xs(c, k, j) * dsk[:, 128 * k:128 * k + 128]
                if k == 0 and c >= NPRE:
                    v = jnp.where(lo, a3[rows, :], v)
                obuf[k, rows, :] = v
            yield
        if c >= NPRE:
            for x in out_b(c):
                x.start()

    def out_b(c):
        return [pltpu.make_async_copy(obuf.at[k - 3, pl.ds(_row0(c), 8 * SEGS[c % 2])],
                                      out_h.at[pl.ds(_row0(c), 8 * SEGS[c % 2]), pl.ds(128 * k, 128)],
                                      osem.at[3 + 4 * c + k - 3]) for k in range(3, 7)]

    def att_prep():
        c_w.wait()
        for k in range(4):
            n = min(128, D - 128 * k)
            blk = wv[128 * k:128 * k + n, :].astype(F32)
            if n < 128:
                blk = jnp.concatenate([blk, jnp.zeros((128 - n, 3 * D), F32)], axis=0)
            wt32[k] = blk.T
            yield
        for g in (1, 2, 0):
            for d in range(DH):
                v = [jnp.concatenate([wt32[k, pl.ds(g * D + hh * 224 + d, 8, stride=DH), :]
                                      for k in range(4)], axis=1) for hh in range(2)]
                wtp[g * D + 16 * d:g * D + 16 * d + 16, :] = _pk(jnp.concatenate(v, axis=0))
                if d % 7 == 6:
                    yield
        c_ax.wait()
        for k in range(4):
            n = min(128, D - 128 * k)
            for t in range(4):
                blk = axv[128 * k:128 * k + n, 512 * t:512 * t + 512].astype(F32)
                if n < 128:
                    blk = jnp.concatenate([blk, jnp.zeros((128 - n, 512), F32)], axis=0)
                bt = blk.T
                for g in range(32):
                    r = XP * (32 * t + g)
                    xa32[k, r:r + 16, :] = bt[16 * g:16 * g + 16]
                yield
        c_wo.wait()
        wo = jnp.concatenate([wov[...].astype(F32), jnp.zeros((D, 64), F32)], axis=1)
        for k in range(4):
            wo32[k] = wo[:, 128 * k:128 * k + 128]
        yield
        for d in range(DH):
            v = [jnp.concatenate([wo32[k, pl.ds(hh * 224 + d, 8, stride=DH), :]
                                  for k in range(4)], axis=1) for hh in range(2)]
            wop[16 * d:16 * d + 16, :] = _pk(jnp.concatenate(v, axis=0))
            if d % 7 == 6:
                yield

    def att_kv(j):
        xj = jnp.concatenate([xa32[k, pl.ds(j, 128, stride=XP), :] for k in range(4)], axis=1).astype(BF16)
        xp[j] = xj
        for g, ext in ((1, kext), (2, vext)):
            r = lax.dot_general(_up(wtp[D * g:D * g + D, :]), xj, NT, preferred_element_type=F32)
            ext[j + 14] = r
            if j >= 2:
                ext[j - 2] = pltpu.roll(r, 1, 1)
            yield

    lane16 = lax.broadcasted_iota(jnp.int32, (16, 128), 1)
    scale = DH ** -0.5

    def att_q(j):
        for i in range(2):
            qbuf[j % 2][224 * i:224 * i + 224, :] = lax.dot_general(
                _up(wtp[224 * i:224 * i + 224, :]), _up(xp[j]), NT, preferred_element_type=F32)
            yield

    def att(j):
        lg = [None] * W
        for d in range(DH):
            qd = qbuf[j % 2][16 * d:16 * d + 16, :]
            for w in range(W):
                t = qd * kext[j + 14 - 2 * w, 16 * d:16 * d + 16, :]
                lg[w] = t if d == 0 else lg[w] + t
            if d % 4 == 3:
                yield
        for w in range(W):
            lg[w] = lg[w] * scale
            if j < 2 * w:
                lg[w] = jnp.where(lane16 == 0, -1e9, lg[w])
        m = lg[0]
        for w in range(1, W):
            m = jnp.maximum(m, lg[w])
        e = [jnp.exp(l - m) for l in lg]
        ssum = e[0]
        for w in range(1, W):
            ssum = ssum + e[w]
        inv = 1.0 / ssum
        p = [x * inv for x in e]
        yield
        for k in range(4):
            os_ = []
            for d in range(8 * k, min(8 * k + 8, DH)):
                acc = None
                for w in range(W):
                    t = p[w] * vext[j + 14 - 2 * w, 16 * d:16 * d + 16, :]
                    acc = t if acc is None else acc + t
                os_.append(acc)
                if d % 4 == 3 and d % 8 != 7:
                    yield
            if k == 3:
                os_.append(jnp.zeros((64, 128), F32))
            ob[j % 2][:, 128 * k:128 * k + 128] = _pk(jnp.concatenate(os_, axis=0).T)
            yield

    def att_o(j):
        for k in range(4):
            v = jnp.dot(_up(ob[j % 2][:, 0:D]), _up(wop[:, 128 * k:128 * k + 128]), preferred_element_type=F32)
            if k == 3:
                n = _row0(NPRE) // NJ
                old = obuf[0, pl.ds(j, n, stride=NJ), :]
                obuf[0, pl.ds(j, n, stride=NJ), :] = jnp.where(lo[0:1], v[:n], old)
                a3[pl.ds(j + 48 * NJ, 80, stride=NJ), :] = v[48:]
            else:
                oa24[k, pl.ds(j, 128, stride=NJ), :] = v
            yield

    z = jnp.zeros((8, 128), F32)
    carry = [(z, z)] * 4
    oa = [pltpu.make_async_copy(oa24.at[k], out_h.at[:, pl.ds(128 * k, 128)], osem.at[k]) for k in range(3)]
    N_X, N_IN, N_SC, N_OUT, N_PREP, N_ATT = 8, 7, 33, 4, 37, 16
    assert NPRE == 3

    def x_all(c):
        return _seq(ssm_t(c), ssm_t(c + 1), ssm_x(c)) if c % 2 == 0 else ssm_x(c)
    _mix((x_all(0), N_X))
    _mix((ssm_in(0), N_IN), (x_all(1), N_X))
    prep_c()
    _mix((ssm_in(1), N_IN), (ssm_scan(0, carry), N_SC), (x_all(2), N_X))
    _mix((_seq(ssm_out(0), ssm_in(2)), N_IN + N_OUT), (ssm_scan(1, carry), N_SC))
    pr_ = att_prep()
    _mix((ssm_out(1), N_OUT), (ssm_scan(2, carry), N_SC), (_take(pr_, 16), 16))
    _mix((ssm_out(2), N_OUT), (pr_, N_PREP - 16))
    for j in range(NJ):
        _mix((att_kv(j), 2))
    for c in c_bx[NPRE + 1:]:
        c.wait()
    _mix((att_q(0), 2))
    for j in range(NJ):
        mx = []
        if j + 1 < NJ:
            mx.append(att_q(j + 1))
        if j >= 1:
            mx.append(att_o(j - 1))
        extra = [(x_all(NPRE), N_X)] if j == NJ - 1 else []
        _mix((_seq(*mx), 6), (att(j), N_ATT), *extra)
    _mix((_seq(att_o(NJ - 1), ssm_in(NPRE)), 4 + N_IN), (x_all(NPRE + 1), N_X))
    for c in oa:
        c.start()
    for c in range(NPRE):
        for x in out_b(c):
            x.start()
    for c in range(NPRE, NC + 1):
        mx, n = [], 0
        if c + 1 < NC:
            mx.append(ssm_in(c + 1))
            n += N_IN
        if c - 1 >= NPRE:
            mx.append(ssm_out(c - 1))
            n += N_OUT
        st = [(_seq(*mx), n)]
        if c < NC:
            st.append((ssm_scan(c, carry), N_SC))
        if c + 2 < NC:
            st.append((x_all(c + 2), N_X))
        _mix(*st)
    for c in oa:
        c.wait()
    for c in range(NC):
        for x in out_b(c):
            x.wait()


@jax.jit
def pallas_concat_heads__sliding_local_dilated__ssm_conv_s5__prompt_kernel(
    A_x, A_wqkv, A_wo, B_x, B_Lambda_re, B_Lambda_im, B_B_re, B_B_im, B_C_re, B_C_im,
    B_log_dt, B_Dskip,
):
    hbm = pl.BlockSpec(memory_space=pltpu.HBM)
    out = pl.pallas_call(
        _kernel,
        out_shape=jax.ShapeDtypeStruct((S, 2 * D), F32),
        in_specs=[hbm] * 12,
        out_specs=hbm,
        scratch_shapes=[
            pltpu.VMEM((D, S), BF16),
            pltpu.VMEM((D, 3 * D), BF16),
            pltpu.VMEM((D, D), BF16),
            pltpu.VMEM((NC, D, T), BF16),
            pltpu.VMEM((2, D, D), BF16),
            pltpu.VMEM((2, D, D), BF16),
            *[pltpu.VMEM((D,), BF16)] * 4,
            pltpu.VMEM((8, 512), F32),
            pltpu.VMEM((896, 512), BF16),
            pltpu.VMEM((512, 896), BF16),
            *[pltpu.VMEM((4, 512, 128), F32)] * 4,
            *[pltpu.VMEM((8 * g, 512), BF16) for g in SEGS],
            *[pltpu.VMEM((8 * g, 896), F32) for g in SEGS],
            *[pltpu.VMEM((8 * g, 896), BF16) for g in SEGS],
            pltpu.VMEM((4, 3 * D, 128), F32),
            pltpu.VMEM((3 * D, 512), BF16),
            pltpu.VMEM((4, D, 128), F32),
            pltpu.VMEM((D, 512), BF16),
            pltpu.VMEM((4, 128 * XP, 128), F32),
            pltpu.VMEM((NJ, 128, 512), BF16),
            pltpu.VMEM((30, D, 128), F32),
            pltpu.VMEM((30, D, 128), F32),
            *[pltpu.VMEM((D, 128), F32)] * 2,
            *[pltpu.VMEM((128, 512), BF16)] * 2,
            pltpu.VMEM((4, S, 128), F32),
            pltpu.VMEM((S, 128), F32),
            pltpu.VMEM((3, S, 128), F32),
            pltpu.SemaphoreType.DMA((11 + NC,)),
            pltpu.SemaphoreType.DMA((3 + 4 * NC,)),
        ],
        compiler_params=pltpu.CompilerParams(vmem_limit_bytes=100 * 1024 * 1024),
    )(A_x[0].T, A_wqkv, A_wo, B_x[0].T, B_Lambda_re, B_Lambda_im,
      B_B_re, B_B_im, B_C_re, B_C_im, B_log_dt, B_Dskip)
    return out.reshape(1, S, 2 * D)
```

```python
import jax
import jax.numpy as jnp
from jax import lax
import jax.experimental.pallas as pl
import jax.experimental.pallas.tpu as pltpu

S, D, H, DH, W = 2048, 448, 16, 28, 8
NJ = 16
T = 256
NC = S // T
SEGS = (36, 28)
NQ, NB, LAG = 2, 4, 1
XP = 20


def _row0(c):
    return 512 * (c // 2) + 8 * SEGS[0] * (c % 2)
NPRE = 3
F32, BF16 = jnp.float32, jnp.bfloat16
NT = (((1,), (1,)), ((), ()))


def _cmul(ar, ai, br, bi):
    return ar * br - ai * bi, ar * bi + ai * br


def _pk(x):
    return x


def _up(x):
    return x


def _seq(*gens):
    for g in gens:
        yield from g


def _take(g, n):
    for _ in range(n):
        next(g)
        yield


def _mix(*streams):
    pos = [0.0] * len(streams)
    live = set(range(len(streams)))
    while live:
        i = min(live, key=lambda a: (pos[a], a))
        try:
            next(streams[i][0])
            pos[i] += 1.0 / streams[i][1]
        except StopIteration:
            live.remove(i)


def _kernel(ax_h, wqkv_h, wo_h, bx_h, lre_h, lim_h, bre_h, bim_h, cre_h, cim_h, ldt_h, dsk_h,
            out_h,
            axv, wv, wov, bxv, bv, cv, pv0, pv1, pv2, pv3, prm, bcat, ccat, xb0, xb1, xb2, xb3,
            wt32, wtp, wo32, wop, xa32, kext, vext, obuf, a3, oa24, isem, osem, *rest):
    xb32 = (xb0, xb1, xb2, xb3)
    ubuf, hbuf = rest[:NB], rest[NB:2 * NB]
    qbuf, ob = rest[2 * NB:2 * NB + NQ], rest[2 * NB + NQ:]
    def cp(i, src, dst):
        return pltpu.make_async_copy(src, dst, isem.at[i])
    c_par = [cp(0, lre_h, pv0), cp(1, lim_h, pv1), cp(2, ldt_h, pv2), cp(3, dsk_h, pv3)]
    c_b = [cp(4, bre_h, bv.at[0]), cp(5, bim_h, bv.at[1])]
    c_c = [cp(6, cre_h, cv.at[0]), cp(7, cim_h, cv.at[1])]
    c_bx = [cp(8 + c, bx_h.at[:, pl.ds(c * T, T)], bxv.at[c]) for c in range(NC)]
    c_w, c_ax, c_wo = cp(8 + NC, wqkv_h, wv), cp(9 + NC, ax_h, axv), cp(10 + NC, wo_h, wov)
    for c in c_par + c_b + c_bx[:1] + c_c + c_bx[1:NPRE] + [c_w, c_ax, c_wo] + c_bx[NPRE:]:
        c.start()

    for c in c_par:
        c.wait()
    prm[...] = jnp.zeros(prm.shape, F32)
    for i in range(4):
        prm[i:i + 1, 0:D] = (pv0, pv1, pv2, pv3)[i][...].astype(F32).reshape(1, D)
    lane5 = lax.broadcasted_iota(jnp.int32, (8, 512), 1)
    lre = jnp.where(lane5 < D, jnp.broadcast_to(prm[0:1, :], (8, 512)), -1.0)
    lim = jnp.broadcast_to(prm[1:2, :], (8, 512))
    dt = jnp.exp(jnp.broadcast_to(prm[2:3, :], (8, 512))).astype(BF16).astype(F32)
    zr, zi = dt * lre, dt * lim
    mag = jnp.exp(zr)
    lr, li = mag * jnp.cos(zi), mag * jnp.sin(zi)
    den = lre * lre + lim * lim
    nr, ni = lr - 1.0, li
    cr = (nr * lre + ni * lim) / den
    ci = (ni * lre - nr * lim) / den
    lane1 = lax.broadcasted_iota(jnp.int32, (8, 128), 1)
    lo = lane1 < 64

    def tiles(r, i):
        r3, i3 = r[:, 384:], i[:, 384:]
        rr = jnp.where(lo, r3, pltpu.roll(r3, 64, 1))
        ii = jnp.where(lo, -i3, pltpu.roll(i3, 64, 1))
        return ([r[:, 128 * k:128 * k + 128] for k in range(3)] + [rr],
                [i[:, 128 * k:128 * k + 128] for k in range(3)] + [ii])
    lam = tiles(lr, li)
    sq = [(lr, li)]
    for _ in range(5):
        sq.append(_cmul(*sq[-1], *sq[-1]))
    pws = []
    for base in (_cmul(*sq[5], *sq[2]), _cmul(*_cmul(*sq[4], *sq[3]), *sq[2])):
        pw = []
        for _ in range(3):
            pw.append(tiles(*base))
            base = _cmul(*base, *base)
        pws.append(pw)
    dsk = pltpu.roll(jnp.broadcast_to(prm[3:4, :], (8, 512)), 64, 1)

    def cstep(m, k, a, b):
        if k < 3:
            return m[0][k] * a - m[1][k] * b, m[0][k] * b + m[1][k] * a
        return m[0][k] * a + m[1][k] * b, m[0][k] * b - m[1][k] * a

    for c in c_b:
        c.wait()
    zb = jnp.zeros((D, 64), F32)
    b_re = jnp.concatenate([zb, bv[0].astype(F32)], axis=1)
    b_im = jnp.concatenate([zb, bv[1].astype(F32)], axis=1)
    bcat[0:384, :] = b_re[0:384]
    bcat[384:768, :] = b_im[0:384]
    bcat[768:832, :] = b_re[384:448]
    bcat[832:896, :] = b_im[384:448]

    def prep_c():
        for c in c_c:
            c.wait()
        c_re = cv[0].astype(F32)
        c_im = cv[1].astype(F32)
        c2r = (2.0 * (c_re * cr[0:1, :D] - c_im * ci[0:1, :D]))
        c2i = (-2.0 * (c_re * ci[0:1, :D] + c_im * cr[0:1, :D]))
        ccat[0:64, :] = jnp.zeros((64, 896), F32)
        ccat[64:512, 0:384] = _pk(c2r[:, 0:384])
        ccat[64:512, 384:768] = _pk(c2i[:, 0:384])
        ccat[64:512, 768:896] = _pk(jnp.concatenate([c2r[:, 384:448], c2i[:, 384:448]], axis=1))

    sub = lax.broadcasted_iota(jnp.int32, (8, 128), 0)

    def ssm_t(c):
        if c < NPRE + 1:
            c_bx[c].wait()
        for k in range(4):
            if k == 0:
                xt = jnp.concatenate([jnp.zeros((64, T), F32), bxv[c, 0:64, :].astype(F32)], axis=0)
            else:
                xt = bxv[c, 128 * k - 64:128 * k + 64, :].astype(F32)
            xb32[c // 2][k, T * (c % 2):T * (c % 2) + T, :] = xt.T
            yield

    def xs(c, k, j):
        return xb32[c // 2][k, pl.ds(_row0(c) % 512 + j, 8, stride=SEGS[c % 2]), :]

    def ssm_in(c):
        s = c % 2
        for n in range(7):
            ubuf[c % NB][:, 128 * n:128 * n + 128] = lax.dot_general(
                jnp.concatenate([jnp.concatenate([xs(c, k, j) for k in range(4)], axis=1)
                                 for j in range(SEGS[s])], axis=0), _up(bcat[128 * n:128 * n + 128, :]), NT, preferred_element_type=F32)
            yield

    def ssm_scan(c, carry):
        s = c % 2
        SEG, pw = SEGS[s], pws[s]

        def u(j, k):
            if k < 3:
                return (ubuf[c % NB][8 * j:8 * j + 8, 128 * k:128 * k + 128],
                        ubuf[c % NB][8 * j:8 * j + 8, 384 + 128 * k:512 + 128 * k])
            m = ubuf[c % NB][8 * j:8 * j + 8, 768:896]
            return m, pltpu.roll(m, 64, 1)
        h = [u(0, k) for k in range(4)]
        for j in range(1, SEG):
            for k in range(4):
                a, b = cstep(lam, k, *h[k])
                ua, ub = u(j, k)
                h[k] = (a + ua, b + ub)
            if j % 2:
                yield
        for k in range(4):
            z = [jnp.where(sub == 0, carry[k][i], pltpu.roll(h[k][i], 1, 0)) for i in range(2)]
            for n in range(3):
                sh = 1 << n
                a, b = cstep(pw[n], k, *[jnp.where(sub >= sh, pltpu.roll(v, sh, 0), 0.0) for v in z])
                z = [z[0] + a, z[1] + b]
            h[k] = tuple(z)
        yield
        for j2 in range(SEG // 2):
            keep = []
            for j in (2 * j2, 2 * j2 + 1):
                for k in range(4):
                    a, b = cstep(lam, k, *h[k])
                    ua, ub = u(j, k)
                    h[k] = (a + ua, b + ub)
                keep.append(jnp.concatenate([h[0][0], h[1][0], h[2][0], h[0][1], h[1][1], h[2][1], h[3][0]], axis=1))
            hbuf[c % NB][16 * j2:16 * j2 + 16, :] = _pk(jnp.concatenate(keep, axis=0))
            yield
        carry[:] = [tuple(jnp.broadcast_to(v[7:8], (8, 128)) for v in h[k]) for k in range(4)]

    def ssm_out(c):
        s = c % 2
        for k in range(4):
            y = lax.dot_general(_up(hbuf[c % NB][...]), _up(ccat[128 * k:128 * k + 128, :]), NT,
                                preferred_element_type=F32)
            for j in range(SEGS[s]):
                rows = pl.ds(_row0(c) + j, 8, stride=SEGS[s])
                v = y[8 * j:8 * j + 8] + xs(c, k, j) * dsk[:, 128 * k:128 * k + 128]
                if k == 0 and c >= NPRE:
                    v = jnp.where(lo, a3[rows, :], v)
                obuf[k, rows, :] = v
            yield
        if c >= NPRE:
            for x in out_b(c):
                x.start()

    def out_b(c):
        return [pltpu.make_async_copy(obuf.at[k - 3, pl.ds(_row0(c), 8 * SEGS[c % 2])],
                                      out_h.at[pl.ds(_row0(c), 8 * SEGS[c % 2]), pl.ds(128 * k, 128)],
                                      osem.at[3 + 4 * c + k - 3]) for k in range(3, 7)]

    def att_prep():
        c_w.wait()
        for k in range(4):
            n = min(128, D - 128 * k)
            blk = wv[128 * k:128 * k + n, :].astype(F32)
            if n < 128:
                blk = jnp.concatenate([blk, jnp.zeros((128 - n, 3 * D), F32)], axis=0)
            wt32[k] = blk.T
            yield
        for g in (1, 2, 0):
            for d in range(DH):
                v = [jnp.concatenate([wt32[k, pl.ds(g * D + hh * 224 + d, 8, stride=DH), :]
                                      for k in range(4)], axis=1) for hh in range(2)]
                wtp[g * D + 16 * d:g * D + 16 * d + 16, :] = _pk(jnp.concatenate(v, axis=0))
                if d % 7 == 6:
                    yield
        c_ax.wait()
        for k in range(4):
            n = min(128, D - 128 * k)
            for t in range(4):
                blk = axv[128 * k:128 * k + n, 512 * t:512 * t + 512].astype(F32)
                if n < 128:
                    blk = jnp.concatenate([blk, jnp.zeros((128 - n, 512), F32)], axis=0)
                bt = blk.T
                for g in range(32):
                    r = XP * (32 * t + g)
                    xa32[k, r:r + 16, :] = bt[16 * g:16 * g + 16]
                yield
        c_wo.wait()
        wo = jnp.concatenate([wov[...].astype(F32), jnp.zeros((D, 64), F32)], axis=1)
        for k in range(4):
            wo32[k] = wo[:, 128 * k:128 * k + 128]
        yield
        for d in range(DH):
            v = [jnp.concatenate([wo32[k, pl.ds(hh * 224 + d, 8, stride=DH), :]
                                  for k in range(4)], axis=1) for hh in range(2)]
            wop[16 * d:16 * d + 16, :] = _pk(jnp.concatenate(v, axis=0))
            if d % 7 == 6:
                yield

    def xa(j):
        return jnp.concatenate([xa32[k, pl.ds(j, 128, stride=XP), :] for k in range(4)], axis=1)

    def att_kv(j):
        xj = xa(j)
        for g, ext in ((1, kext), (2, vext)):
            r = lax.dot_general(_up(wtp[D * g:D * g + D, :]), xj, NT, preferred_element_type=F32)
            ext[j + 14] = r
            if j >= 2:
                ext[j - 2] = pltpu.roll(r, 1, 1)
            yield

    lane16 = lax.broadcasted_iota(jnp.int32, (16, 128), 1)
    scale = DH ** -0.5

    def att_q(j):
        for i in range(2):
            qbuf[j % NQ][224 * i:224 * i + 224, :] = lax.dot_general(
                _up(wtp[224 * i:224 * i + 224, :]), xa(j), NT, preferred_element_type=F32)
            yield

    def att(j):
        lg = [None] * W
        for d in range(DH):
            qd = qbuf[j % NQ][16 * d:16 * d + 16, :]
            for w in range(W):
                t = qd * kext[j + 14 - 2 * w, 16 * d:16 * d + 16, :]
                lg[w] = t if d == 0 else lg[w] + t
            if d % 4 == 3:
                yield
        for w in range(W):
            lg[w] = lg[w] * scale
            if j < 2 * w:
                lg[w] = jnp.where(lane16 == 0, -1e9, lg[w])
        m = lg[0]
        for w in range(1, W):
            m = jnp.maximum(m, lg[w])
        e = [jnp.exp(l - m) for l in lg]
        ssum = e[0]
        for w in range(1, W):
            ssum = ssum + e[w]
        inv = 1.0 / ssum
        p = [x * inv for x in e]
        yield
        for k in range(4):
            os_ = []
            for d in range(8 * k, min(8 * k + 8, DH)):
                acc = None
                for w in range(W):
                    t = p[w] * vext[j + 14 - 2 * w, 16 * d:16 * d + 16, :]
                    acc = t if acc is None else acc + t
                os_.append(acc)
                if d % 4 == 3 and d % 8 != 7:
                    yield
            if k == 3:
                os_.append(jnp.zeros((64, 128), F32))
            ob[(j // 2) % NQ][128 * (j % 2):128 * (j % 2) + 128, 128 * k:128 * k + 128] = _pk(jnp.concatenate(os_, axis=0).T)
            yield

    def att_o(jp):
        for k in range(4):
            vv = jnp.dot(ob[jp % NQ][:, 0:D], wop[:, 128 * k:128 * k + 128], preferred_element_type=F32)
            for i in range(2):
                j, v = 2 * jp + i, vv[128 * i:128 * i + 128]
                if k == 3:
                    n = _row0(NPRE) // NJ
                    old = obuf[0, pl.ds(j, n, stride=NJ), :]
                    obuf[0, pl.ds(j, n, stride=NJ), :] = jnp.where(lo[0:1], v[:n], old)
                    a3[pl.ds(j + 48 * NJ, 80, stride=NJ), :] = v[48:]
                else:
                    oa24[k, pl.ds(j, 128, stride=NJ), :] = v
            yield

    z = jnp.zeros((8, 128), F32)
    carry = [(z, z)] * 4
    oa = [pltpu.make_async_copy(oa24.at[k], out_h.at[:, pl.ds(128 * k, 128)], osem.at[k]) for k in range(3)]
    N_X, N_IN, N_SC, N_OUT, N_PREP, N_ATT = 8, 7, 33, 4, 37, 16
    assert NPRE == 3

    def x_all(c):
        return _seq(ssm_t(c), ssm_t(c + 1)) if c % 2 == 0 else _seq()
    _mix((x_all(0), N_X))
    _mix((ssm_in(0), N_IN), (x_all(1), N_X))
    prep_c()
    _mix((ssm_in(1), N_IN), (ssm_scan(0, carry), N_SC), (x_all(2), N_X))
    _mix((_seq(ssm_out(0), ssm_in(2)), N_IN + N_OUT), (ssm_scan(1, carry), N_SC))
    pr_ = att_prep()
    _mix((ssm_out(1), N_OUT), (ssm_scan(2, carry), N_SC), (_take(pr_, 16), 16))
    _mix((ssm_out(2), N_OUT), (pr_, N_PREP - 16))
    for j in range(NJ):
        _mix((att_kv(j), 2))
    for c in c_bx[NPRE + 1:]:
        c.wait()
    _mix((att_q(0), 2))
    for jp in range(NJ // 2):
        j = 2 * jp
        mx = [att_q(j + 1)]
        if jp >= 1:
            mx.append(att_o(jp - 1))
        if j + 2 < NJ:
            mx.append(att_q(j + 2))
        extra = [(x_all(NPRE), N_X)] if j == NJ - 2 else []
        _mix((_seq(*mx), 8), (_seq(att(j), att(j + 1)), 2 * N_ATT), *extra)
    _mix((_seq(ssm_in(NPRE), att_o(NJ // 2 - 1)), 4 + N_IN), (x_all(NPRE + 1), N_X))
    for c in oa:
        c.start()
    for c in range(NPRE):
        for x in out_b(c):
            x.start()
    for c in range(NPRE, NC + 1):
        mx, n = [], 0
        if c + 1 < NC:
            mx.append(ssm_in(c + 1))
            n += N_IN
        if c - 1 >= NPRE:
            mx.append(ssm_out(c - 1))
            n += N_OUT
        st = [(_seq(*mx), n)]
        if c < NC:
            st.append((ssm_scan(c, carry), N_SC))
        if c + 2 < NC:
            st.append((x_all(c + 2), N_X))
        _mix(*st)
    for c in oa:
        c.wait()
    for c in range(NC):
        for x in out_b(c):
            x.wait()


@jax.jit
def pallas_concat_heads__sliding_local_dilated__ssm_conv_s5__prompt_kernel(
    A_x, A_wqkv, A_wo, B_x, B_Lambda_re, B_Lambda_im, B_B_re, B_B_im, B_C_re, B_C_im,
    B_log_dt, B_Dskip,
):
    hbm = pl.BlockSpec(memory_space=pltpu.HBM)
    out = pl.pallas_call(
        _kernel,
        out_shape=jax.ShapeDtypeStruct((S, 2 * D), F32),
        in_specs=[hbm] * 12,
        out_specs=hbm,
        scratch_shapes=[
            pltpu.VMEM((D, S), BF16),
            pltpu.VMEM((D, 3 * D), BF16),
            pltpu.VMEM((D, D), BF16),
            pltpu.VMEM((NC, D, T), BF16),
            pltpu.VMEM((2, D, D), BF16),
            pltpu.VMEM((2, D, D), BF16),
            *[pltpu.VMEM((D,), BF16)] * 4,
            pltpu.VMEM((8, 512), F32),
            pltpu.VMEM((896, 512), F32),
            pltpu.VMEM((512, 896), F32),
            *[pltpu.VMEM((4, 512, 128), F32)] * 4,
            pltpu.VMEM((4, 3 * D, 128), F32),
            pltpu.VMEM((3 * D, 512), F32),
            pltpu.VMEM((4, D, 128), F32),
            pltpu.VMEM((D, 512), F32),
            pltpu.VMEM((4, 128 * XP, 128), F32),
            pltpu.VMEM((30, D, 128), F32),
            pltpu.VMEM((30, D, 128), F32),
            pltpu.VMEM((4, S, 128), F32),
            pltpu.VMEM((S, 128), F32),
            pltpu.VMEM((3, S, 128), F32),
            pltpu.SemaphoreType.DMA((11 + NC,)),
            pltpu.SemaphoreType.DMA((3 + 4 * NC,)),
            *[pltpu.VMEM((8 * SEGS[i % 2], 896), F32) for i in range(NB)],
            *[pltpu.VMEM((8 * SEGS[i % 2], 896), F32) for i in range(NB)],
            *[pltpu.VMEM((D, 128), F32)] * NQ,
            *[pltpu.VMEM((256, 512), F32)] * NQ,
        ],
        compiler_params=pltpu.CompilerParams(vmem_limit_bytes=100 * 1024 * 1024),
    )(A_x[0].T, A_wqkv, A_wo, B_x[0].T, B_Lambda_re, B_Lambda_im,
      B_B_re, B_B_im, B_C_re, B_C_im, B_log_dt, B_Dskip)
    return out.reshape(1, S, 2 * D)
```

```python
import jax
import jax.numpy as jnp
from jax import lax
import jax.experimental.pallas as pl
import jax.experimental.pallas.tpu as pltpu

S, D, H, DH, W = 2048, 448, 16, 28, 8
NJ = 16
T = 256
NC = S // T
SEGS = (36, 28)
NQ, NB, LAG = 4, 2, 1
JP = [(4 * (i // 2) + i % 2, 4 * (i // 2) + i % 2 + 2) for i in range(8)]
XP = 20


def _row0(c):
    return 512 * (c // 2) + 8 * SEGS[0] * (c % 2)
NPRE = 3
F32, BF16 = jnp.float32, jnp.bfloat16
NT = (((1,), (1,)), ((), ()))


def _cmul(ar, ai, br, bi):
    return ar * br - ai * bi, ar * bi + ai * br


def _pk(x):
    return x


def _up(x):
    return x


def _seq(*gens):
    for g in gens:
        yield from g


def _take(g, n):
    for _ in range(n):
        next(g)
        yield


def _mix(*streams):
    pos = [0.0] * len(streams)
    live = set(range(len(streams)))
    while live:
        i = min(live, key=lambda a: (pos[a], a))
        try:
            next(streams[i][0])
            pos[i] += 1.0 / streams[i][1]
        except StopIteration:
            live.remove(i)


def _kernel(ax_h, wqkv_h, wo_h, bx_h, lre_h, lim_h, bre_h, bim_h, cre_h, cim_h, ldt_h, dsk_h,
            out_h,
            axv, wv, wov, bxv, bv, cv, pv0, pv1, pv2, pv3, prm, bcat, ccat, xb0, xb1, xb2, xb3,
            wt32, wtp, wo32, wop, xa32, kext, vext, obuf, a3, oa24, isem, osem, *rest):
    xb32 = (xb0, xb1, xb2, xb3)
    ubuf, hbuf = rest[:NB], rest[NB:2 * NB]
    qbuf, ob = rest[2 * NB:2 * NB + NQ], rest[2 * NB + NQ:]
    def cp(i, src, dst):
        return pltpu.make_async_copy(src, dst, isem.at[i])
    c_par = [cp(0, lre_h, pv0), cp(1, lim_h, pv1), cp(2, ldt_h, pv2), cp(3, dsk_h, pv3)]
    c_b = [cp(4, bre_h, bv.at[0]), cp(5, bim_h, bv.at[1])]
    c_c = [cp(6, cre_h, cv.at[0]), cp(7, cim_h, cv.at[1])]
    c_bx = [cp(8 + c, bx_h.at[:, pl.ds(c * T, T)], bxv.at[c]) for c in range(NC)]
    c_w, c_ax, c_wo = cp(8 + NC, wqkv_h, wv), cp(9 + NC, ax_h, axv), cp(10 + NC, wo_h, wov)
    for c in c_par + c_b + c_bx[:2]:
        c.start()

    for c in c_par:
        c.wait()
    prm[...] = jnp.zeros(prm.shape, F32)
    for i in range(4):
        prm[i:i + 1, 0:D] = (pv0, pv1, pv2, pv3)[i][...].astype(F32).reshape(1, D)
    lane5 = lax.broadcasted_iota(jnp.int32, (8, 512), 1)
    lre = jnp.where(lane5 < D, jnp.broadcast_to(prm[0:1, :], (8, 512)), -1.0)
    lim = jnp.broadcast_to(prm[1:2, :], (8, 512))
    dt = jnp.exp(jnp.broadcast_to(prm[2:3, :], (8, 512))).astype(BF16).astype(F32)
    zr, zi = dt * lre, dt * lim
    mag = jnp.exp(zr)
    lr, li = mag * jnp.cos(zi), mag * jnp.sin(zi)
    den = lre * lre + lim * lim
    nr, ni = lr - 1.0, li
    cr = (nr * lre + ni * lim) / den
    ci = (ni * lre - nr * lim) / den
    lane1 = lax.broadcasted_iota(jnp.int32, (8, 128), 1)
    lo = lane1 < 64

    def tiles(r, i):
        r3, i3 = r[:, 384:], i[:, 384:]
        rr = jnp.where(lo, r3, pltpu.roll(r3, 64, 1))
        ii = jnp.where(lo, -i3, pltpu.roll(i3, 64, 1))
        return ([r[:, 128 * k:128 * k + 128] for k in range(3)] + [rr],
                [i[:, 128 * k:128 * k + 128] for k in range(3)] + [ii])
    lam = tiles(lr, li)
    sq = [(lr, li)]
    for _ in range(5):
        sq.append(_cmul(*sq[-1], *sq[-1]))
    pws = []
    for base in (_cmul(*sq[5], *sq[2]), _cmul(*_cmul(*sq[4], *sq[3]), *sq[2])):
        pw = []
        for _ in range(3):
            pw.append(tiles(*base))
            base = _cmul(*base, *base)
        pws.append(pw)
    dsk = pltpu.roll(jnp.broadcast_to(prm[3:4, :], (8, 512)), 64, 1)

    def cstep(m, k, a, b):
        if k < 3:
            return m[0][k] * a - m[1][k] * b, m[0][k] * b + m[1][k] * a
        return m[0][k] * a + m[1][k] * b, m[0][k] * b - m[1][k] * a

    for c in c_b + c_bx[:2]:
        c.wait()
    for c in c_c + c_bx[2:4]:
        c.start()
    zb = jnp.zeros((D, 64), F32)
    b_re = jnp.concatenate([zb, bv[0].astype(F32)], axis=1)
    b_im = jnp.concatenate([zb, bv[1].astype(F32)], axis=1)
    bcat[0:384, :] = b_re[0:384]
    bcat[384:768, :] = b_im[0:384]
    bcat[768:832, :] = b_re[384:448]
    bcat[832:896, :] = b_im[384:448]

    def prep_c():
        for c in c_c + c_bx[2:4]:
            c.wait()
        for c in (c_w, c_ax, c_wo):
            c.start()
        ccat[0:64, :] = jnp.zeros((64, 896), F32)
        cr3 = jnp.where(lo, cr[:, 384:], pltpu.roll(cr[:, 384:], 64, 1))[0:1]
        ci3 = jnp.where(lo, ci[:, 384:], pltpu.roll(ci[:, 384:], 64, 1))[0:1]
        for r in range(0, D, 32):
            c_re = cv[0, r:r + 32, :].astype(F32)
            c_im = cv[1, r:r + 32, :].astype(F32)
            c2r = 2.0 * (c_re * cr[0:1, :D] - c_im * ci[0:1, :D])
            c2i = -2.0 * (c_re * ci[0:1, :D] + c_im * cr[0:1, :D])
            ccat[64 + r:96 + r, 0:384] = c2r[:, 0:384]
            ccat[64 + r:96 + r, 384:768] = c2i[:, 0:384]
            ccat[64 + r:96 + r, 768:896] = jnp.concatenate([c2r[:, 384:448], c2i[:, 384:448]], axis=1)
            yield

    sub = lax.broadcasted_iota(jnp.int32, (8, 128), 0)

    def ssm_t(c):
        for k in range(4):
            if k == 0:
                xt = jnp.concatenate([jnp.zeros((64, T), F32), bxv[c, 0:64, :].astype(F32)], axis=0)
            else:
                xt = bxv[c, 128 * k - 64:128 * k + 64, :].astype(F32)
            xb32[c // 2][k, T * (c % 2):T * (c % 2) + T, :] = xt.T
            yield

    def xs(c, k, j):
        return xb32[c // 2][k, pl.ds(_row0(c) % 512 + j, 8, stride=SEGS[c % 2]), :]

    def ssm_in(c):
        s = c % 2
        for n in range(7):
            ubuf[c % NB][:, 128 * n:128 * n + 128] = lax.dot_general(
                jnp.concatenate([jnp.concatenate([xs(c, k, j) for k in range(4)], axis=1)
                                 for j in range(SEGS[s])], axis=0), _up(bcat[128 * n:128 * n + 128, :]), NT, preferred_element_type=F32)
            yield

    def ssm_scan(c, carry):
        s = c % 2
        SEG, pw = SEGS[s], pws[s]

        def u(j, k):
            if k < 3:
                return (ubuf[c % NB][8 * j:8 * j + 8, 128 * k:128 * k + 128],
                        ubuf[c % NB][8 * j:8 * j + 8, 384 + 128 * k:512 + 128 * k])
            m = ubuf[c % NB][8 * j:8 * j + 8, 768:896]
            return m, pltpu.roll(m, 64, 1)
        h = [u(0, k) for k in range(4)]
        for j in range(1, SEG):
            for k in range(4):
                a, b = cstep(lam, k, *h[k])
                ua, ub = u(j, k)
                h[k] = (a + ua, b + ub)
            if j % 2:
                yield
        for k in range(4):
            z = [jnp.where(sub == 0, carry[k][i], pltpu.roll(h[k][i], 1, 0)) for i in range(2)]
            for n in range(3):
                sh = 1 << n
                a, b = cstep(pw[n], k, *[jnp.where(sub >= sh, pltpu.roll(v, sh, 0), 0.0) for v in z])
                z = [z[0] + a, z[1] + b]
            h[k] = tuple(z)
        yield
        for j2 in range(SEG // 2):
            keep = []
            for j in (2 * j2, 2 * j2 + 1):
                for k in range(4):
                    a, b = cstep(lam, k, *h[k])
                    ua, ub = u(j, k)
                    h[k] = (a + ua, b + ub)
                keep.append(jnp.concatenate([h[0][0], h[1][0], h[2][0], h[0][1], h[1][1], h[2][1], h[3][0]], axis=1))
            hbuf[c % NB][16 * j2:16 * j2 + 16, :] = _pk(jnp.concatenate(keep, axis=0))
            yield
        carry[:] = [tuple(jnp.broadcast_to(v[7:8], (8, 128)) for v in h[k]) for k in range(4)]

    def ssm_out(c):
        s = c % 2
        for k in range(4):
            y = lax.dot_general(_up(hbuf[c % NB][...]), _up(ccat[128 * k:128 * k + 128, :]), NT,
                                preferred_element_type=F32)
            for j in range(SEGS[s]):
                rows = pl.ds(_row0(c) + j, 8, stride=SEGS[s])
                v = y[8 * j:8 * j + 8] + xs(c, k, j) * dsk[:, 128 * k:128 * k + 128]
                if k == 0 and c >= NPRE:
                    v = jnp.where(lo, a3[rows, :], v)
                obuf[k, rows, :] = v
            yield
        if c >= NPRE:
            for x in out_b(c):
                x.start()

    def out_b(c):
        return [pltpu.make_async_copy(obuf.at[k - 3, pl.ds(_row0(c), 8 * SEGS[c % 2])],
                                      out_h.at[pl.ds(_row0(c), 8 * SEGS[c % 2]), pl.ds(128 * k, 128)],
                                      osem.at[3 + 4 * c + k - 3]) for k in range(3, 7)]

    def att_prep():
        for c in (c_w, c_ax, c_wo):
            c.wait()
        for c in c_bx[4:]:
            c.start()
        for k in range(4):
            n = min(128, D - 128 * k)
            blk = wv[128 * k:128 * k + n, :].astype(F32)
            if n < 128:
                blk = jnp.concatenate([blk, jnp.zeros((128 - n, 3 * D), F32)], axis=0)
            wt32[k] = blk.T
            yield
        for g in (1, 2, 0):
            for d in range(DH):
                v = [jnp.concatenate([wt32[k, pl.ds(g * D + hh * 224 + d, 8, stride=DH), :]
                                      for k in range(4)], axis=1) for hh in range(2)]
                wtp[g * D + 16 * d:g * D + 16 * d + 16, :] = _pk(jnp.concatenate(v, axis=0))
                if d % 7 == 6:
                    yield
        for k in range(4):
            n = min(128, D - 128 * k)
            for t in range(4):
                blk = axv[128 * k:128 * k + n, 512 * t:512 * t + 512].astype(F32)
                if n < 128:
                    blk = jnp.concatenate([blk, jnp.zeros((128 - n, 512), F32)], axis=0)
                bt = blk.T
                for g in range(32):
                    r = XP * (32 * t + g)
                    xa32[k, r:r + 16, :] = bt[16 * g:16 * g + 16]
                yield
        wo = jnp.concatenate([wov[...].astype(F32), jnp.zeros((D, 64), F32)], axis=1)
        for k in range(4):
            wo32[k] = wo[:, 128 * k:128 * k + 128]
        yield
        for d in range(DH):
            v = [jnp.concatenate([wo32[k, pl.ds(hh * 224 + d, 8, stride=DH), :]
                                  for k in range(4)], axis=1) for hh in range(2)]
            wop[16 * d:16 * d + 16, :] = _pk(jnp.concatenate(v, axis=0))
            if d % 7 == 6:
                yield

    def xa(j):
        return jnp.concatenate([xa32[k, pl.ds(j, 128, stride=XP), :] for k in range(4)], axis=1)

    def att_kv(j):
        xj = xa(j)
        for g, ext in ((1, kext), (2, vext)):
            r = lax.dot_general(_up(wtp[D * g:D * g + D, :]), xj, NT, preferred_element_type=F32)
            ext[j + 14] = r
            if j >= 2:
                ext[j - 2] = pltpu.roll(r, 1, 1)
            yield

    lane16 = lax.broadcasted_iota(jnp.int32, (16, 128), 1)
    scale = DH ** -0.5

    def att_q(j):
        for i in range(2):
            qbuf[j % NQ][224 * i:224 * i + 224, :] = lax.dot_general(
                _up(wtp[224 * i:224 * i + 224, :]), xa(j), NT, preferred_element_type=F32)
            yield

    def att(jp):
        js = JP[jp]
        P = {}
        for hh in range(2):
            lg = {}
            for d in range(DH):
                r = slice(16 * d + 8 * hh, 16 * d + 8 * hh + 8)
                kk = {e: kext[e, r, :] for e in range(js[0], js[1] + 15, 2)}
                for j in js:
                    qd = qbuf[j % NQ][r, :]
                    for w in range(W):
                        t = qd * kk[j + 14 - 2 * w]
                        lg[j, w] = t if d == 0 else lg[j, w] + t
                if d % 4 == 3:
                    yield
            for j in js:
                l = [lg[j, w] * scale for w in range(W)]
                l = [jnp.where(lane1 == 0, -1e9, l[w]) if j < 2 * w else l[w] for w in range(W)]
                m = l[0]
                for w in range(1, W):
                    m = jnp.maximum(m, l[w])
                e = [jnp.exp(x - m) for x in l]
                ssum = e[0]
                for w in range(1, W):
                    ssum = ssum + e[w]
                inv = 1.0 / ssum
                P[hh, j] = [x * inv for x in e]
            yield
        for k in range(4):
            os_ = {j: [] for j in js}
            for d in range(8 * k, min(8 * k + 8, DH)):
                for hh in range(2):
                    r = slice(16 * d + 8 * hh, 16 * d + 8 * hh + 8)
                    vv = {e: vext[e, r, :] for e in range(js[0], js[1] + 15, 2)}
                    for j in js:
                        acc = None
                        for w in range(W):
                            t = P[hh, j][w] * vv[j + 14 - 2 * w]
                            acc = t if acc is None else acc + t
                        os_[j].append(acc)
                if d % 2 == 1:
                    yield
            for i, j in enumerate(js):
                if k == 3:
                    os_[j].append(jnp.zeros((64, 128), F32))
                ob[jp % 2][128 * i:128 * i + 128, 128 * k:128 * k + 128] = jnp.concatenate(os_[j], axis=0).T

    def att_o(jp):
        for k in range(4):
            vv = jnp.dot(ob[jp % 2][:, 0:D], wop[:, 128 * k:128 * k + 128], preferred_element_type=F32)
            for i in range(2):
                j, v = JP[jp][i], vv[128 * i:128 * i + 128]
                if k == 3:
                    n = _row0(NPRE) // NJ
                    old = obuf[0, pl.ds(j, n, stride=NJ), :]
                    obuf[0, pl.ds(j, n, stride=NJ), :] = jnp.where(lo[0:1], v[:n], old)
                    a3[pl.ds(j + 48 * NJ, 80, stride=NJ), :] = v[48:]
                else:
                    oa24[k, pl.ds(j, 128, stride=NJ), :] = v
            yield

    z = jnp.zeros((8, 128), F32)
    carry = [(z, z)] * 4
    oa = [pltpu.make_async_copy(oa24.at[k], out_h.at[:, pl.ds(128 * k, 128)], osem.at[k]) for k in range(3)]
    N_X, N_IN, N_SC, N_OUT, N_PREP, N_ATT = 8, 7, 33, 4, 37, 16
    assert NPRE == 3

    def x_all(c):
        return _seq(ssm_t(c), ssm_t(c + 1)) if c % 2 == 0 else _seq()
    _mix((x_all(0), N_X))
    _mix((ssm_in(0), N_IN), (x_all(1), N_X))
    _mix((prep_c(), 14), (ssm_in(1), N_IN), (ssm_scan(0, carry), N_SC), (x_all(2), N_X))
    _mix((_seq(ssm_out(0), ssm_in(2)), N_IN + N_OUT), (ssm_scan(1, carry), N_SC))
    pr_ = att_prep()
    _mix((ssm_out(1), N_OUT), (ssm_scan(2, carry), N_SC), (_take(pr_, 16), 16))
    _mix((ssm_out(2), N_OUT), (pr_, N_PREP - 16))
    for j in range(NJ):
        _mix((att_kv(j), 2))
    for c in c_bx[NPRE + 1:]:
        c.wait()
    _mix((_seq(att_q(0), att_q(2)), 2))
    for jp in range(NJ // 2):
        mx = []
        if jp + 1 < NJ // 2:
            mx += [att_q(j) for j in JP[jp + 1]]
        if jp >= 1:
            mx.append(att_o(jp - 1))
        extra = [(x_all(NPRE), N_X)] if jp == NJ // 2 - 1 else []
        _mix((_seq(*mx), 8), (att(jp), 30), *extra)
    _mix((_seq(ssm_in(NPRE), att_o(NJ // 2 - 1)), 4 + N_IN), (x_all(NPRE + 1), N_X))
    for c in oa:
        c.start()
    for c in range(NPRE):
        for x in out_b(c):
            x.start()
    for c in range(NPRE, NC + 1):
        mx, n = [], 0
        if c + 1 < NC:
            mx.append(ssm_in(c + 1))
            n += N_IN
        if c - 1 >= NPRE:
            mx.append(ssm_out(c - 1))
            n += N_OUT
        st = [(_seq(*mx), n)]
        if c < NC:
            st.append((ssm_scan(c, carry), N_SC))
        if c + 2 < NC:
            st.append((x_all(c + 2), N_X))
        _mix(*st)
    for c in oa:
        c.wait()
    for c in range(NC):
        for x in out_b(c):
            x.wait()


@jax.jit
def pallas_concat_heads__sliding_local_dilated__ssm_conv_s5__prompt_kernel(
    A_x, A_wqkv, A_wo, B_x, B_Lambda_re, B_Lambda_im, B_B_re, B_B_im, B_C_re, B_C_im,
    B_log_dt, B_Dskip,
):
    hbm = pl.BlockSpec(memory_space=pltpu.HBM)
    out = pl.pallas_call(
        _kernel,
        out_shape=jax.ShapeDtypeStruct((S, 2 * D), F32),
        in_specs=[hbm] * 12,
        out_specs=hbm,
        scratch_shapes=[
            pltpu.VMEM((D, S), BF16),
            pltpu.VMEM((D, 3 * D), BF16),
            pltpu.VMEM((D, D), BF16),
            pltpu.VMEM((NC, D, T), BF16),
            pltpu.VMEM((2, D, D), BF16),
            pltpu.VMEM((2, D, D), BF16),
            *[pltpu.VMEM((D,), BF16)] * 4,
            pltpu.VMEM((8, 512), F32),
            pltpu.VMEM((896, 512), F32),
            pltpu.VMEM((512, 896), F32),
            *[pltpu.VMEM((4, 512, 128), F32)] * 4,
            pltpu.VMEM((4, 3 * D, 128), F32),
            pltpu.VMEM((3 * D, 512), F32),
            pltpu.VMEM((4, D, 128), F32),
            pltpu.VMEM((D, 512), F32),
            pltpu.VMEM((4, 128 * XP, 128), F32),
            pltpu.VMEM((30, D, 128), F32),
            pltpu.VMEM((30, D, 128), F32),
            pltpu.VMEM((4, S, 128), F32),
            pltpu.VMEM((S, 128), F32),
            pltpu.VMEM((3, S, 128), F32),
            pltpu.SemaphoreType.DMA((11 + NC,)),
            pltpu.SemaphoreType.DMA((3 + 4 * NC,)),
            *[pltpu.VMEM((8 * SEGS[i % 2], 896), F32) for i in range(NB)],
            *[pltpu.VMEM((8 * SEGS[i % 2], 896), F32) for i in range(NB)],
            *[pltpu.VMEM((D, 128), F32)] * NQ,
            *[pltpu.VMEM((256, 512), F32)] * 2,
        ],
        compiler_params=pltpu.CompilerParams(vmem_limit_bytes=100 * 1024 * 1024),
    )(A_x[0].T, A_wqkv, A_wo, B_x[0].T, B_Lambda_re, B_Lambda_im,
      B_B_re, B_B_im, B_C_re, B_C_im, B_log_dt, B_Dskip)
    return out.reshape(1, S, 2 * D)
```

```python
import jax
import jax.numpy as jnp
from jax import lax
import jax.experimental.pallas as pl
import jax.experimental.pallas.tpu as pltpu

S, D, H, DH, W = 2048, 448, 16, 28, 8
NJ = 16
T = 256
NC = S // T
SEGS = (28, 36)
NQ, NB, LAG = 4, 2, 1
JP = [(4 * (i // 2) + i % 2, 4 * (i // 2) + i % 2 + 2) for i in range(8)]
XP = 20


def _row0(c):
    return 512 * (c // 2) + 8 * SEGS[0] * (c % 2)
NPRE = 3
F32, BF16 = jnp.float32, jnp.bfloat16
NT = (((1,), (1,)), ((), ()))


def _cmul(ar, ai, br, bi):
    return ar * br - ai * bi, ar * bi + ai * br


def _pk(x):
    return x


def _up(x):
    return x


def _seq(*gens):
    for g in gens:
        yield from g


def _take(g, n):
    for _ in range(n):
        next(g)
        yield


def _mix(*streams):
    pos = [0.0] * len(streams)
    live = set(range(len(streams)))
    while live:
        i = min(live, key=lambda a: (pos[a], a))
        try:
            next(streams[i][0])
            pos[i] += 1.0 / streams[i][1]
        except StopIteration:
            live.remove(i)


def _kernel(ax_h, wqkv_h, wo_h, bx_h, lre_h, lim_h, bre_h, bim_h, cre_h, cim_h, ldt_h, dsk_h,
            out_h,
            axv, wv, wov, bxv, bv, cv, pv0, pv1, pv2, pv3, prm, bcat, ccat, xb0, xb1, xb2, xb3,
            wt32, wtp, wo32, wop, xa32, kext, vext, obuf, a3, oa24, isem, osem, *rest):
    xb32 = (xb0, xb1, xb2, xb3)
    ubuf, hbuf = rest[:NB], rest[NB:2 * NB]
    qbuf, ob = rest[2 * NB:2 * NB + NQ], rest[2 * NB + NQ:]
    def cp(i, src, dst):
        return pltpu.make_async_copy(src, dst, isem.at[i])
    c_par = [cp(0, lre_h, pv0), cp(1, lim_h, pv1), cp(2, ldt_h, pv2), cp(3, dsk_h, pv3)]
    c_b = [cp(4, bre_h, bv.at[0]), cp(5, bim_h, bv.at[1])]
    c_c = [cp(6, cre_h, cv.at[0]), cp(7, cim_h, cv.at[1])]
    c_bx = [cp(8 + c, bx_h.at[:, pl.ds(c * T, T)], bxv.at[c]) for c in range(NC)]
    c_w, c_ax, c_wo = cp(8 + NC, wqkv_h, wv), cp(9 + NC, ax_h, axv), cp(10 + NC, wo_h, wov)
    for c in c_bx[:1] + c_b[:1] + c_par + c_b[1:]:
        c.start()

    for c in c_par:
        c.wait()
    prm[...] = jnp.zeros(prm.shape, F32)
    for i in range(4):
        prm[i:i + 1, 0:D] = (pv0, pv1, pv2, pv3)[i][...].astype(F32).reshape(1, D)
    lane5 = lax.broadcasted_iota(jnp.int32, (8, 512), 1)
    lre = jnp.where(lane5 < D, jnp.broadcast_to(prm[0:1, :], (8, 512)), -1.0)
    lim = jnp.broadcast_to(prm[1:2, :], (8, 512))
    dt = jnp.exp(jnp.broadcast_to(prm[2:3, :], (8, 512))).astype(BF16).astype(F32)
    zr, zi = dt * lre, dt * lim
    mag = jnp.exp(zr)
    lr, li = mag * jnp.cos(zi), mag * jnp.sin(zi)
    den = lre * lre + lim * lim
    nr, ni = lr - 1.0, li
    cr = (nr * lre + ni * lim) / den
    ci = (ni * lre - nr * lim) / den
    lane1 = lax.broadcasted_iota(jnp.int32, (8, 128), 1)
    lo = lane1 < 64

    def tiles(r, i):
        r3, i3 = r[:, 384:], i[:, 384:]
        rr = jnp.where(lo, r3, pltpu.roll(r3, 64, 1))
        ii = jnp.where(lo, -i3, pltpu.roll(i3, 64, 1))
        return ([r[:, 128 * k:128 * k + 128] for k in range(3)] + [rr],
                [i[:, 128 * k:128 * k + 128] for k in range(3)] + [ii])
    lam = tiles(lr, li)
    sq = [(lr, li)]
    for _ in range(5):
        sq.append(_cmul(*sq[-1], *sq[-1]))
    pws = []
    for base in (_cmul(*_cmul(*sq[4], *sq[3]), *sq[2]), _cmul(*sq[5], *sq[2])):
        pw = []
        for _ in range(3):
            pw.append(tiles(*base))
            base = _cmul(*base, *base)
        pws.append(pw)
    dsk = pltpu.roll(jnp.broadcast_to(prm[3:4, :], (8, 512)), 64, 1)

    def cstep(m, k, a, b):
        if k < 3:
            return m[0][k] * a - m[1][k] * b, m[0][k] * b + m[1][k] * a
        return m[0][k] * a + m[1][k] * b, m[0][k] * b - m[1][k] * a

    def prep_b(i):
        c_b[i].wait()
        for r in range(0, D, 64):
            v = jnp.concatenate([jnp.zeros((64, 64), F32), bv[i, r:r + 64, :].astype(F32)], axis=1)
            r2 = 384 * i + r if r < 384 else 768 + 64 * i
            bcat[r2:r2 + 64, :] = v

    def prep_c():
        for c in c_c:
            c.wait()
        for c in (c_w, c_ax):
            c.start()
        ccat[0:64, :] = jnp.zeros((64, 896), F32)
        cr3 = jnp.where(lo, cr[:, 384:], pltpu.roll(cr[:, 384:], 64, 1))[0:1]
        ci3 = jnp.where(lo, ci[:, 384:], pltpu.roll(ci[:, 384:], 64, 1))[0:1]
        for r in range(0, D, 32):
            c_re = cv[0, r:r + 32, :].astype(F32)
            c_im = cv[1, r:r + 32, :].astype(F32)
            c2r = 2.0 * (c_re * cr[0:1, :D] - c_im * ci[0:1, :D])
            c2i = -2.0 * (c_re * ci[0:1, :D] + c_im * cr[0:1, :D])
            ccat[64 + r:96 + r, 0:384] = c2r[:, 0:384]
            ccat[64 + r:96 + r, 384:768] = c2i[:, 0:384]
            ccat[64 + r:96 + r, 768:896] = jnp.concatenate([c2r[:, 384:448], c2i[:, 384:448]], axis=1)
            yield

    sub = lax.broadcasted_iota(jnp.int32, (8, 128), 0)

    def ssm_t(c):
        for k in range(4):
            if k == 0:
                xt = jnp.concatenate([jnp.zeros((64, T), F32), bxv[c, 0:64, :].astype(F32)], axis=0)
            else:
                xt = bxv[c, 128 * k - 64:128 * k + 64, :].astype(F32)
            xb32[c // 2][k, T * (c % 2):T * (c % 2) + T, :] = xt.T
            yield

    def xs(c, k, j):
        return xb32[c // 2][k, pl.ds(_row0(c) % 512 + j, 8, stride=SEGS[c % 2]), :]

    def ssm_in(c):
        s = c % 2
        for n in range(7):
            ubuf[c % NB][:, 128 * n:128 * n + 128] = lax.dot_general(
                jnp.concatenate([jnp.concatenate([xs(c, k, j) for k in range(4)], axis=1)
                                 for j in range(SEGS[s])], axis=0), _up(bcat[128 * n:128 * n + 128, :]), NT, preferred_element_type=F32)
            yield

    def ssm_scan(c, carry):
        s = c % 2
        SEG, pw = SEGS[s], pws[s]

        def u(j, k):
            if k < 3:
                return (ubuf[c % NB][8 * j:8 * j + 8, 128 * k:128 * k + 128],
                        ubuf[c % NB][8 * j:8 * j + 8, 384 + 128 * k:512 + 128 * k])
            m = ubuf[c % NB][8 * j:8 * j + 8, 768:896]
            return m, pltpu.roll(m, 64, 1)
        h = [u(0, k) for k in range(4)]
        for j in range(1, SEG):
            for k in range(4):
                a, b = cstep(lam, k, *h[k])
                ua, ub = u(j, k)
                h[k] = (a + ua, b + ub)
            if j % 2:
                yield
        for k in range(4):
            z = [jnp.where(sub == 0, carry[k][i], pltpu.roll(h[k][i], 1, 0)) for i in range(2)]
            for n in range(3):
                sh = 1 << n
                a, b = cstep(pw[n], k, *[jnp.where(sub >= sh, pltpu.roll(v, sh, 0), 0.0) for v in z])
                z = [z[0] + a, z[1] + b]
            h[k] = tuple(z)
        yield
        for j2 in range(SEG // 2):
            keep = []
            for j in (2 * j2, 2 * j2 + 1):
                for k in range(4):
                    a, b = cstep(lam, k, *h[k])
                    ua, ub = u(j, k)
                    h[k] = (a + ua, b + ub)
                keep.append(jnp.concatenate([h[0][0], h[1][0], h[2][0], h[0][1], h[1][1], h[2][1], h[3][0]], axis=1))
            hbuf[c % NB][16 * j2:16 * j2 + 16, :] = _pk(jnp.concatenate(keep, axis=0))
            yield
        carry[:] = [tuple(jnp.broadcast_to(v[7:8], (8, 128)) for v in h[k]) for k in range(4)]

    def ssm_out(c):
        s = c % 2
        for k in range(4):
            y = lax.dot_general(_up(hbuf[c % NB][...]), _up(ccat[128 * k:128 * k + 128, :]), NT,
                                preferred_element_type=F32)
            for j in range(SEGS[s]):
                rows = pl.ds(_row0(c) + j, 8, stride=SEGS[s])
                v = y[8 * j:8 * j + 8] + xs(c, k, j) * dsk[:, 128 * k:128 * k + 128]
                if k == 0 and c >= NPRE:
                    v = jnp.where(lo, a3[rows, :], v)
                obuf[k, rows, :] = v
            if c == NC - 1:
                out_b(c)[k].start()
            yield
        if NPRE <= c < NC - 1:
            for x in out_b(c):
                x.start()

    def out_b(c):
        return [pltpu.make_async_copy(obuf.at[k - 3, pl.ds(_row0(c), 8 * SEGS[c % 2])],
                                      out_h.at[pl.ds(_row0(c), 8 * SEGS[c % 2]), pl.ds(128 * k, 128)],
                                      osem.at[3 + 4 * c + k - 3]) for k in range(3, 7)]

    def att_prep():
        c_w.wait()
        for k in range(4):
            n = min(128, D - 128 * k)
            blk = wv[128 * k:128 * k + n, :].astype(F32)
            if n < 128:
                blk = jnp.concatenate([blk, jnp.zeros((128 - n, 3 * D), F32)], axis=0)
            wt32[k] = blk.T
            yield
        for g in (1, 2, 0):
            for d in range(DH):
                v = [jnp.concatenate([wt32[k, pl.ds(g * D + hh * 224 + d, 8, stride=DH), :]
                                      for k in range(4)], axis=1) for hh in range(2)]
                wtp[g * D + 16 * d:g * D + 16 * d + 16, :] = _pk(jnp.concatenate(v, axis=0))
                if d % 7 == 6:
                    yield
        c_ax.wait()
        for c in [c_wo] + c_bx[4:]:
            c.start()
        for k in range(4):
            n = min(128, D - 128 * k)
            for t in range(4):
                blk = axv[128 * k:128 * k + n, 512 * t:512 * t + 512].astype(F32)
                if n < 128:
                    blk = jnp.concatenate([blk, jnp.zeros((128 - n, 512), F32)], axis=0)
                bt = blk.T
                for g in range(32):
                    r = XP * (32 * t + g)
                    xa32[k, r:r + 16, :] = bt[16 * g:16 * g + 16]
                yield

    def wo_prep():
        c_wo.wait()
        for c in c_bx[4:]:
            c.wait()
        wo = jnp.concatenate([wov[...].astype(F32), jnp.zeros((D, 64), F32)], axis=1)
        for k in range(4):
            wo32[k] = wo[:, 128 * k:128 * k + 128]
        yield
        for d in range(DH):
            v = [jnp.concatenate([wo32[k, pl.ds(hh * 224 + d, 8, stride=DH), :]
                                  for k in range(4)], axis=1) for hh in range(2)]
            wop[16 * d:16 * d + 16, :] = _pk(jnp.concatenate(v, axis=0))
            if d % 7 == 6:
                yield

    def xa(j):
        return jnp.concatenate([xa32[k, pl.ds(j, 128, stride=XP), :] for k in range(4)], axis=1)

    def att_kv(j):
        xj = xa(j)
        for g, ext in ((1, kext), (2, vext)):
            r = lax.dot_general(_up(wtp[D * g:D * g + D, :]), xj, NT, preferred_element_type=F32)
            ext[j + 14] = r
            if j >= 2:
                ext[j - 2] = pltpu.roll(r, 1, 1)
            yield

    lane16 = lax.broadcasted_iota(jnp.int32, (16, 128), 1)
    scale = DH ** -0.5

    def att_q(j):
        for i in range(2):
            qbuf[j % NQ][224 * i:224 * i + 224, :] = lax.dot_general(
                _up(wtp[224 * i:224 * i + 224, :]), xa(j), NT, preferred_element_type=F32)
            yield

    def att(jp):
        js = JP[jp]
        P = {}
        for hh in range(2):
            lg = {}
            for d in range(DH):
                r = slice(16 * d + 8 * hh, 16 * d + 8 * hh + 8)
                kk = {e: kext[e, r, :] for e in range(js[0], js[1] + 15, 2)}
                for j in js:
                    qd = qbuf[j % NQ][r, :]
                    for w in range(W):
                        t = qd * kk[j + 14 - 2 * w]
                        lg[j, w] = t if d == 0 else lg[j, w] + t
                if d % 4 == 3:
                    yield
            for j in js:
                l = [lg[j, w] * scale for w in range(W)]
                l = [jnp.where(lane1 == 0, -1e9, l[w]) if j < 2 * w else l[w] for w in range(W)]
                m = l[0]
                for w in range(1, W):
                    m = jnp.maximum(m, l[w])
                e = [jnp.exp(x - m) for x in l]
                ssum = e[0]
                for w in range(1, W):
                    ssum = ssum + e[w]
                inv = 1.0 / ssum
                P[hh, j] = [x * inv for x in e]
            yield
        for k in range(4):
            os_ = {j: [] for j in js}
            for d in range(8 * k, min(8 * k + 8, DH)):
                for hh in range(2):
                    r = slice(16 * d + 8 * hh, 16 * d + 8 * hh + 8)
                    vv = {e: vext[e, r, :] for e in range(js[0], js[1] + 15, 2)}
                    for j in js:
                        acc = None
                        for w in range(W):
                            t = P[hh, j][w] * vv[j + 14 - 2 * w]
                            acc = t if acc is None else acc + t
                        os_[j].append(acc)
                if d % 2 == 1:
                    yield
            for i, j in enumerate(js):
                if k == 3:
                    os_[j].append(jnp.zeros((64, 128), F32))
                ob[jp % 2][128 * i:128 * i + 128, 128 * k:128 * k + 128] = jnp.concatenate(os_[j], axis=0).T

    def att_o(jp):
        for k in range(4):
            vv = jnp.dot(ob[jp % 2][:, 0:D], wop[:, 128 * k:128 * k + 128], preferred_element_type=F32)
            for i in range(2):
                j, v = JP[jp][i], vv[128 * i:128 * i + 128]
                if k == 3:
                    n = _row0(NPRE) // NJ
                    old = obuf[0, pl.ds(j, n, stride=NJ), :]
                    obuf[0, pl.ds(j, n, stride=NJ), :] = jnp.where(lo[0:1], v[:n], old)
                    m = n // 8 * 8
                    a3[pl.ds(j + m * NJ, 128 - m, stride=NJ), :] = v[m:]
                else:
                    oa24[k, pl.ds(j, 128, stride=NJ), :] = v
            yield

    z = jnp.zeros((8, 128), F32)
    carry = [(z, z)] * 4
    oa = [pltpu.make_async_copy(oa24.at[k], out_h.at[:, pl.ds(128 * k, 128)], osem.at[k]) for k in range(3)]
    N_X, N_IN, N_SC, N_OUT, N_PREP, N_ATT = 8, 7, 33, 4, 37, 16
    assert NPRE == 3

    def x_all(c):
        return _seq(ssm_t(c), ssm_t(c + 1)) if c % 2 == 0 else _seq()
    def call(f, *a):
        f(*a)
        yield

    c_bx[0].wait()
    prep_b(0)
    for c in c_bx[1:2] + c_c:
        c.start()
    _mix((ssm_t(0), 4))
    in0 = ssm_in(0)
    _mix((_take(in0, 2), 2))
    prep_b(1)
    c_bx[1].wait()
    for c in c_bx[2:4]:
        c.start()
    _mix((in0, 5), (ssm_t(1), 4))
    in1, sc0 = ssm_in(1), ssm_scan(0, carry)
    _mix((_take(in1, 2), 2), (_take(sc0, 10), 10))
    c_bx[2].wait()
    c_bx[3].wait()
    _mix((prep_c(), 14), (in1, 5), (sc0, N_SC - 10), (x_all(2), N_X))
    _mix((_seq(ssm_out(0), ssm_in(2)), N_IN + N_OUT), (ssm_scan(1, carry), N_SC))
    pr_ = att_prep()
    _mix((ssm_out(1), N_OUT), (ssm_scan(2, carry), N_SC), (_take(pr_, 16), 16))
    _mix((ssm_out(2), N_OUT), (pr_, 16))
    for j in range(NJ - 2):
        _mix((att_kv(j), 2))
    _mix((wo_prep(), 5), (_seq(att_kv(NJ - 2), att_kv(NJ - 1)), 4))
    _mix((_seq(att_q(0), att_q(2)), 2))
    for jp in range(NJ // 2):
        mx = []
        if jp + 1 < NJ // 2:
            mx += [att_q(j) for j in JP[jp + 1]]
        if jp >= 1:
            mx.append(att_o(jp - 1))
        extra = [(x_all(NPRE), N_X)] if jp == NJ // 2 - 1 else []
        _mix((_seq(*mx), 8), (att(jp), 30), *extra)
    _mix((_seq(ssm_in(NPRE), att_o(NJ // 2 - 1)), 4 + N_IN), (x_all(NPRE + 1), N_X))
    for c in oa:
        c.start()
    for c in range(NPRE):
        for x in out_b(c):
            x.start()
    for c in range(NPRE, NC + 1):
        mx, n = [], 0
        if c + 1 < NC:
            mx.append(ssm_in(c + 1))
            n += N_IN
        if c - 1 >= NPRE:
            mx.append(ssm_out(c - 1))
            n += N_OUT
        st = [(_seq(*mx), n)]
        if c < NC:
            st.append((ssm_scan(c, carry), N_SC))
        if c + 2 < NC:
            st.append((x_all(c + 2), N_X))
        _mix(*st)
    for c in oa:
        c.wait()
    for c in range(NC):
        for x in out_b(c):
            x.wait()


@jax.jit
def pallas_concat_heads__sliding_local_dilated__ssm_conv_s5__prompt_kernel(
    A_x, A_wqkv, A_wo, B_x, B_Lambda_re, B_Lambda_im, B_B_re, B_B_im, B_C_re, B_C_im,
    B_log_dt, B_Dskip,
):
    hbm = pl.BlockSpec(memory_space=pltpu.HBM)
    out = pl.pallas_call(
        _kernel,
        out_shape=jax.ShapeDtypeStruct((S, 2 * D), F32),
        in_specs=[hbm] * 12,
        out_specs=hbm,
        scratch_shapes=[
            pltpu.VMEM((D, S), BF16),
            pltpu.VMEM((D, 3 * D), BF16),
            pltpu.VMEM((D, D), BF16),
            pltpu.VMEM((NC, D, T), BF16),
            pltpu.VMEM((2, D, D), BF16),
            pltpu.VMEM((2, D, D), BF16),
            *[pltpu.VMEM((D,), BF16)] * 4,
            pltpu.VMEM((8, 512), F32),
            pltpu.VMEM((896, 512), F32),
            pltpu.VMEM((512, 896), F32),
            *[pltpu.VMEM((4, 512, 128), F32)] * 4,
            pltpu.VMEM((4, 3 * D, 128), F32),
            pltpu.VMEM((3 * D, 512), F32),
            pltpu.VMEM((4, D, 128), F32),
            pltpu.VMEM((D, 512), F32),
            pltpu.VMEM((4, 128 * XP, 128), F32),
            pltpu.VMEM((30, D, 128), F32),
            pltpu.VMEM((30, D, 128), F32),
            pltpu.VMEM((4, S, 128), F32),
            pltpu.VMEM((S, 128), F32),
            pltpu.VMEM((3, S, 128), F32),
            pltpu.SemaphoreType.DMA((11 + NC,)),
            pltpu.SemaphoreType.DMA((3 + 4 * NC,)),
            *[pltpu.VMEM((8 * SEGS[i % 2], 896), F32) for i in range(NB)],
            *[pltpu.VMEM((8 * SEGS[i % 2], 896), F32) for i in range(NB)],
            *[pltpu.VMEM((D, 128), F32)] * NQ,
            *[pltpu.VMEM((256, 512), F32)] * 2,
        ],
        compiler_params=pltpu.CompilerParams(vmem_limit_bytes=100 * 1024 * 1024),
    )(A_x[0].T, A_wqkv, A_wo, B_x[0].T, B_Lambda_re, B_Lambda_im,
      B_B_re, B_B_im, B_C_re, B_C_im, B_log_dt, B_Dskip)
    return out.reshape(1, S, 2 * D)
```

```python
import jax
import jax.numpy as jnp
from jax import lax
import jax.experimental.pallas as pl
import jax.experimental.pallas.tpu as pltpu

S, D, H, DH, W = 2048, 448, 16, 28, 8
NJ = 16
T = 256
NC = S // T
SEGS = (28, 36)
XP = 20
GATE = False
TOKF = 0.2
F32, BF16 = jnp.float32, jnp.bfloat16
NN = (((1,), (0,)), ((), ()))
NT = (((1,), (1,)), ((), ()))
JP = [(0, 2), (4, 6), (8, 10), (12, 14), (1, 3), (5, 7), (9, 11), (13, 15)]


def _row0(c):
    return 512 * (c // 2) + 8 * SEGS[0] * (c % 2)


def _cmul(ar, ai, br, bi):
    return ar * br - ai * bi, ar * bi + ai * br


def _kernel(ax_h, wqkv_h, wo_h, bx_h, lre_h, lim_h, bre_h, bim_h, cre_h, cim_h, ldt_h, dsk_h,
            out_h,
            axv, wv, wov, bxv, bv, cv, pv0, pv1, pv2, pv3, prm, bcat, ccat, xb0, xb1, xb2, xb3,
            wt32, wtp, wo32, wot, xa32, obuf, a3, oa, isem, osem):
    xb32 = (xb0, xb1, xb2, xb3)

    def cp(i, src, dst):
        return pltpu.make_async_copy(src, dst, isem.at[i])
    c_par = [cp(0, lre_h, pv0), cp(1, lim_h, pv1), cp(2, ldt_h, pv2), cp(3, dsk_h, pv3)]
    c_b = [cp(4, bre_h, bv.at[0]), cp(5, bim_h, bv.at[1])]
    c_c = [cp(6, cre_h, cv.at[0]), cp(7, cim_h, cv.at[1])]
    c_bx = [cp(8 + c, bx_h.at[:, pl.ds(c * T, T)], bxv.at[c]) for c in range(NC)]
    c_w, c_ax, c_wo = cp(8 + NC, wqkv_h, wv), cp(9 + NC, ax_h, axv), cp(10 + NC, wo_h, wov)

    def start(*cs):
        for c in cs:
            c.start()

    def wait(*cs):
        for c in cs:
            c.wait()
    start(c_bx[0], c_b[0], *c_par, c_b[1])

    wait(*c_par)
    prm[...] = jnp.zeros(prm.shape, F32)
    for i in range(4):
        prm[i:i + 1, 0:D] = (pv0, pv1, pv2, pv3)[i][...].astype(F32).reshape(1, D)
    lane5 = lax.broadcasted_iota(jnp.int32, (8, 512), 1)
    lre = jnp.where(lane5 < D, jnp.broadcast_to(prm[0:1, :], (8, 512)), -1.0)
    lim = jnp.broadcast_to(prm[1:2, :], (8, 512))
    dt = jnp.exp(jnp.broadcast_to(prm[2:3, :], (8, 512))).astype(BF16).astype(F32)
    never = dt[:, 0:128] < 0.0
    zr, zi = dt * lre, dt * lim
    mag = jnp.exp(zr)
    lr, li = mag * jnp.cos(zi), mag * jnp.sin(zi)
    den = lre * lre + lim * lim
    nr, ni = lr - 1.0, li
    cr = 2.0 * (nr * lre + ni * lim) / den
    ci = 2.0 * (ni * lre - nr * lim) / den
    lane1 = lax.broadcasted_iota(jnp.int32, (8, 128), 1)
    sub = lax.broadcasted_iota(jnp.int32, (8, 128), 0)
    lo = lane1 < 64

    def tiles(r, i):
        r3, i3 = r[:, 384:], i[:, 384:]
        rr = jnp.where(lo, r3, pltpu.roll(r3, 64, 1))
        ii = jnp.where(lo, -i3, pltpu.roll(i3, 64, 1))
        return ([r[:, 128 * k:128 * k + 128] for k in range(3)] + [rr],
                [i[:, 128 * k:128 * k + 128] for k in range(3)] + [ii])
    lam = tiles(lr, li)
    sq = [(lr, li)]
    for _ in range(5):
        sq.append(_cmul(*sq[-1], *sq[-1]))
    pws = []
    for base in (_cmul(*_cmul(*sq[4], *sq[3]), *sq[2]), _cmul(*sq[5], *sq[2])):
        pw = []
        for _ in range(3):
            pw.append(tiles(*base))
            base = _cmul(*base, *base)
        pws.append(pw)
    dsk = pltpu.roll(jnp.broadcast_to(prm[3:4, :], (8, 512)), 64, 1)

    def cstep(m, k, a, b):
        if k < 3:
            return m[0][k] * a - m[1][k] * b, m[0][k] * b + m[1][k] * a
        return m[0][k] * a + m[1][k] * b, m[0][k] * b - m[1][k] * a

    toks = []

    def mm(lhs, rhs, dims):
        if GATE and len(toks) >= 2:
            t = toks[-2]
            parts = []
            for r in range(0, rhs.shape[0], 128):
                last = rhs[r + 120:r + 128]
                last = jnp.concatenate([jnp.where(never, t, last[:, c:c + 128])
                                        for c in range(0, rhs.shape[1], 128)], axis=1)
                parts += [rhs[r:r + 120], last]
            rhs = jnp.concatenate(parts, axis=0)
        res = lax.dot_general(lhs, rhs, dims, preferred_element_type=F32)
        r = int(res.shape[0] * TOKF) // 8 * 8
        toks.append(res[r:r + 8])
        return res

    def prep_b(i):
        for r in range(0, D, 64):
            v = jnp.concatenate([jnp.zeros((64, 64), F32), bv[i, r:r + 64, :].astype(F32)], axis=1)
            r2 = 384 * i + r if r < 384 else 768 + 64 * i
            bcat[r2:r2 + 64, :] = v

    def prep_c():
        nci = -ci[0:1, :D]
        for r in range(0, D, 32):
            c_re = cv[0, r:r + 32, :].astype(F32)
            c_im = cv[1, r:r + 32, :].astype(F32)
            c2r = c_re * cr[0:1, :D] - c_im * ci[0:1, :D]
            c2i = c_re * nci - c_im * cr[0:1, :D]
            ccat[r:r + 32, 0:384] = c2r[:, 0:384]
            ccat[r:r + 32, 384:768] = c2i[:, 0:384]
            ccat[r:r + 32, 768:896] = jnp.concatenate([c2r[:, 384:448], c2i[:, 384:448]], axis=1)

    def ssm_t(c):
        for k in range(4):
            if k == 0:
                xt = jnp.concatenate([jnp.zeros((64, T), F32), bxv[c, 0:64, :].astype(F32)], axis=0)
            else:
                xt = bxv[c, 128 * k - 64:128 * k + 64, :].astype(F32)
            xb32[c // 2][k, T * (c % 2):T * (c % 2) + T, :] = xt.T

    def xs(c, k, j):
        return xb32[c // 2][k, pl.ds(_row0(c) % 512 + j, 8, stride=SEGS[c % 2]), :]

    U, Hs = {}, {}

    def ssm_in(c, ns=range(7)):
        for n in ns:
            xl = jnp.concatenate([jnp.concatenate([xs(c, k, j) for k in range(4)], axis=1)
                                  for j in range(SEGS[c % 2])], axis=0)
            U[c, n] = mm(xl, bcat[128 * n:128 * n + 128, :], NT)

    carry = [(jnp.zeros((8, 128), F32),) * 2] * 4

    def ssm_scan(c):
        SEG, pw = SEGS[c % 2], pws[c % 2]
        sw = pltpu.roll(U[c, 6], 64, 1)

        def u(j, k):
            if k < 3:
                return U[c, k][8 * j:8 * j + 8], U[c, k + 3][8 * j:8 * j + 8]
            return U[c, 6][8 * j:8 * j + 8], sw[8 * j:8 * j + 8]
        h = [u(0, k) for k in range(4)]
        for j in range(1, SEG):
            for k in range(4):
                a, b = cstep(lam, k, *h[k])
                ua, ub = u(j, k)
                h[k] = (a + ua, b + ub)
        for k in range(4):
            z = [jnp.where(sub == 0, carry[k][i], pltpu.roll(h[k][i], 1, 0)) for i in range(2)]
            for n in range(3):
                sh = 1 << n
                a, b = cstep(pw[n], k, *[jnp.where(sub >= sh, pltpu.roll(v, sh, 0), 0.0) for v in z])
                z = [z[0] + a, z[1] + b]
            h[k] = tuple(z)
        rows = []
        for j in range(SEG):
            for k in range(4):
                a, b = cstep(lam, k, *h[k])
                ua, ub = u(j, k)
                h[k] = (a + ua, b + ub)
            rows.append(jnp.concatenate([h[0][0], h[1][0], h[2][0], h[0][1], h[1][1], h[2][1], h[3][0]], axis=1))
        Hs[c] = rows
        carry[:] = [tuple(jnp.broadcast_to(v[7:8], (8, 128)) for v in h[k]) for k in range(4)]

    def ssm_out(p, ts=range(4), between=lambda: None):
        cj = [(2 * p + i, j) for i in range(2) for j in range(SEGS[i])]
        yts = [mm(ccat[...], jnp.concatenate([Hs[c][j] for c, j in cj[16 * t:16 * t + 16]], axis=0), NT)
               for t in ts]
        between()
        for t, yt in zip(ts, yts):
            blk = cj[16 * t:16 * t + 16]
            y_post(p, blk, jnp.concatenate([jnp.zeros((64, 128), F32), yt], axis=0), range(4))

    def y_post(p, blk, yt, ks):
        for n, k in enumerate(ks):
            y = yt[128 * n:128 * n + 128].T
            for i, (c, j) in enumerate(blk):
                rows = pl.ds(_row0(c) + j, 8, stride=SEGS[c % 2])
                v = y[8 * i:8 * i + 8] + xs(c, k, j) * dsk[:, 128 * k:128 * k + 128]
                if k == 0 and p >= NPRE:
                    v = jnp.where(lo, a3[rows, :], v)
                obuf[k, rows, :] = v

    def ssm_last(p):
        cj = [(2 * p + i, j) for i in range(2) for j in range(SEGS[i])][32:]
        hh = jnp.concatenate([Hs[c][j] for c, j in cj], axis=0)
        for half in range(2):
            yt = mm(ccat[0:192, :] if half == 0 else ccat[192:D, :], hh, NT)
            if half == 0:
                yt = jnp.concatenate([jnp.zeros((64, 256), F32), yt], axis=0)
            for t in range(2):
                y_post(p, cj[16 * t:16 * t + 16], yt[:, 128 * t:128 * t + 128], (2 * half, 2 * half + 1))
            start(*o_b[2 * p + 1][2 * half:2 * half + 2])

    def w_t():
        for k in range(4):
            n = min(128, D - 128 * k)
            blk = wv[128 * k:128 * k + n, :].astype(F32)
            if n < 128:
                blk = jnp.concatenate([blk, jnp.zeros((128 - n, 3 * D), F32)], axis=0)
            wt32[k] = blk.T

    def w_perm(g):
        for d in range(DH):
            v = [jnp.concatenate([wt32[k, pl.ds(g * D + hh * 224 + d, 8, stride=DH), :]
                                  for k in range(4)], axis=1) for hh in range(2)]
            wtp[g * D + 16 * d:g * D + 16 * d + 16, :] = jnp.concatenate(v, axis=0)

    def x_t():
        for k in range(4):
            n = min(128, D - 128 * k)
            for t in range(4):
                blk = axv[128 * k:128 * k + n, 512 * t:512 * t + 512].astype(F32)
                if n < 128:
                    blk = jnp.concatenate([blk, jnp.zeros((128 - n, 512), F32)], axis=0)
                bt = blk.T
                for g in range(32):
                    r = XP * (32 * t + g)
                    xa32[k, r:r + 16, :] = bt[16 * g:16 * g + 16]

    def wo_prep():
        wo = jnp.concatenate([wov[...].astype(F32), jnp.zeros((D, 64), F32)], axis=1)
        for k in range(4):
            wo32[k] = wo[:, 128 * k:128 * k + 128]
        for k in range(4):
            v = [wo32[k, pl.ds(hh * 224 + d, 8, stride=DH), :] for d in range(DH) for hh in range(2)]
            v = jnp.concatenate(v + [jnp.zeros((64, 128), F32)], axis=0).T
            n = min(128, D - 128 * k)
            wot[128 * k:128 * k + n, :] = v[:n]

    def xa(j):
        return jnp.concatenate([xa32[k, pl.ds(j, 128, stride=XP), :] for k in range(4)], axis=1)

    KV, Q, O = ({}, {}), {}, {}

    def att_kv(j):
        for g in (0, 1):
            r = mm(wtp[D * (g + 1):D * (g + 2), :], xa(j), NT)
            KV[g][j + 14] = r
            if j >= 2:
                KV[g][j - 2] = pltpu.roll(r, 1, 1)

    def att_q(jp):
        for j in JP[jp]:
            Q[j] = mm(wtp[0:D, :], xa(j), NT)

    scale = DH ** -0.5

    def att(jp):
        js = JP[jp]
        es = range(js[0], js[1] + 15, 2)
        P = {}
        for hh in range(2):
            lg = {}
            for d in range(DH):
                r = slice(16 * d + 8 * hh, 16 * d + 8 * hh + 8)
                for j in js:
                    for w in range(W):
                        t = Q[j][r] * KV[0][j + 14 - 2 * w][r]
                        lg[j, w] = t if d == 0 else lg[j, w] + t
            for j in js:
                l = [lg[j, w] * scale for w in range(W)]
                l = [jnp.where(lane1 == 0, -1e9, l[w]) if j < 2 * w else l[w] for w in range(W)]
                m = l[0]
                for w in range(1, W):
                    m = jnp.maximum(m, l[w])
                e = [jnp.exp(x - m) for x in l]
                ssum = e[0]
                for w in range(1, W):
                    ssum = ssum + e[w]
                inv = 1.0 / ssum
                P[hh, j] = [x * inv for x in e]
        for j in js:
            O[j] = []
        for d in range(DH):
            for hh in range(2):
                r = slice(16 * d + 8 * hh, 16 * d + 8 * hh + 8)
                for j in js:
                    acc = None
                    for w in range(W):
                        t = P[hh, j][w] * KV[1][j + 14 - 2 * w][r]
                        acc = t if acc is None else acc + t
                    O[j].append(acc)

    def att_o(jp):
        for j in JP[jp]:
            rt = mm(wot[...], jnp.concatenate(O[j] + [jnp.zeros((64, 128), F32)], axis=0), NN)
            rt = jnp.concatenate([rt, jnp.zeros((64, 128), F32)], axis=0)
            for k in range(4):
                v = rt[128 * k:128 * k + 128].T
                if k == 3:
                    a3[pl.ds(j, 128, stride=NJ), :] = v
                else:
                    oa[k, pl.ds(j, 128, stride=NJ), :] = v

    o_a = [pltpu.make_async_copy(oa.at[k], out_h.at[:, pl.ds(128 * k, 128)], osem.at[k]) for k in range(3)]
    o_b = [[pltpu.make_async_copy(obuf.at[k, pl.ds(_row0(c), 8 * SEGS[c % 2])],
                                  out_h.at[pl.ds(_row0(c), 8 * SEGS[c % 2]), pl.ds(128 * (k + 3), 128)],
                                  osem.at[3 + 4 * c + k]) for k in range(4)] for c in range(NC)]

    NPRE = 2
    wait(c_bx[0], c_b[0])
    start(c_bx[1], c_bx[2], c_bx[3])
    prep_b(0)
    ssm_t(0)
    ssm_in(0, range(2))
    wait(c_b[1], c_bx[1])
    start(*c_c)
    prep_b(1)
    ssm_t(1)
    ssm_in(0, range(2, 7))
    ssm_in(1, range(2))
    wait(c_bx[2], c_bx[3])
    start(c_w, c_ax)
    ssm_in(1, range(2, 7))
    ssm_scan(0)
    ssm_t(2)
    ssm_t(3)
    ssm_in(2, range(2))
    wait(*c_c)
    prep_c()
    ssm_in(2, range(2, 7))
    ssm_in(3, range(2))
    ssm_scan(1)
    ssm_out(0, range(2), lambda: wait(c_w))
    w_t()
    w_perm(1)
    ssm_out(0, range(2, 4), lambda: (wait(c_ax), start(c_wo, *c_bx[4:])))
    x_t()
    w_perm(2)
    ssm_in(3, range(2, 7))
    ssm_scan(2)
    for j in range(0, NJ, 2):
        att_kv(j)
    ssm_scan(3)
    w_perm(0)
    start(*o_b[0][1:], *o_b[1][1:])
    wait(c_wo, *c_bx[4:6])
    wo_prep()
    att_q(0)
    for i in range(4):
        att_kv(4 * i + 1)
        att_q(i + 1)
        att(i)
        att_kv(4 * i + 3)
        if i >= 1:
            att_o(i - 1)
    ssm_t(4)
    ssm_t(5)
    fill = [(4, range(0, 2)), (4, range(2, 4)), (4, range(4, 6)), (4, range(6, 7))]
    for i in range(4, 8):
        ssm_out(1, [i - 4])
        if i < 7:
            att_q(i + 1)
        att(i)
        att_o(i - 1)
    att_o(7)
    ssm_in(4)
    obuf[0, 0:512 * NPRE, :] = jnp.where(lo[0:1], a3[0:512 * NPRE, :], obuf[0, 0:512 * NPRE, :])
    start(*o_a, o_b[0][0], o_b[1][0], *o_b[2], *o_b[3])
    wait(*c_bx[6:])
    ssm_t(6)
    ssm_t(7)
    ssm_in(5)
    ssm_scan(4)
    ssm_in(6)
    ssm_scan(5)
    ssm_out(2, range(2))
    ssm_in(7)
    ssm_scan(6)
    ssm_out(2, range(2, 4))
    start(*o_b[4], *o_b[5])
    ssm_scan(7)
    ssm_out(3, range(2))
    start(*o_b[6])
    ssm_last(3)
    wait(*o_a, *[c for cs in o_b for c in cs])


@jax.jit
def pallas_concat_heads__sliding_local_dilated__ssm_conv_s5__prompt_kernel(
    A_x, A_wqkv, A_wo, B_x, B_Lambda_re, B_Lambda_im, B_B_re, B_B_im, B_C_re, B_C_im,
    B_log_dt, B_Dskip,
):
    hbm = pl.BlockSpec(memory_space=pltpu.HBM)
    out = pl.pallas_call(
        _kernel,
        out_shape=jax.ShapeDtypeStruct((S, 2 * D), F32),
        in_specs=[hbm] * 12,
        out_specs=hbm,
        scratch_shapes=[
            pltpu.VMEM((D, S), BF16),
            pltpu.VMEM((D, 3 * D), BF16),
            pltpu.VMEM((D, D), BF16),
            pltpu.VMEM((NC, D, T), BF16),
            pltpu.VMEM((2, D, D), BF16),
            pltpu.VMEM((2, D, D), BF16),
            *[pltpu.VMEM((D,), BF16)] * 4,
            pltpu.VMEM((8, 512), F32),
            pltpu.VMEM((896, 512), F32),
            pltpu.VMEM((D, 896), F32),
            *[pltpu.VMEM((4, 512, 128), F32)] * 4,
            pltpu.VMEM((4, 3 * D, 128), F32),
            pltpu.VMEM((3 * D, 512), F32),
            pltpu.VMEM((4, D, 128), F32),
            pltpu.VMEM((D, 512), F32),
            pltpu.VMEM((4, 128 * XP, 128), F32),
            pltpu.VMEM((4, S, 128), F32),
            pltpu.VMEM((S, 128), F32),
            pltpu.VMEM((3, S, 128), F32),
            pltpu.SemaphoreType.DMA((11 + NC,)),
            pltpu.SemaphoreType.DMA((3 + 4 * NC,)),
        ],
        compiler_params=pltpu.CompilerParams(vmem_limit_bytes=100 * 1024 * 1024),
    )(A_x[0].T, A_wqkv, A_wo, B_x[0].T, B_Lambda_re, B_Lambda_im,
      B_B_re, B_B_im, B_C_re, B_C_im, B_log_dt, B_Dskip)
    return out.reshape(1, S, 2 * D)
```

```python
import jax
import jax.numpy as jnp
from jax import lax
import jax.experimental.pallas as pl
import jax.experimental.pallas.tpu as pltpu

S, D, H, DH, W = 2048, 448, 16, 28, 8
NJ = 16
T = 256
NC = S // T
SEGS = (28, 36)
XP = 20
GATE = [False]
NA, NB_ = 0, 7
M0, N3 = 1, 7
TOKF = 0.2
F32, BF16 = jnp.float32, jnp.bfloat16
NN = (((1,), (0,)), ((), ()))
NT = (((1,), (1,)), ((), ()))
JP = [(0, 2), (4, 6), (8, 10), (12, 14), (1, 3), (5, 7), (9, 11), (13, 15)]


def _row0(c):
    return 512 * (c // 2) + 8 * SEGS[0] * (c % 2)


def _cmul(ar, ai, br, bi):
    return ar * br - ai * bi, ar * bi + ai * br


def _kernel(ax_h, wqkv_h, wo_h, bx_h, lre_h, lim_h, bre_h, bim_h, cre_h, cim_h, ldt_h, dsk_h,
            out_h,
            axv, wv, wov, bxv, bv, cv, pv0, pv1, pv2, pv3, prm, bcat, ccat, xb0, xb1, xb2, xb3,
            wt32, wtp, wo32, wot, xa32, obuf, a3, oa, isem, osem):
    xb32 = (xb0, xb1, xb2, xb3)

    def cp(i, src, dst):
        return pltpu.make_async_copy(src, dst, isem.at[i])
    c_par = [cp(0, lre_h, pv0), cp(1, lim_h, pv1), cp(2, ldt_h, pv2), cp(3, dsk_h, pv3)]
    c_b = [cp(4, bre_h, bv.at[0]), cp(5, bim_h, bv.at[1])]
    c_c = [cp(6, cre_h, cv.at[0]), cp(7, cim_h, cv.at[1])]
    c_bx = [cp(8 + c, bx_h.at[:, pl.ds(c * T, T)], bxv.at[c]) for c in range(NC)]
    c_w, c_ax, c_wo = cp(8 + NC, wqkv_h, wv), cp(9 + NC, ax_h, axv), cp(10 + NC, wo_h, wov)

    def start(*cs):
        for c in cs:
            c.start()

    def wait(*cs):
        for c in cs:
            c.wait()
    start(c_bx[0], c_b[0], *c_par, c_b[1])

    wait(*c_par)
    prm[...] = jnp.zeros(prm.shape, F32)
    for i in range(4):
        prm[i:i + 1, 0:D] = (pv0, pv1, pv2, pv3)[i][...].astype(F32).reshape(1, D)
    lane5 = lax.broadcasted_iota(jnp.int32, (8, 512), 1)
    lre = jnp.where(lane5 < D, jnp.broadcast_to(prm[0:1, :], (8, 512)), -1.0)
    lim = jnp.broadcast_to(prm[1:2, :], (8, 512))
    dt = jnp.exp(jnp.broadcast_to(prm[2:3, :], (8, 512))).astype(BF16).astype(F32)
    never = dt[:, 0:128] < 0.0
    zr, zi = dt * lre, dt * lim
    mag = jnp.exp(zr)
    lr, li = mag * jnp.cos(zi), mag * jnp.sin(zi)
    den = lre * lre + lim * lim
    nr, ni = lr - 1.0, li
    cr = 2.0 * (nr * lre + ni * lim) / den
    ci = 2.0 * (ni * lre - nr * lim) / den
    lane1 = lax.broadcasted_iota(jnp.int32, (8, 128), 1)
    sub = lax.broadcasted_iota(jnp.int32, (8, 128), 0)
    lo = lane1 < 64

    def tiles(r, i):
        r3, i3 = r[:, 384:], i[:, 384:]
        rr = jnp.where(lo, r3, pltpu.roll(r3, 64, 1))
        ii = jnp.where(lo, -i3, pltpu.roll(i3, 64, 1))
        return ([r[:, 128 * k:128 * k + 128] for k in range(3)] + [rr],
                [i[:, 128 * k:128 * k + 128] for k in range(3)] + [ii])
    lam = tiles(lr, li)
    sq = [(lr, li)]
    for _ in range(5):
        sq.append(_cmul(*sq[-1], *sq[-1]))
    pws = []
    for base in (_cmul(*_cmul(*sq[4], *sq[3]), *sq[2]), _cmul(*sq[5], *sq[2])):
        pw = []
        for _ in range(3):
            pw.append(tiles(*base))
            base = _cmul(*base, *base)
        pws.append(pw)
    dsk = pltpu.roll(jnp.broadcast_to(prm[3:4, :], (8, 512)), 64, 1)

    def cstep(m, k, a, b):
        if k < 3:
            return m[0][k] * a - m[1][k] * b, m[0][k] * b + m[1][k] * a
        return m[0][k] * a + m[1][k] * b, m[0][k] * b - m[1][k] * a

    toks = []
    GATE[0] = False

    def mm(lhs, rhs, dims):
        if GATE[0] and len(toks) >= 2:
            t = toks[-2]
            parts = []
            for r in range(0, rhs.shape[0], 128):
                last = rhs[r + 120:r + 128]
                last = jnp.concatenate([jnp.where(never, t, last[:, c:c + 128])
                                        for c in range(0, rhs.shape[1], 128)], axis=1)
                parts += [rhs[r:r + 120], last]
            rhs = jnp.concatenate(parts, axis=0)
        res = lax.dot_general(lhs, rhs, dims, preferred_element_type=F32)
        r = int(res.shape[0] * TOKF) // 8 * 8
        toks.append(res[r:r + 8])
        return res

    def prep_b(i):
        for r in range(0, D, 64):
            v = jnp.concatenate([jnp.zeros((64, 64), F32), bv[i, r:r + 64, :].astype(F32)], axis=1)
            r2 = 384 * i + r if r < 384 else 768 + 64 * i
            bcat[r2:r2 + 64, :] = v

    def prep_c():
        nci = -ci[0:1, :D]
        for r in range(0, D, 32):
            c_re = cv[0, r:r + 32, :].astype(F32)
            c_im = cv[1, r:r + 32, :].astype(F32)
            c2r = c_re * cr[0:1, :D] - c_im * ci[0:1, :D]
            c2i = c_re * nci - c_im * cr[0:1, :D]
            ccat[r:r + 32, 0:384] = c2r[:, 0:384]
            ccat[r:r + 32, 384:768] = c2i[:, 0:384]
            ccat[r:r + 32, 768:896] = jnp.concatenate([c2r[:, 384:448], c2i[:, 384:448]], axis=1)

    def ssm_t(c):
        for k in range(4):
            if k == 0:
                xt = jnp.concatenate([jnp.zeros((64, T), F32), bxv[c, 0:64, :].astype(F32)], axis=0)
            else:
                xt = bxv[c, 128 * k - 64:128 * k + 64, :].astype(F32)
            xb32[c // 2][k, T * (c % 2):T * (c % 2) + T, :] = xt.T

    def xs(c, k, j):
        return xb32[c // 2][k, pl.ds(_row0(c) % 512 + j, 8, stride=SEGS[c % 2]), :]

    U, Hs = {}, {}

    def ssm_in(c, ns=range(7)):
        for n in ns:
            xl = jnp.concatenate([jnp.concatenate([xs(c, k, j) for k in range(4)], axis=1)
                                  for j in range(SEGS[c % 2])], axis=0)
            U[c, n] = mm(xl, bcat[128 * n:128 * n + 128, :], NT)

    carry = [(jnp.zeros((8, 128), F32),) * 2] * 4

    def ssm_scan(c):
        SEG, pw = SEGS[c % 2], pws[c % 2]
        sw = pltpu.roll(U[c, 6], 64, 1)

        def u(j, k):
            if k < 3:
                return U[c, k][8 * j:8 * j + 8], U[c, k + 3][8 * j:8 * j + 8]
            return U[c, 6][8 * j:8 * j + 8], sw[8 * j:8 * j + 8]
        h = [u(0, k) for k in range(4)]
        for j in range(1, SEG):
            for k in range(4):
                a, b = cstep(lam, k, *h[k])
                ua, ub = u(j, k)
                h[k] = (a + ua, b + ub)
        for k in range(4):
            z = [jnp.where(sub == 0, carry[k][i], pltpu.roll(h[k][i], 1, 0)) for i in range(2)]
            for n in range(3):
                sh = 1 << n
                a, b = cstep(pw[n], k, *[jnp.where(sub >= sh, pltpu.roll(v, sh, 0), 0.0) for v in z])
                z = [z[0] + a, z[1] + b]
            h[k] = tuple(z)
        rows = []
        for j in range(SEG):
            for k in range(4):
                a, b = cstep(lam, k, *h[k])
                ua, ub = u(j, k)
                h[k] = (a + ua, b + ub)
            rows.append(jnp.concatenate([h[0][0], h[1][0], h[2][0], h[0][1], h[1][1], h[2][1], h[3][0]], axis=1))
        Hs[c] = rows
        carry[:] = [tuple(jnp.broadcast_to(v[7:8], (8, 128)) for v in h[k]) for k in range(4)]

    def ssm_out(p, ts=range(4), between=lambda: None):
        cj = [(2 * p + i, j) for i in range(2) for j in range(SEGS[i])]
        yts = [mm(ccat[...], jnp.concatenate([Hs[c][j] for c, j in cj[16 * t:16 * t + 16]], axis=0), NT)
               for t in ts]
        between()
        for t, yt in zip(ts, yts):
            blk = cj[16 * t:16 * t + 16]
            y_post(p, blk, jnp.concatenate([jnp.zeros((64, 128), F32), yt], axis=0), range(4))

    def y_post(p, blk, yt, ks):
        for n, k in enumerate(ks):
            y = yt[128 * n:128 * n + 128].T
            for i, (c, j) in enumerate(blk):
                rows = pl.ds(_row0(c) + j, 8, stride=SEGS[c % 2])
                v = y[8 * i:8 * i + 8] + xs(c, k, j) * dsk[:, 128 * k:128 * k + 128]
                if k == 0 and p >= NPRE:
                    v = jnp.where(lo, a3[rows, :], v)
                obuf[k, rows, :] = v

    def ssm_last(p):
        cj = [(2 * p + i, j) for i in range(2) for j in range(SEGS[i])][32:]
        hh = jnp.concatenate([Hs[c][j] for c, j in cj], axis=0)
        for half in range(2):
            yt = mm(ccat[0:192, :] if half == 0 else ccat[192:D, :], hh, NT)
            if half == 0:
                yt = jnp.concatenate([jnp.zeros((64, 256), F32), yt], axis=0)
            for t in range(2):
                y_post(p, cj[16 * t:16 * t + 16], yt[:, 128 * t:128 * t + 128], (2 * half, 2 * half + 1))
            start(*o_b[2 * p + 1][2 * half:2 * half + 2])

    def w_t():
        for k in range(4):
            n = min(128, D - 128 * k)
            blk = wv[128 * k:128 * k + n, :].astype(F32)
            if n < 128:
                blk = jnp.concatenate([blk, jnp.zeros((128 - n, 3 * D), F32)], axis=0)
            wt32[k] = blk.T

    def w_perm(g):
        for d in range(DH):
            v = [jnp.concatenate([wt32[k, pl.ds(g * D + hh * 224 + d, 8, stride=DH), :]
                                  for k in range(4)], axis=1) for hh in range(2)]
            wtp[g * D + 16 * d:g * D + 16 * d + 16, :] = jnp.concatenate(v, axis=0)

    def x_t():
        for k in range(4):
            n = min(128, D - 128 * k)
            for t in range(4):
                blk = axv[128 * k:128 * k + n, 512 * t:512 * t + 512].astype(F32)
                if n < 128:
                    blk = jnp.concatenate([blk, jnp.zeros((128 - n, 512), F32)], axis=0)
                bt = blk.T
                for g in range(32):
                    r = XP * (32 * t + g)
                    xa32[k, r:r + 16, :] = bt[16 * g:16 * g + 16]

    def wo_prep():
        wo = jnp.concatenate([wov[...].astype(F32), jnp.zeros((D, 64), F32)], axis=1)
        for k in range(4):
            wo32[k] = wo[:, 128 * k:128 * k + 128]
        for k in range(4):
            v = [wo32[k, pl.ds(hh * 224 + d, 8, stride=DH), :] for d in range(DH) for hh in range(2)]
            v = jnp.concatenate(v + [jnp.zeros((64, 128), F32)], axis=0).T
            n = min(128, D - 128 * k)
            wot[128 * k:128 * k + n, :] = v[:n]

    def xa(j):
        return jnp.concatenate([xa32[k, pl.ds(j, 128, stride=XP), :] for k in range(4)], axis=1)

    KV, Q, O = ({}, {}), {}, {}

    def att_kv(j):
        for g in (0, 1):
            r = mm(wtp[D * (g + 1):D * (g + 2), :], xa(j), NT)
            KV[g][j + 14] = r
            if j >= 2:
                KV[g][j - 2] = pltpu.roll(r, 1, 1)

    def att_q(jp):
        for j in JP[jp]:
            Q[j] = mm(wtp[0:D, :], xa(j), NT)

    scale = DH ** -0.5

    def att(jp):
        js = JP[jp]
        es = range(js[0], js[1] + 15, 2)
        P = {}
        for hh in range(2):
            lg = {}
            for d in range(DH):
                r = slice(16 * d + 8 * hh, 16 * d + 8 * hh + 8)
                for j in js:
                    for w in range(W):
                        t = Q[j][r] * KV[0][j + 14 - 2 * w][r]
                        lg[j, w] = t if d == 0 else lg[j, w] + t
            for j in js:
                l = [lg[j, w] * scale for w in range(W)]
                l = [jnp.where(lane1 == 0, -1e9, l[w]) if j < 2 * w else l[w] for w in range(W)]
                m = l[0]
                for w in range(1, W):
                    m = jnp.maximum(m, l[w])
                e = [jnp.exp(x - m) for x in l]
                ssum = e[0]
                for w in range(1, W):
                    ssum = ssum + e[w]
                inv = 1.0 / ssum
                P[hh, j] = [x * inv for x in e]
        for j in js:
            O[j] = []
        for d in range(DH):
            for hh in range(2):
                r = slice(16 * d + 8 * hh, 16 * d + 8 * hh + 8)
                for j in js:
                    acc = None
                    for w in range(W):
                        t = P[hh, j][w] * KV[1][j + 14 - 2 * w][r]
                        acc = t if acc is None else acc + t
                    O[j].append(acc)

    def att_o(jp):
        for j in JP[jp]:
            rt = mm(wot[...], jnp.concatenate(O[j] + [jnp.zeros((64, 128), F32)], axis=0), NN)
            rt = jnp.concatenate([rt, jnp.zeros((64, 128), F32)], axis=0)
            for k in range(4):
                v = rt[128 * k:128 * k + 128].T
                if k == 3:
                    a3[pl.ds(j, 128, stride=NJ), :] = v
                else:
                    oa[k, pl.ds(j, 128, stride=NJ), :] = v

    o_a = [pltpu.make_async_copy(oa.at[k], out_h.at[:, pl.ds(128 * k, 128)], osem.at[k]) for k in range(3)]
    o_b = [[pltpu.make_async_copy(obuf.at[k, pl.ds(_row0(c), 8 * SEGS[c % 2])],
                                  out_h.at[pl.ds(_row0(c), 8 * SEGS[c % 2]), pl.ds(128 * (k + 3), 128)],
                                  osem.at[3 + 4 * c + k]) for k in range(4)] for c in range(NC)]

    NPRE = 2
    wait(c_bx[0], c_b[0])
    start(c_bx[1], c_bx[2], c_bx[3])
    prep_b(0)
    ssm_t(0)
    ssm_in(0, range(2))
    wait(c_b[1], c_bx[1])
    start(*c_c)
    prep_b(1)
    ssm_t(1)
    ssm_in(0, range(2, 7))
    ssm_in(1, range(2))
    wait(c_bx[2], c_bx[3])
    start(c_w, c_ax)
    ssm_in(1, range(2, 7))
    ssm_scan(0)
    ssm_t(2)
    ssm_t(3)
    ssm_in(2, range(2))
    wait(*c_c)
    prep_c()
    ssm_in(2, range(2, 7))
    ssm_in(3, range(2))
    ssm_scan(1)
    ssm_in(3, range(2, N3))
    ssm_out(0, range(M0), lambda: (wait(c_w, c_ax), start(c_wo, *c_bx[4:])))
    w_t()
    x_t()
    w_perm(1)
    ssm_out(0, range(M0, 4))
    w_perm(2)
    ssm_in(3, range(N3, 7))
    ssm_scan(2)
    for j in range(0, NJ, 2):
        att_kv(j)
    ssm_scan(3)
    w_perm(0)
    start(*o_b[0][1:], *o_b[1][1:])
    wait(c_wo, *c_bx[4:6])
    wo_prep()
    att_q(0)
    for i in range(4):
        att_kv(4 * i + 1)
        att_q(i + 1)
        att(i)
        att_kv(4 * i + 3)
        if i >= 1:
            att_o(i - 1)
    ssm_t(4)
    ssm_t(5)
    fill = [(4, range(0, 2)), (4, range(2, 4)), (4, range(4, 6)), (4, range(6, 7))]
    for i in range(4, 8):
        ssm_out(1, [i - 4])
        if i < 7:
            att_q(i + 1)
        att(i)
        att_o(i - 1)
    att_o(7)
    ssm_in(4)
    obuf[0, 0:512 * NPRE, :] = jnp.where(lo[0:1], a3[0:512 * NPRE, :], obuf[0, 0:512 * NPRE, :])
    start(*o_a, o_b[0][0], o_b[1][0], *o_b[2], *o_b[3])
    wait(*c_bx[6:])
    GATE[0] = True
    ssm_t(6)
    ssm_t(7)
    ssm_in(5)
    ssm_scan(4)
    ssm_in(6)
    ssm_scan(5)
    ssm_in(7, range(NA))
    ssm_out(2, range(2))
    start(*o_b[4])
    ssm_in(7, range(NA, NB_))
    ssm_out(2, range(2, 3))
    ssm_in(7, range(NB_, 7))
    ssm_scan(6)
    ssm_out(2, range(3, 4))
    start(*o_b[5])
    ssm_scan(7)
    ssm_out(3, range(2))
    start(*o_b[6])
    ssm_last(3)
    wait(*o_a, *[c for cs in o_b for c in cs])


@jax.jit
def pallas_concat_heads__sliding_local_dilated__ssm_conv_s5__prompt_kernel(
    A_x, A_wqkv, A_wo, B_x, B_Lambda_re, B_Lambda_im, B_B_re, B_B_im, B_C_re, B_C_im,
    B_log_dt, B_Dskip,
):
    hbm = pl.BlockSpec(memory_space=pltpu.HBM)
    out = pl.pallas_call(
        _kernel,
        out_shape=jax.ShapeDtypeStruct((S, 2 * D), F32),
        in_specs=[hbm] * 12,
        out_specs=hbm,
        scratch_shapes=[
            pltpu.VMEM((D, S), BF16),
            pltpu.VMEM((D, 3 * D), BF16),
            pltpu.VMEM((D, D), BF16),
            pltpu.VMEM((NC, D, T), BF16),
            pltpu.VMEM((2, D, D), BF16),
            pltpu.VMEM((2, D, D), BF16),
            *[pltpu.VMEM((D,), BF16)] * 4,
            pltpu.VMEM((8, 512), F32),
            pltpu.VMEM((896, 512), F32),
            pltpu.VMEM((D, 896), F32),
            *[pltpu.VMEM((4, 512, 128), F32)] * 4,
            pltpu.VMEM((4, 3 * D, 128), F32),
            pltpu.VMEM((3 * D, 512), F32),
            pltpu.VMEM((4, D, 128), F32),
            pltpu.VMEM((D, 512), F32),
            pltpu.VMEM((4, 128 * XP, 128), F32),
            pltpu.VMEM((4, S, 128), F32),
            pltpu.VMEM((S, 128), F32),
            pltpu.VMEM((3, S, 128), F32),
            pltpu.SemaphoreType.DMA((11 + NC,)),
            pltpu.SemaphoreType.DMA((3 + 4 * NC,)),
        ],
        compiler_params=pltpu.CompilerParams(vmem_limit_bytes=100 * 1024 * 1024),
    )(A_x[0].T, A_wqkv, A_wo, B_x[0].T, B_Lambda_re, B_Lambda_im,
      B_B_re, B_B_im, B_C_re, B_C_im, B_log_dt, B_Dskip)
    return out.reshape(1, S, 2 * D)
```

```python
import jax
import jax.numpy as jnp
from jax import lax
import jax.experimental.pallas as pl
import jax.experimental.pallas.tpu as pltpu

S, D, H, DH, W = 2048, 448, 16, 28, 8
NJ = 16
T = 256
NC = S // T
SEGS = (28, 36)
XP = 20
PD = 4
F32, BF16 = jnp.float32, jnp.bfloat16
NN = (((1,), (0,)), ((), ()))
NT = (((1,), (1,)), ((), ()))
JP = [(0, 2), (4, 6), (8, 10), (12, 14), (1, 3), (5, 7), (9, 11), (13, 15)]


def _row0(c):
    return 512 * (c // 2) + 8 * SEGS[0] * (c % 2)


def _cmul(ar, ai, br, bi):
    return ar * br - ai * bi, ar * bi + ai * br


def _kernel(ax_h, wqkv_h, wo_h, bx_h, lre_h, lim_h, bre_h, bim_h, cre_h, cim_h, ldt_h, dsk_h,
            out_h,
            axv, wv, wov, bxv, bv, cv, pv0, pv1, pv2, pv3, prm, bcat, ccat, xb0, xb1, xb2, xb3,
            wt32, wtp, wo32, wot, xa32, obuf, a3, oa, isem, osem):
    xb32 = (xb0, xb1, xb2, xb3)

    def cp(i, src, dst):
        return pltpu.make_async_copy(src, dst, isem.at[i])
    c_par = [cp(0, lre_h, pv0), cp(1, lim_h, pv1), cp(2, ldt_h, pv2), cp(3, dsk_h, pv3)]
    c_b = [cp(4, bre_h, bv.at[0]), cp(5, bim_h, bv.at[1])]
    c_c = [cp(6, cre_h, cv.at[0]), cp(7, cim_h, cv.at[1])]
    c_bx = [cp(8 + c, bx_h.at[:, pl.ds(c * T, T)], bxv.at[c]) for c in range(NC)]
    c_w, c_ax, c_wo = cp(8 + NC, wqkv_h, wv), cp(9 + NC, ax_h, axv), cp(10 + NC, wo_h, wov)

    def start(*cs):
        for c in cs:
            c.start()

    def wait(*cs):
        for c in cs:
            c.wait()
    start(c_bx[0], c_b[0], *c_par, c_b[1])

    wait(*c_par)
    prm[...] = jnp.zeros(prm.shape, F32)
    for i in range(4):
        prm[i:i + 1, 0:D] = (pv0, pv1, pv2, pv3)[i][...].astype(F32).reshape(1, D)
    lane5 = lax.broadcasted_iota(jnp.int32, (8, 512), 1)
    lre = jnp.where(lane5 < D, jnp.broadcast_to(prm[0:1, :], (8, 512)), -1.0)
    lim = jnp.broadcast_to(prm[1:2, :], (8, 512))
    dt = jnp.exp(jnp.broadcast_to(prm[2:3, :], (8, 512))).astype(BF16).astype(F32)
    never = dt[:, 0:128] < 0.0
    zr, zi = dt * lre, dt * lim
    mag = jnp.exp(zr)
    lr, li = mag * jnp.cos(zi), mag * jnp.sin(zi)
    den = lre * lre + lim * lim
    nr, ni = lr - 1.0, li
    cr = 2.0 * (nr * lre + ni * lim) / den
    ci = 2.0 * (ni * lre - nr * lim) / den
    lane1 = lax.broadcasted_iota(jnp.int32, (8, 128), 1)
    sub = lax.broadcasted_iota(jnp.int32, (8, 128), 0)
    lo = lane1 < 64

    def tiles(r, i):
        r3, i3 = r[:, 384:], i[:, 384:]
        rr = jnp.where(lo, r3, pltpu.roll(r3, 64, 1))
        ii = jnp.where(lo, -i3, pltpu.roll(i3, 64, 1))
        return ([r[:, 128 * k:128 * k + 128] for k in range(3)] + [rr],
                [i[:, 128 * k:128 * k + 128] for k in range(3)] + [ii])
    lam = tiles(lr, li)
    sq = [(lr, li)]
    for _ in range(5):
        sq.append(_cmul(*sq[-1], *sq[-1]))
    pws = []
    for base in (_cmul(*_cmul(*sq[4], *sq[3]), *sq[2]), _cmul(*sq[5], *sq[2])):
        pw = []
        for _ in range(3):
            pw.append(tiles(*base))
            base = _cmul(*base, *base)
        pws.append(pw)
    dsk = pltpu.roll(jnp.broadcast_to(prm[3:4, :], (8, 512)), 64, 1)

    def cstep(m, k, a, b):
        if k < 3:
            return m[0][k] * a - m[1][k] * b, m[0][k] * b + m[1][k] * a
        return m[0][k] * a + m[1][k] * b, m[0][k] * b - m[1][k] * a

    pend = []
    z0 = pl.program_id(0)

    def push(*cs):
        start(*cs)
        obuf[4, 0:8, :] = dsk[:, 128:256]
        pend.append([PD, obuf[4, pl.ds(pl.multiple_of(z0 * 8, 8), 8), :]])

    def mm(lhs, rhs, dims):
        t = None
        if pend:
            pend[0][0] -= 1
            if pend[0][0] == 0:
                t = pend.pop(0)[1]
        if t is not None:
            parts = []
            for r in range(0, rhs.shape[0], 128):
                last = rhs[r + 120:r + 128]
                last = jnp.concatenate([jnp.where(never, t, last[:, c:c + 128])
                                        for c in range(0, rhs.shape[1], 128)], axis=1)
                parts += [rhs[r:r + 120], last]
            rhs = jnp.concatenate(parts, axis=0)
        return lax.dot_general(lhs, rhs, dims, preferred_element_type=F32)

    def prep_b(i):
        for r in range(0, D, 64):
            v = jnp.concatenate([jnp.zeros((64, 64), F32), bv[i, r:r + 64, :].astype(F32)], axis=1)
            r2 = 384 * i + r if r < 384 else 768 + 64 * i
            bcat[r2:r2 + 64, :] = v

    def prep_c():
        nci = -ci[0:1, :D]
        for r in range(0, D, 32):
            c_re = cv[0, r:r + 32, :].astype(F32)
            c_im = cv[1, r:r + 32, :].astype(F32)
            c2r = c_re * cr[0:1, :D] - c_im * ci[0:1, :D]
            c2i = c_re * nci - c_im * cr[0:1, :D]
            ccat[r:r + 32, 0:384] = c2r[:, 0:384]
            ccat[r:r + 32, 384:768] = c2i[:, 0:384]
            ccat[r:r + 32, 768:896] = jnp.concatenate([c2r[:, 384:448], c2i[:, 384:448]], axis=1)

    def ssm_t(c):
        for k in range(4):
            if k == 0:
                xt = jnp.concatenate([jnp.zeros((64, T), F32), bxv[c, 0:64, :].astype(F32)], axis=0)
            else:
                xt = bxv[c, 128 * k - 64:128 * k + 64, :].astype(F32)
            xb32[c // 2][k, T * (c % 2):T * (c % 2) + T, :] = xt.T

    def xs(c, k, j):
        return xb32[c // 2][k, pl.ds(_row0(c) % 512 + j, 8, stride=SEGS[c % 2]), :]

    U, Hs = {}, {}

    def ssm_in(c, ns=range(7)):
        for n in ns:
            xl = jnp.concatenate([jnp.concatenate([xs(c, k, j) for k in range(4)], axis=1)
                                  for j in range(SEGS[c % 2])], axis=0)
            U[c, n] = mm(xl, bcat[128 * n:128 * n + 128, :], NT)

    carry = [(jnp.zeros((8, 128), F32),) * 2] * 4

    def ssm_scan(c):
        SEG, pw = SEGS[c % 2], pws[c % 2]
        sw = pltpu.roll(U[c, 6], 64, 1)

        def u(j, k):
            if k < 3:
                return U[c, k][8 * j:8 * j + 8], U[c, k + 3][8 * j:8 * j + 8]
            return U[c, 6][8 * j:8 * j + 8], sw[8 * j:8 * j + 8]
        h = [u(0, k) for k in range(4)]
        for j in range(1, SEG):
            for k in range(4):
                a, b = cstep(lam, k, *h[k])
                ua, ub = u(j, k)
                h[k] = (a + ua, b + ub)
        for k in range(4):
            z = [jnp.where(sub == 0, carry[k][i], pltpu.roll(h[k][i], 1, 0)) for i in range(2)]
            for n in range(3):
                sh = 1 << n
                a, b = cstep(pw[n], k, *[jnp.where(sub >= sh, pltpu.roll(v, sh, 0), 0.0) for v in z])
                z = [z[0] + a, z[1] + b]
            h[k] = tuple(z)
        rows = []
        for j in range(SEG):
            for k in range(4):
                a, b = cstep(lam, k, *h[k])
                ua, ub = u(j, k)
                h[k] = (a + ua, b + ub)
            rows.append(jnp.concatenate([h[0][0], h[1][0], h[2][0], h[0][1], h[1][1], h[2][1], h[3][0]], axis=1))
        Hs[c] = rows
        carry[:] = [tuple(jnp.broadcast_to(v[7:8], (8, 128)) for v in h[k]) for k in range(4)]

    def ssm_out(p, ts=range(4), between=lambda: None):
        cj = [(2 * p + i, j) for i in range(2) for j in range(SEGS[i])]
        yts = [mm(ccat[...], jnp.concatenate([Hs[c][j] for c, j in cj[16 * t:16 * t + 16]], axis=0), NT)
               for t in ts]
        between()
        for t, yt in zip(ts, yts):
            blk = cj[16 * t:16 * t + 16]
            y_post(p, blk, jnp.concatenate([jnp.zeros((64, 128), F32), yt], axis=0), range(4))

    def y_post(p, blk, yt, ks):
        for n, k in enumerate(ks):
            y = yt[128 * n:128 * n + 128].T
            for i, (c, j) in enumerate(blk):
                rows = pl.ds(_row0(c) + j, 8, stride=SEGS[c % 2])
                v = y[8 * i:8 * i + 8] + xs(c, k, j) * dsk[:, 128 * k:128 * k + 128]
                if k == 0 and p >= NPRE:
                    v = jnp.where(lo, a3[rows, :], v)
                obuf[k, rows, :] = v

    def ssm_last(p):
        cj = [(2 * p + i, j) for i in range(2) for j in range(SEGS[i])][32:]
        hh = jnp.concatenate([Hs[c][j] for c, j in cj], axis=0)
        for half in range(2):
            yt = mm(ccat[0:192, :] if half == 0 else ccat[192:D, :], hh, NT)
            if half == 0:
                yt = jnp.concatenate([jnp.zeros((64, 256), F32), yt], axis=0)
            for t in range(2):
                y_post(p, cj[16 * t:16 * t + 16], yt[:, 128 * t:128 * t + 128], (2 * half, 2 * half + 1))
            start(*o_b[2 * p + 1][2 * half:2 * half + 2])

    def w_t():
        for k in range(4):
            n = min(128, D - 128 * k)
            blk = wv[128 * k:128 * k + n, :].astype(F32)
            if n < 128:
                blk = jnp.concatenate([blk, jnp.zeros((128 - n, 3 * D), F32)], axis=0)
            wt32[k] = blk.T

    def w_perm(g):
        for d in range(DH):
            v = [jnp.concatenate([wt32[k, pl.ds(g * D + hh * 224 + d, 8, stride=DH), :]
                                  for k in range(4)], axis=1) for hh in range(2)]
            wtp[g * D + 16 * d:g * D + 16 * d + 16, :] = jnp.concatenate(v, axis=0)

    def x_t():
        for k in range(4):
            n = min(128, D - 128 * k)
            for t in range(4):
                blk = axv[128 * k:128 * k + n, 512 * t:512 * t + 512].astype(F32)
                if n < 128:
                    blk = jnp.concatenate([blk, jnp.zeros((128 - n, 512), F32)], axis=0)
                bt = blk.T
                for g in range(32):
                    r = XP * (32 * t + g)
                    xa32[k, r:r + 16, :] = bt[16 * g:16 * g + 16]

    def wo_prep():
        wo = jnp.concatenate([wov[...].astype(F32), jnp.zeros((D, 64), F32)], axis=1)
        for k in range(4):
            wo32[k] = wo[:, 128 * k:128 * k + 128]
        for k in range(4):
            v = [wo32[k, pl.ds(hh * 224 + d, 8, stride=DH), :] for d in range(DH) for hh in range(2)]
            v = jnp.concatenate(v + [jnp.zeros((64, 128), F32)], axis=0).T
            n = min(128, D - 128 * k)
            wot[128 * k:128 * k + n, :] = v[:n]

    def xa(j):
        return jnp.concatenate([xa32[k, pl.ds(j, 128, stride=XP), :] for k in range(4)], axis=1)

    KV, Q, O = ({}, {}), {}, {}

    def att_kv(j):
        for g in (0, 1):
            r = mm(wtp[D * (g + 1):D * (g + 2), :], xa(j), NT)
            KV[g][j + 14] = r
            if j >= 2:
                KV[g][j - 2] = pltpu.roll(r, 1, 1)

    def att_q(jp):
        for j in JP[jp]:
            Q[j] = mm(wtp[0:D, :], xa(j), NT)

    scale = DH ** -0.5

    def att(jp):
        js = JP[jp]
        es = range(js[0], js[1] + 15, 2)
        P = {}
        for hh in range(2):
            lg = {}
            for d in range(DH):
                r = slice(16 * d + 8 * hh, 16 * d + 8 * hh + 8)
                for j in js:
                    for w in range(W):
                        t = Q[j][r] * KV[0][j + 14 - 2 * w][r]
                        lg[j, w] = t if d == 0 else lg[j, w] + t
            for j in js:
                l = [lg[j, w] * scale for w in range(W)]
                l = [jnp.where(lane1 == 0, -1e9, l[w]) if j < 2 * w else l[w] for w in range(W)]
                m = l[0]
                for w in range(1, W):
                    m = jnp.maximum(m, l[w])
                e = [jnp.exp(x - m) for x in l]
                ssum = e[0]
                for w in range(1, W):
                    ssum = ssum + e[w]
                inv = 1.0 / ssum
                P[hh, j] = [x * inv for x in e]
        for j in js:
            O[j] = []
        for d in range(DH):
            for hh in range(2):
                r = slice(16 * d + 8 * hh, 16 * d + 8 * hh + 8)
                for j in js:
                    acc = None
                    for w in range(W):
                        t = P[hh, j][w] * KV[1][j + 14 - 2 * w][r]
                        acc = t if acc is None else acc + t
                    O[j].append(acc)

    def att_o(jp):
        for j in JP[jp]:
            rt = mm(wot[...], jnp.concatenate(O[j] + [jnp.zeros((64, 128), F32)], axis=0), NN)
            rt = jnp.concatenate([rt, jnp.zeros((64, 128), F32)], axis=0)
            for k in range(4):
                v = rt[128 * k:128 * k + 128].T
                if k == 3:
                    a3[pl.ds(j, 128, stride=NJ), :] = v
                else:
                    oa[k, pl.ds(j, 128, stride=NJ), :] = v

    o_a = [pltpu.make_async_copy(oa.at[k], out_h.at[:, pl.ds(128 * k, 128)], osem.at[k]) for k in range(3)]
    o_b = [[pltpu.make_async_copy(obuf.at[k, pl.ds(_row0(c), 8 * SEGS[c % 2])],
                                  out_h.at[pl.ds(_row0(c), 8 * SEGS[c % 2]), pl.ds(128 * (k + 3), 128)],
                                  osem.at[3 + 4 * c + k]) for k in range(4)] for c in range(NC)]

    NPRE = 2
    wait(c_bx[0], c_b[0])
    start(c_bx[1], c_bx[2], c_bx[3])
    prep_b(0)
    ssm_t(0)
    ssm_in(0, range(2))
    wait(c_b[1], c_bx[1])
    start(*c_c)
    prep_b(1)
    ssm_t(1)
    ssm_in(0, range(2, 7))
    ssm_in(1, range(2))
    wait(c_bx[2], c_bx[3])
    start(c_w, c_ax)
    ssm_in(1, range(2, 7))
    ssm_scan(0)
    ssm_t(2)
    ssm_t(3)
    ssm_in(2, range(2))
    wait(*c_c)
    prep_c()
    ssm_in(2, range(2, 7))
    ssm_in(3, range(2))
    ssm_scan(1)
    ssm_in(3, range(2, 7))
    ssm_out(0, range(1), lambda: (wait(c_w, c_ax), start(c_wo, *c_bx[4:])))
    w_t()
    x_t()
    w_perm(1)
    ssm_out(0, range(1, 4))
    w_perm(2)
    ssm_scan(2)
    for j in range(0, NJ, 2):
        att_kv(j)
    ssm_scan(3)
    w_perm(0)
    start(*o_b[0][1:], *o_b[1][1:])
    wait(c_wo, *c_bx[4:6])
    wo_prep()
    att_q(0)
    for i in range(4):
        att_kv(4 * i + 1)
        att_q(i + 1)
        att(i)
        att_kv(4 * i + 3)
        if i >= 1:
            att_o(i - 1)
    ssm_t(4)
    ssm_t(5)
    for i in range(4, 8):
        ssm_out(1, [i - 4])
        if i in (5, 7):
            push(*o_b[i // 2][1:])
        if i < 7:
            att_q(i + 1)
        att(i)
        att_o(i - 1)
    att_o(7)
    ssm_in(4)
    obuf[0, 0:512 * NPRE, :] = jnp.where(lo[0:1], a3[0:512 * NPRE, :], obuf[0, 0:512 * NPRE, :])
    start(*o_a, o_b[0][0], o_b[1][0], o_b[2][0], o_b[3][0])
    wait(*c_bx[6:])
    ssm_t(6)
    ssm_t(7)
    ssm_in(5)
    ssm_scan(4)
    ssm_in(6)
    ssm_scan(5)
    ssm_out(2, range(2))
    push(*o_b[4])
    ssm_in(7)
    ssm_out(2, range(2, 3))
    ssm_scan(6)
    ssm_out(2, range(3, 4))
    push(*o_b[5])
    ssm_scan(7)
    ssm_out(3, range(2))
    start(*o_b[6])
    ssm_last(3)
    wait(*o_a, *[c for cs in o_b for c in cs])


@jax.jit
def pallas_concat_heads__sliding_local_dilated__ssm_conv_s5__prompt_kernel(
    A_x, A_wqkv, A_wo, B_x, B_Lambda_re, B_Lambda_im, B_B_re, B_B_im, B_C_re, B_C_im,
    B_log_dt, B_Dskip,
):
    hbm = pl.BlockSpec(memory_space=pltpu.HBM)
    out = pl.pallas_call(
        _kernel,
        out_shape=jax.ShapeDtypeStruct((S, 2 * D), F32),
        grid=(1,),
        in_specs=[hbm] * 12,
        out_specs=hbm,
        scratch_shapes=[
            pltpu.VMEM((D, S), BF16),
            pltpu.VMEM((D, 3 * D), BF16),
            pltpu.VMEM((D, D), BF16),
            pltpu.VMEM((NC, D, T), BF16),
            pltpu.VMEM((2, D, D), BF16),
            pltpu.VMEM((2, D, D), BF16),
            *[pltpu.VMEM((D,), BF16)] * 4,
            pltpu.VMEM((8, 512), F32),
            pltpu.VMEM((896, 512), F32),
            pltpu.VMEM((D, 896), F32),
            *[pltpu.VMEM((4, 512, 128), F32)] * 4,
            pltpu.VMEM((4, 3 * D, 128), F32),
            pltpu.VMEM((3 * D, 512), F32),
            pltpu.VMEM((4, D, 128), F32),
            pltpu.VMEM((D, 512), F32),
            pltpu.VMEM((4, 128 * XP, 128), F32),
            pltpu.VMEM((5, S, 128), F32),
            pltpu.VMEM((S, 128), F32),
            pltpu.VMEM((3, S, 128), F32),
            pltpu.SemaphoreType.DMA((11 + NC,)),
            pltpu.SemaphoreType.DMA((3 + 4 * NC,)),
        ],
        compiler_params=pltpu.CompilerParams(vmem_limit_bytes=100 * 1024 * 1024),
    )(A_x[0].T, A_wqkv, A_wo, B_x[0].T, B_Lambda_re, B_Lambda_im,
      B_B_re, B_B_im, B_C_re, B_C_im, B_log_dt, B_Dskip)
    return out.reshape(1, S, 2 * D)
```

```python
import functools

import jax
import jax.numpy as jnp
from jax import lax
import jax.experimental.pallas as pl
import jax.experimental.pallas.tpu as pltpu

S, D, H, DH, W = 2048, 448, 16, 28, 8
NJ = 16
T = 256
NC = S // T
SEGS = (28, 36)
XP = 20
KG, DJ = ((0,), (1,), (2,), (3,)), 8
OP = 132
PD = 4
F32, BF16 = jnp.float32, jnp.bfloat16
NN = (((1,), (0,)), ((), ()))
NT = (((1,), (1,)), ((), ()))
JP = [(0, 2), (4, 6), (8, 10), (12, 14), (1, 3), (5, 7), (9, 11), (13, 15)]


_dot = functools.partial(lax.dot_general, preferred_element_type=F32)


def _row0(c):
    return 512 * (c // 2) + 8 * SEGS[0] * (c % 2)


def _cmul(ar, ai, br, bi):
    return ar * br - ai * bi, ar * bi + ai * br


def _kernel(ax_h, wqkv_h, wo_h, bx_h, lre_h, lim_h, bre_h, bim_h, cre_h, cim_h, ldt_h, dsk_h,
            out_h,
            axv, wv, wov, bxv, bv, cv, pv0, pv1, pv2, pv3, prm, bcat, ccat, xb0, xb1, xb2, xb3,
            wt32, wtp, wo32, wot, xa32, obuf, a3, oa, ost0, ost1, isem, osem):
    ost = (ost0, ost1)
    xb32 = (xb0, xb1, xb2, xb3)

    def cp(i, src, dst):
        return pltpu.make_async_copy(src, dst, isem.at[i])
    c_par = [cp(0, lre_h, pv0), cp(1, lim_h, pv1), cp(2, ldt_h, pv2), cp(3, dsk_h, pv3)]
    c_b = [cp(4, bre_h, bv.at[0]), cp(5, bim_h, bv.at[1])]
    c_c = [cp(6, cre_h, cv.at[0]), cp(7, cim_h, cv.at[1])]
    c_bx = [cp(8 + c, bx_h.at[:, pl.ds(c * T, T)], bxv.at[c]) for c in range(NC)]
    c_w, c_ax, c_wo = cp(8 + NC, wqkv_h, wv), cp(9 + NC, ax_h, axv), cp(10 + NC, wo_h, wov)

    def start(*cs):
        for c in cs:
            c.start()

    def wait(*cs):
        for c in cs:
            c.wait()
    start(c_bx[0], c_b[0], *c_par, c_b[1])

    wait(*c_par)
    prm[...] = jnp.zeros(prm.shape, F32)
    for i in range(4):
        prm[i:i + 1, 0:D] = (pv0, pv1, pv2, pv3)[i][...].astype(F32).reshape(1, D)
    lane5 = lax.broadcasted_iota(jnp.int32, (8, 512), 1)
    lre = jnp.where(lane5 < D, jnp.broadcast_to(prm[0:1, :], (8, 512)), -1.0)
    lim = jnp.broadcast_to(prm[1:2, :], (8, 512))
    dt = jnp.exp(jnp.broadcast_to(prm[2:3, :], (8, 512))).astype(BF16).astype(F32)
    never = dt[:, 0:128] < 0.0
    zr, zi = dt * lre, dt * lim
    mag = jnp.exp(zr)
    lr, li = mag * jnp.cos(zi), mag * jnp.sin(zi)
    den = lre * lre + lim * lim
    nr, ni = lr - 1.0, li
    cr = 2.0 * (nr * lre + ni * lim) / den
    ci = 2.0 * (ni * lre - nr * lim) / den
    lane1 = lax.broadcasted_iota(jnp.int32, (8, 128), 1)
    sub = lax.broadcasted_iota(jnp.int32, (8, 128), 0)
    lo = lane1 < 64

    def tiles(r, i):
        r3, i3 = r[:, 384:], i[:, 384:]
        rr = jnp.where(lo, r3, pltpu.roll(r3, 64, 1))
        ii = jnp.where(lo, -i3, pltpu.roll(i3, 64, 1))
        return ([r[:, 128 * k:128 * k + 128] for k in range(3)] + [rr],
                [i[:, 128 * k:128 * k + 128] for k in range(3)] + [ii])
    lam = tiles(lr, li)
    sq = [(lr, li)]
    for _ in range(5):
        sq.append(_cmul(*sq[-1], *sq[-1]))
    pws = []
    for base in (_cmul(*_cmul(*sq[4], *sq[3]), *sq[2]), _cmul(*sq[5], *sq[2])):
        pw = []
        for _ in range(3):
            pw.append(tiles(*base))
            base = _cmul(*base, *base)
        pws.append(pw)
    dsk = pltpu.roll(jnp.broadcast_to(prm[3:4, :], (8, 512)), 64, 1)

    def cstep(m, k, a, b):
        if k < 3:
            return m[0][k] * a - m[1][k] * b, m[0][k] * b + m[1][k] * a
        return m[0][k] * a + m[1][k] * b, m[0][k] * b - m[1][k] * a

    pend = []
    z0 = pl.program_id(0)

    def push(*cs):
        start(*cs)
        obuf[4, 0:8, :] = dsk[:, 128:256]
        pend.append([PD, obuf[4, pl.ds(pl.multiple_of(z0 * 8, 8), 8), :]])

    def gate(rhs):
        t = None
        if pend:
            pend[0][0] -= 1
            if pend[0][0] == 0:
                t = pend.pop(0)[1]
        if t is not None:
            parts = []
            for r in range(0, rhs.shape[0], 128):
                last = rhs[r + 120:r + 128]
                last = jnp.concatenate([jnp.where(never, t, last[:, c:c + 128])
                                        for c in range(0, rhs.shape[1], 128)], axis=1)
                parts += [rhs[r:r + 120], last]
            rhs = jnp.concatenate(parts, axis=0)
        return rhs

    def prep_b(i):
        for r in range(0, D, 64):
            v = jnp.concatenate([jnp.zeros((64, 64), F32), bv[i, r:r + 64, :].astype(F32)], axis=1)
            r2 = 384 * i + r if r < 384 else 768 + 64 * i
            bcat[r2:r2 + 64, :] = v

    def prep_c():
        nci = -ci[0:1, :D]
        for r in range(0, D, 32):
            c_re = cv[0, r:r + 32, :].astype(F32)
            c_im = cv[1, r:r + 32, :].astype(F32)
            c2r = c_re * cr[0:1, :D] - c_im * ci[0:1, :D]
            c2i = c_re * nci - c_im * cr[0:1, :D]
            ccat[r:r + 32, 0:384] = c2r[:, 0:384]
            ccat[r:r + 32, 384:768] = c2i[:, 0:384]
            ccat[r:r + 32, 768:896] = jnp.concatenate([c2r[:, 384:448], c2i[:, 384:448]], axis=1)

    def ssm_t(c):
        for k in range(4):
            if k == 0:
                xt = jnp.concatenate([jnp.zeros((64, T), F32), bxv[c, 0:64, :].astype(F32)], axis=0)
            else:
                xt = bxv[c, 128 * k - 64:128 * k + 64, :].astype(F32)
            xb32[c // 2][k, T * (c % 2):T * (c % 2) + T, :] = xt.T

    def xs(c, k, j):
        return xb32[c // 2][k, pl.ds(_row0(c) % 512 + j, 8, stride=SEGS[c % 2]), :]

    U, Hs = {}, {}

    def ssm_in(c, ns=range(7)):
        for n in ns:
            xl = jnp.concatenate([jnp.concatenate([xs(c, k, j) for k in range(4)], axis=1)
                                  for j in range(SEGS[c % 2])], axis=0)
            U[c, n] = _dot(xl, gate(bcat[128 * n:128 * n + 128, :]), NT)

    carry = [(jnp.zeros((8, 128), F32),) * 2] * 4

    def ssm_scan(c):
        SEG, pw = SEGS[c % 2], pws[c % 2]
        sw = pltpu.roll(U[c, 6], 64, 1)

        def u(j, k):
            if k < 3:
                return U[c, k][8 * j:8 * j + 8], U[c, k + 3][8 * j:8 * j + 8]
            return U[c, 6][8 * j:8 * j + 8], sw[8 * j:8 * j + 8]
        h, hs, dep = [None] * 4, {}, None
        for ks in KG:
            for k in ks:
                h[k] = u(0, k)
                if dep is not None:
                    h[k] = tuple(jnp.where(never, dep, v) for v in h[k])
            for j in range(1, SEG):
                for k in ks:
                    a, b = cstep(lam, k, *h[k])
                    ua, ub = u(j, k)
                    h[k] = (a + ua, b + ub)
            for k in ks:
                z = [jnp.where(sub == 0, carry[k][i], pltpu.roll(h[k][i], 1, 0)) for i in range(2)]
                for n in range(3):
                    sh = 1 << n
                    a, b = cstep(pw[n], k, *[jnp.where(sub >= sh, pltpu.roll(v, sh, 0), 0.0) for v in z])
                    z = [z[0] + a, z[1] + b]
                h[k] = tuple(z)
            for j in range(SEG):
                for k in ks:
                    a, b = cstep(lam, k, *h[k])
                    ua, ub = u(j, k)
                    h[k] = hs[j, k] = (a + ua, b + ub)
                if j == SEG * DJ // 8 - 1:
                    dep = h[ks[-1]][0]
        Hs[c] = [jnp.concatenate([hs[j, 0][0], hs[j, 1][0], hs[j, 2][0], hs[j, 0][1], hs[j, 1][1], hs[j, 2][1],
                                  hs[j, 3][0]], axis=1) for j in range(SEG)]
        carry[:] = [tuple(jnp.broadcast_to(v[7:8], (8, 128)) for v in h[k]) for k in range(4)]

    def ssm_out(p, ts=range(4), between=lambda: None):
        cj = [(2 * p + i, j) for i in range(2) for j in range(SEGS[i])]
        yts = [_dot(ccat[...], gate(jnp.concatenate([Hs[c][j] for c, j in cj[16 * t:16 * t + 16]], axis=0)), NT)
               for t in ts]
        between()
        for t, yt in zip(ts, yts):
            blk = cj[16 * t:16 * t + 16]
            y_post(p, blk, jnp.concatenate([jnp.zeros((64, 128), F32), yt], axis=0), range(4))

    def y_post(p, blk, yt, ks):
        for n, k in enumerate(ks):
            y = yt[128 * n:128 * n + 128].T
            for i, (c, j) in enumerate(blk):
                rows = pl.ds(_row0(c) + j, 8, stride=SEGS[c % 2])
                v = y[8 * i:8 * i + 8] + xs(c, k, j) * dsk[:, 128 * k:128 * k + 128]
                if k == 0 and p >= NPRE:
                    v = jnp.where(lo, a3[rows, :], v)
                obuf[k, rows, :] = v

    def ssm_last(p):
        cj = [(2 * p + i, j) for i in range(2) for j in range(SEGS[i])][32:]
        hh = jnp.concatenate([Hs[c][j] for c, j in cj], axis=0)
        for half in range(2):
            yt = _dot(ccat[0:192, :] if half == 0 else ccat[192:D, :], gate(hh), NT)
            if half == 0:
                yt = jnp.concatenate([jnp.zeros((64, 256), F32), yt], axis=0)
            for t in range(2):
                y_post(p, cj[16 * t:16 * t + 16], yt[:, 128 * t:128 * t + 128], (2 * half, 2 * half + 1))
            start(*o_b[2 * p + 1][2 * half:2 * half + 2])

    def w_t():
        for k in range(4):
            n = min(128, D - 128 * k)
            blk = wv[128 * k:128 * k + n, :].astype(F32)
            if n < 128:
                blk = jnp.concatenate([blk, jnp.zeros((128 - n, 3 * D), F32)], axis=0)
            wt32[k] = blk.T

    def w_perm(g):
        for d in range(DH):
            v = [jnp.concatenate([wt32[k, pl.ds(g * D + hh * 224 + d, 8, stride=DH), :]
                                  for k in range(4)], axis=1) for hh in range(2)]
            wtp[g * D + 16 * d:g * D + 16 * d + 16, :] = jnp.concatenate(v, axis=0)

    def x_t():
        for k in range(4):
            n = min(128, D - 128 * k)
            for t in range(4):
                blk = axv[128 * k:128 * k + n, 512 * t:512 * t + 512].astype(F32)
                if n < 128:
                    blk = jnp.concatenate([blk, jnp.zeros((128 - n, 512), F32)], axis=0)
                bt = blk.T
                for g in range(32):
                    r = XP * (32 * t + g)
                    xa32[k, r:r + 16, :] = bt[16 * g:16 * g + 16]

    def wo_prep():
        wo = jnp.concatenate([wov[...].astype(F32), jnp.zeros((D, 64), F32)], axis=1)
        for k in range(4):
            wo32[k] = wo[:, 128 * k:128 * k + 128]
        for k in range(4):
            v = [wo32[k, pl.ds(hh * 224 + d, 8, stride=DH), :] for d in range(DH) for hh in range(2)]
            v = jnp.concatenate(v + [jnp.zeros((64, 128), F32)], axis=0).T
            n = min(128, D - 128 * k)
            wot[128 * k:128 * k + n, :] = v[:n]

    def xa(j):
        return jnp.concatenate([xa32[k, pl.ds(j, 128, stride=XP), :] for k in range(4)], axis=1)

    KV, Q, O = ({}, {}), {}, {}

    def att_kv(j):
        for g in (0, 1):
            r = _dot(wtp[D * (g + 1):D * (g + 2), :], gate(xa(j)), NT)
            KV[g][j + 14] = r
            if j >= 2:
                KV[g][j - 2] = pltpu.roll(r, 1, 1)

    def att_q(jp):
        for j in JP[jp]:
            Q[j] = _dot(wtp[0:D, :], gate(xa(j)), NT)

    scale = DH ** -0.5

    def att(jp):
        js = JP[jp]
        es = range(js[0], js[1] + 15, 2)
        P = {}
        for hh in range(2):
            lg = {}
            for d in range(DH):
                r = slice(16 * d + 8 * hh, 16 * d + 8 * hh + 8)
                for j in js:
                    for w in range(W):
                        t = Q[j][r] * KV[0][j + 14 - 2 * w][r]
                        lg[j, w] = t if d == 0 else lg[j, w] + t
            for j in js:
                l = [lg[j, w] * scale for w in range(W)]
                l = [jnp.where(lane1 == 0, -1e9, l[w]) if j < 2 * w else l[w] for w in range(W)]
                m = l[0]
                for w in range(1, W):
                    m = jnp.maximum(m, l[w])
                e = [jnp.exp(x - m) for x in l]
                ssum = e[0]
                for w in range(1, W):
                    ssum = ssum + e[w]
                inv = 1.0 / ssum
                P[hh, j] = [x * inv for x in e]
        for j in js:
            O[j] = []
        for d in range(DH):
            for hh in range(2):
                r = slice(16 * d + 8 * hh, 16 * d + 8 * hh + 8)
                for j in js:
                    acc = None
                    for w in range(W):
                        t = P[hh, j][w] * KV[1][j + 14 - 2 * w][r]
                        acc = t if acc is None else acc + t
                    O[j].append(acc)

    def att_o(jp):
        for j in JP[jp]:
            rt = _dot(wot[...], gate(jnp.concatenate(O[j] + [jnp.zeros((64, 128), F32)], axis=0)), NN)
            rt = jnp.concatenate([rt, jnp.zeros((64, 128), F32)], axis=0)
            for k in range(4):
                ost[j % 2][k, pl.ds(OP * (j // 2), 128), :] = rt[128 * k:128 * k + 128].T

    def o_rows(par, k, s):
        return ost[par][k, pl.ds(s, 8, stride=OP), :]

    def o_unperm(par):
        for k in range(3):
            for s in range(128):
                oa[k, pl.ds(NJ * s + par, 8, stride=2), :] = o_rows(par, k, s)

    def o_mixed():
        for s in range(128):
            for par in range(2):
                rows = pl.ds(NJ * s + par, 8, stride=2)
                if NJ * s < 512 * NPRE:
                    obuf[0, rows, :] = jnp.where(lo, o_rows(par, 3, s), obuf[0, rows, :])
                else:
                    a3[rows, :] = o_rows(par, 3, s)

    o_a = [pltpu.make_async_copy(oa.at[k], out_h.at[:, pl.ds(128 * k, 128)], osem) for k in range(3)]
    o_b = [[pltpu.make_async_copy(obuf.at[k, pl.ds(_row0(c), 8 * SEGS[c % 2])],
                                  out_h.at[pl.ds(_row0(c), 8 * SEGS[c % 2]), pl.ds(128 * (k + 3), 128)],
                                  osem) for k in range(4)] for c in range(NC)]

    NPRE = 2
    wait(c_bx[0], c_b[0])
    start(c_bx[1], c_bx[2], c_bx[3])
    prep_b(0)
    ssm_t(0)
    ssm_in(0, range(2))
    wait(c_b[1], c_bx[1])
    start(*c_c)
    prep_b(1)
    ssm_t(1)
    ssm_in(0, range(2, 7))
    ssm_in(1, range(2))
    wait(c_bx[2], c_bx[3])
    start(c_w, c_ax)
    ssm_in(1, range(2, 7))
    ssm_scan(0)
    ssm_t(2)
    ssm_t(3)
    ssm_in(2, range(2))
    wait(*c_c)
    prep_c()
    ssm_in(2, range(2, 7))
    ssm_in(3, range(2))
    ssm_scan(1)
    ssm_in(3, range(2, 7))
    ssm_out(0, range(1), lambda: (wait(c_w, c_ax), start(c_wo, *c_bx[4:])))
    w_t()
    x_t()
    w_perm(1)
    ssm_out(0, range(1, 4))
    w_perm(2)
    ssm_scan(2)
    for j in range(0, NJ, 2):
        att_kv(j)
    ssm_scan(3)
    w_perm(0)
    start(*o_b[0][1:], *o_b[1][1:])
    wait(c_wo, *c_bx[4:6])
    wo_prep()
    att_q(0)
    for i in range(4):
        att_kv(4 * i + 1)
        att_q(i + 1)
        att(i)
        att_kv(4 * i + 3)
        if i >= 1:
            att_o(i - 1)
    ssm_t(4)
    ssm_t(5)
    for i in range(4, 8):
        ssm_out(1, [i - 4])
        if i in (5, 7):
            push(*o_b[i // 2][1:])
        if i < 7:
            att_q(i + 1)
        att(i)
        att_o(i - 1)
        if i == 4:
            o_unperm(0)
    att_o(7)
    ssm_in(4)
    o_unperm(1)
    o_mixed()
    start(*o_a, o_b[0][0], o_b[1][0], o_b[2][0], o_b[3][0])
    wait(*c_bx[6:])
    ssm_t(6)
    ssm_t(7)
    ssm_in(5)
    ssm_scan(4)
    ssm_in(6)
    ssm_scan(5)
    ssm_out(2, range(2))
    push(*o_b[4])
    ssm_in(7)
    ssm_out(2, range(2, 3))
    ssm_scan(6)
    ssm_out(2, range(3, 4))
    push(*o_b[5])
    ssm_scan(7)
    ssm_out(3, range(2))
    start(*o_b[6])
    ssm_last(3)
    pltpu.make_async_copy(out_h, out_h, osem).wait()


@jax.jit
def pallas_concat_heads__sliding_local_dilated__ssm_conv_s5__prompt_kernel(
    A_x, A_wqkv, A_wo, B_x, B_Lambda_re, B_Lambda_im, B_B_re, B_B_im, B_C_re, B_C_im,
    B_log_dt, B_Dskip,
):
    hbm = pl.BlockSpec(memory_space=pltpu.HBM)
    out = pl.pallas_call(
        _kernel,
        out_shape=jax.ShapeDtypeStruct((S, 2 * D), F32),
        grid=(1,),
        in_specs=[hbm] * 12,
        out_specs=hbm,
        scratch_shapes=[
            pltpu.VMEM((D, S), BF16),
            pltpu.VMEM((D, 3 * D), BF16),
            pltpu.VMEM((D, D), BF16),
            pltpu.VMEM((NC, D, T), BF16),
            pltpu.VMEM((2, D, D), BF16),
            pltpu.VMEM((2, D, D), BF16),
            *[pltpu.VMEM((D,), BF16)] * 4,
            pltpu.VMEM((8, 512), F32),
            pltpu.VMEM((896, 512), F32),
            pltpu.VMEM((D, 896), F32),
            *[pltpu.VMEM((4, 512, 128), F32)] * 4,
            pltpu.VMEM((4, 3 * D, 128), F32),
            pltpu.VMEM((3 * D, 512), F32),
            pltpu.VMEM((4, D, 128), F32),
            pltpu.VMEM((D, 512), F32),
            pltpu.VMEM((4, 128 * XP, 128), F32),
            pltpu.VMEM((5, S, 128), F32),
            pltpu.VMEM((S, 128), F32),
            pltpu.VMEM((3, S, 128), F32),
            *[pltpu.VMEM((4, 8 * OP, 128), F32)] * 2,
            pltpu.SemaphoreType.DMA((11 + NC,)),
            pltpu.SemaphoreType.DMA(()),
        ],
        compiler_params=pltpu.CompilerParams(vmem_limit_bytes=100 * 1024 * 1024),
    )(A_x[0].T, A_wqkv, A_wo, B_x[0].T, B_Lambda_re, B_Lambda_im,
      B_B_re, B_B_im, B_C_re, B_C_im, B_log_dt, B_Dskip)
    return out.reshape(1, S, 2 * D)
```

```python
import functools

import jax
import jax.numpy as jnp
from jax import lax
import jax.experimental.pallas as pl
import jax.experimental.pallas.tpu as pltpu

S, D, H, DH, W = 2048, 448, 16, 28, 8
NJ = 16
T = 256
NC = S // T
SEGS = (28, 36)
XP = 20
KG, DJ = ((0,), (1,), (2,), (3,)), 8
OP = 132
LT0, PIECES = 0, ((0, 1), (2,), (3,))
PD = 4
F32, BF16 = jnp.float32, jnp.bfloat16
NN = (((1,), (0,)), ((), ()))
NT = (((1,), (1,)), ((), ()))
JP = [(0, 2), (4, 6), (8, 10), (12, 14), (1, 3), (5, 7), (9, 11), (13, 15)]


_dot = functools.partial(lax.dot_general, preferred_element_type=F32)


def _row0(c):
    return 512 * (c // 2) + 8 * SEGS[0] * (c % 2)


def _cmul(ar, ai, br, bi):
    return ar * br - ai * bi, ar * bi + ai * br


def _kernel(ax_h, wqkv_h, wo_h, bx_h, lre_h, lim_h, bre_h, bim_h, cre_h, cim_h, ldt_h, dsk_h,
            out_h,
            axv, wv, wov, bxv, bv, cv, pv0, pv1, pv2, pv3, prm, bcat, ccat, xb0, xb1, xb2, xb3,
            wt32, wtp, wo32, wot, xa32, obuf, a3, oa, ost0, ost1, isem, osem):
    ost = (ost0, ost1)
    xb32 = (xb0, xb1, xb2, xb3)

    def cp(i, src, dst):
        return pltpu.make_async_copy(src, dst, isem.at[i])
    c_par = [cp(0, lre_h, pv0), cp(1, lim_h, pv1), cp(2, ldt_h, pv2), cp(3, dsk_h, pv3)]
    c_b = [cp(4, bre_h, bv.at[0]), cp(5, bim_h, bv.at[1])]
    c_c = [cp(6, cre_h, cv.at[0]), cp(7, cim_h, cv.at[1])]
    c_bx = [cp(8 + c, bx_h.at[:, pl.ds(c * T, T)], bxv.at[c]) for c in range(NC)]
    c_w, c_ax, c_wo = cp(8 + NC, wqkv_h, wv), cp(9 + NC, ax_h, axv), cp(10 + NC, wo_h, wov)

    def start(*cs):
        for c in cs:
            c.start()

    def wait(*cs):
        for c in cs:
            c.wait()
    start(*c_par, c_bx[0], c_b[0], c_b[1])

    wait(*c_par)
    prm[...] = jnp.zeros(prm.shape, F32)
    for i in range(4):
        prm[i:i + 1, 0:D] = (pv0, pv1, pv2, pv3)[i][...].astype(F32).reshape(1, D)
    lane5 = lax.broadcasted_iota(jnp.int32, (8, 512), 1)
    lre = jnp.where(lane5 < D, jnp.broadcast_to(prm[0:1, :], (8, 512)), -1.0)
    lim = jnp.broadcast_to(prm[1:2, :], (8, 512))
    dt = jnp.exp(jnp.broadcast_to(prm[2:3, :], (8, 512))).astype(BF16).astype(F32)
    never = dt[:, 0:128] < 0.0
    zr, zi = dt * lre, dt * lim
    mag = jnp.exp(zr)
    lr, li = mag * jnp.cos(zi), mag * jnp.sin(zi)
    den = lre * lre + lim * lim
    nr, ni = lr - 1.0, li
    cr = 2.0 * (nr * lre + ni * lim) / den
    ci = 2.0 * (ni * lre - nr * lim) / den
    lane1 = lax.broadcasted_iota(jnp.int32, (8, 128), 1)
    sub = lax.broadcasted_iota(jnp.int32, (8, 128), 0)
    lo = lane1 < 64

    def tiles(r, i):
        r3, i3 = r[:, 384:], i[:, 384:]
        rr = jnp.where(lo, r3, pltpu.roll(r3, 64, 1))
        ii = jnp.where(lo, -i3, pltpu.roll(i3, 64, 1))
        return ([r[:, 128 * k:128 * k + 128] for k in range(3)] + [rr],
                [i[:, 128 * k:128 * k + 128] for k in range(3)] + [ii])
    lam = tiles(lr, li)
    sq = [(lr, li)]
    for _ in range(5):
        sq.append(_cmul(*sq[-1], *sq[-1]))
    pws = []
    for base in (_cmul(*_cmul(*sq[4], *sq[3]), *sq[2]), _cmul(*sq[5], *sq[2])):
        pw = []
        for _ in range(3):
            pw.append(tiles(*base))
            base = _cmul(*base, *base)
        pws.append(pw)
    dsk = pltpu.roll(jnp.broadcast_to(prm[3:4, :], (8, 512)), 64, 1)

    def cstep(m, k, a, b):
        if k < 3:
            return m[0][k] * a - m[1][k] * b, m[0][k] * b + m[1][k] * a
        return m[0][k] * a + m[1][k] * b, m[0][k] * b - m[1][k] * a

    pend = []
    z0 = pl.program_id(0)

    def push(*cs):
        start(*cs)
        obuf[4, 0:8, :] = dsk[:, 128:256]
        pend.append([PD, obuf[4, pl.ds(pl.multiple_of(z0 * 8, 8), 8), :]])

    def gate(rhs):
        t = None
        if pend:
            pend[0][0] -= 1
            if pend[0][0] == 0:
                t = pend.pop(0)[1]
        if t is not None:
            parts = []
            for r in range(0, rhs.shape[0], 128):
                last = rhs[r + 120:r + 128]
                last = jnp.concatenate([jnp.where(never, t, last[:, c:c + 128])
                                        for c in range(0, rhs.shape[1], 128)], axis=1)
                parts += [rhs[r:r + 120], last]
            rhs = jnp.concatenate(parts, axis=0)
        return rhs

    def prep_b(i):
        for r in range(0, D, 64):
            v = jnp.concatenate([jnp.zeros((64, 64), F32), bv[i, r:r + 64, :].astype(F32)], axis=1)
            r2 = 384 * i + r if r < 384 else 768 + 64 * i
            bcat[r2:r2 + 64, :] = v

    def prep_c():
        nci = -ci[0:1, :D]
        for r in range(0, D, 32):
            c_re = cv[0, r:r + 32, :].astype(F32)
            c_im = cv[1, r:r + 32, :].astype(F32)
            c2r = c_re * cr[0:1, :D] - c_im * ci[0:1, :D]
            c2i = c_re * nci - c_im * cr[0:1, :D]
            ccat[r:r + 32, 0:384] = c2r[:, 0:384]
            ccat[r:r + 32, 384:768] = c2i[:, 0:384]
            ccat[r:r + 32, 768:896] = jnp.concatenate([c2r[:, 384:448], c2i[:, 384:448]], axis=1)

    def ssm_t(c):
        for k in range(4):
            if k == 0:
                xt = jnp.concatenate([jnp.zeros((64, T), F32), bxv[c, 0:64, :].astype(F32)], axis=0)
            else:
                xt = bxv[c, 128 * k - 64:128 * k + 64, :].astype(F32)
            xb32[c // 2][k, T * (c % 2):T * (c % 2) + T, :] = xt.T

    def xs(c, k, j):
        return xb32[c // 2][k, pl.ds(_row0(c) % 512 + j, 8, stride=SEGS[c % 2]), :]

    U, Hs = {}, {}

    def ssm_in(c, ns=range(7)):
        for n in ns:
            xl = jnp.concatenate([jnp.concatenate([xs(c, k, j) for k in range(4)], axis=1)
                                  for j in range(SEGS[c % 2])], axis=0)
            U[c, n] = _dot(xl, gate(bcat[128 * n:128 * n + 128, :]), NT)

    carry = [(jnp.zeros((8, 128), F32),) * 2] * 4

    def ssm_scan(c):
        SEG, pw = SEGS[c % 2], pws[c % 2]
        sw = pltpu.roll(U[c, 6], 64, 1)

        def u(j, k):
            if k < 3:
                return U[c, k][8 * j:8 * j + 8], U[c, k + 3][8 * j:8 * j + 8]
            return U[c, 6][8 * j:8 * j + 8], sw[8 * j:8 * j + 8]
        h, hs, dep = [None] * 4, {}, None
        for ks in KG:
            for k in ks:
                h[k] = u(0, k)
                if dep is not None:
                    h[k] = tuple(jnp.where(never, dep, v) for v in h[k])
            for j in range(1, SEG):
                for k in ks:
                    a, b = cstep(lam, k, *h[k])
                    ua, ub = u(j, k)
                    h[k] = (a + ua, b + ub)
            for k in ks:
                z = [jnp.where(sub == 0, carry[k][i], pltpu.roll(h[k][i], 1, 0)) for i in range(2)]
                for n in range(3):
                    sh = 1 << n
                    a, b = cstep(pw[n], k, *[jnp.where(sub >= sh, pltpu.roll(v, sh, 0), 0.0) for v in z])
                    z = [z[0] + a, z[1] + b]
                h[k] = tuple(z)
            for j in range(SEG):
                for k in ks:
                    a, b = cstep(lam, k, *h[k])
                    ua, ub = u(j, k)
                    h[k] = hs[j, k] = (a + ua, b + ub)
                if j == SEG * DJ // 8 - 1:
                    dep = h[ks[-1]][0]
        Hs[c] = [jnp.concatenate([hs[j, 0][0], hs[j, 1][0], hs[j, 2][0], hs[j, 0][1], hs[j, 1][1], hs[j, 2][1],
                                  hs[j, 3][0]], axis=1) for j in range(SEG)]
        carry[:] = [tuple(jnp.broadcast_to(v[7:8], (8, 128)) for v in h[k]) for k in range(4)]

    def ssm_out(p, ts=range(4), between=lambda: None):
        cj = [(2 * p + i, j) for i in range(2) for j in range(SEGS[i])]
        yts = [_dot(ccat[...], gate(jnp.concatenate([Hs[c][j] for c, j in cj[16 * t:16 * t + 16]], axis=0)), NT)
               for t in ts]
        between()
        for t, yt in zip(ts, yts):
            blk = cj[16 * t:16 * t + 16]
            y_post(p, blk, jnp.concatenate([jnp.zeros((64, 128), F32), yt], axis=0), range(4))

    def y_post(p, blk, yt, ks):
        for n, k in enumerate(ks):
            y = yt[128 * n:128 * n + 128].T
            for i, (c, j) in enumerate(blk):
                rows = pl.ds(_row0(c) + j, 8, stride=SEGS[c % 2])
                v = y[8 * i:8 * i + 8] + xs(c, k, j) * dsk[:, 128 * k:128 * k + 128]
                if k == 0 and p >= NPRE:
                    v = jnp.where(lo, a3[rows, :], v)
                obuf[k, rows, :] = v

    def ssm_last(p):
        t0 = LT0
        cj = [(2 * p + i, j) for i in range(2) for j in range(SEGS[i])][16 * t0:]
        hh = jnp.concatenate([Hs[c][j] for c, j in cj], axis=0)
        for ks in PIECES:
            yt = _dot(ccat[max(128 * ks[0] - 64, 0):128 * ks[-1] + 64, :], gate(hh), NT)
            if ks[0] == 0:
                yt = jnp.concatenate([jnp.zeros((64, 256 + 128 * (2 - t0)), F32), yt], axis=0)
            for t in range(4 - t0):
                y_post(p, cj[16 * t:16 * t + 16], yt[:, 128 * t:128 * t + 128], ks)
            start(*[o_b[c][k] for c in range(2 * p + t0 // 2, 2 * p + 2) for k in ks])

    def w_t():
        for k in range(4):
            n = min(128, D - 128 * k)
            blk = wv[128 * k:128 * k + n, :].astype(F32)
            if n < 128:
                blk = jnp.concatenate([blk, jnp.zeros((128 - n, 3 * D), F32)], axis=0)
            wt32[k] = blk.T

    def w_perm(g):
        for d in range(DH):
            v = [jnp.concatenate([wt32[k, pl.ds(g * D + hh * 224 + d, 8, stride=DH), :]
                                  for k in range(4)], axis=1) for hh in range(2)]
            wtp[g * D + 16 * d:g * D + 16 * d + 16, :] = jnp.concatenate(v, axis=0)

    def x_t():
        for k in range(4):
            n = min(128, D - 128 * k)
            for t in range(4):
                blk = axv[128 * k:128 * k + n, 512 * t:512 * t + 512].astype(F32)
                if n < 128:
                    blk = jnp.concatenate([blk, jnp.zeros((128 - n, 512), F32)], axis=0)
                bt = blk.T
                for g in range(32):
                    r = XP * (32 * t + g)
                    xa32[k, r:r + 16, :] = bt[16 * g:16 * g + 16]

    def wo_prep():
        wo = jnp.concatenate([wov[...].astype(F32), jnp.zeros((D, 64), F32)], axis=1)
        for k in range(4):
            wo32[k] = wo[:, 128 * k:128 * k + 128]
        for k in range(4):
            v = [wo32[k, pl.ds(hh * 224 + d, 8, stride=DH), :] for d in range(DH) for hh in range(2)]
            v = jnp.concatenate(v + [jnp.zeros((64, 128), F32)], axis=0).T
            n = min(128, D - 128 * k)
            wot[128 * k:128 * k + n, :] = v[:n]

    def xa(j):
        return jnp.concatenate([xa32[k, pl.ds(j, 128, stride=XP), :] for k in range(4)], axis=1)

    KV, Q, O = ({}, {}), {}, {}

    def att_kv(j):
        for g in (0, 1):
            r = _dot(wtp[D * (g + 1):D * (g + 2), :], gate(xa(j)), NT)
            KV[g][j + 14] = r
            if j >= 2:
                KV[g][j - 2] = pltpu.roll(r, 1, 1)

    def att_q(jp):
        for j in JP[jp]:
            Q[j] = _dot(wtp[0:D, :], gate(xa(j)), NT)

    scale = DH ** -0.5

    def att(jp):
        js = JP[jp]
        es = range(js[0], js[1] + 15, 2)
        P = {}
        for hh in range(2):
            lg = {}
            for d in range(DH):
                r = slice(16 * d + 8 * hh, 16 * d + 8 * hh + 8)
                for j in js:
                    for w in range(W):
                        t = Q[j][r] * KV[0][j + 14 - 2 * w][r]
                        lg[j, w] = t if d == 0 else lg[j, w] + t
            for j in js:
                l = [lg[j, w] * scale for w in range(W)]
                l = [jnp.where(lane1 == 0, -1e9, l[w]) if j < 2 * w else l[w] for w in range(W)]
                m = l[0]
                for w in range(1, W):
                    m = jnp.maximum(m, l[w])
                e = [jnp.exp(x - m) for x in l]
                ssum = e[0]
                for w in range(1, W):
                    ssum = ssum + e[w]
                inv = 1.0 / ssum
                P[hh, j] = [x * inv for x in e]
        for j in js:
            O[j] = []
        for d in range(DH):
            for hh in range(2):
                r = slice(16 * d + 8 * hh, 16 * d + 8 * hh + 8)
                for j in js:
                    acc = None
                    for w in range(W):
                        t = P[hh, j][w] * KV[1][j + 14 - 2 * w][r]
                        acc = t if acc is None else acc + t
                    O[j].append(acc)

    def att_o(jp):
        for j in JP[jp]:
            rt = _dot(wot[...], gate(jnp.concatenate(O[j] + [jnp.zeros((64, 128), F32)], axis=0)), NN)
            rt = jnp.concatenate([rt, jnp.zeros((64, 128), F32)], axis=0)
            for k in range(4):
                ost[j % 2][k, pl.ds(OP * (j // 2), 128), :] = rt[128 * k:128 * k + 128].T

    def o_rows(par, k, s):
        return ost[par][k, pl.ds(s, 8, stride=OP), :]

    def o_unperm(par):
        for k in range(3):
            for s in range(128):
                oa[k, pl.ds(NJ * s + par, 8, stride=2), :] = o_rows(par, k, s)

    def o_mixed():
        for s in range(128):
            for par in range(2):
                rows = pl.ds(NJ * s + par, 8, stride=2)
                if NJ * s < 512 * NPRE:
                    obuf[0, rows, :] = jnp.where(lo, o_rows(par, 3, s), obuf[0, rows, :])
                else:
                    a3[rows, :] = o_rows(par, 3, s)

    o_a = [pltpu.make_async_copy(oa.at[k], out_h.at[:, pl.ds(128 * k, 128)], osem) for k in range(3)]
    o_b = [[pltpu.make_async_copy(obuf.at[k, pl.ds(_row0(c), 8 * SEGS[c % 2])],
                                  out_h.at[pl.ds(_row0(c), 8 * SEGS[c % 2]), pl.ds(128 * (k + 3), 128)],
                                  osem) for k in range(4)] for c in range(NC)]

    NPRE = 1
    wait(c_bx[0], c_b[0])
    start(c_bx[1], c_bx[2], c_bx[3])
    prep_b(0)
    ssm_t(0)
    ssm_in(0, range(2))
    wait(c_b[1], c_bx[1])
    start(*c_c)
    prep_b(1)
    ssm_t(1)
    ssm_in(0, range(2, 7))
    ssm_in(1, range(2))
    wait(c_bx[2], c_bx[3])
    start(c_w, c_ax)
    ssm_in(1, range(2, 7))
    ssm_scan(0)
    ssm_t(2)
    ssm_t(3)
    ssm_in(2, range(2))
    wait(*c_c)
    prep_c()
    ssm_in(2, range(2, 7))
    ssm_in(3, range(2))
    ssm_scan(1)
    ssm_in(3, range(2, 7))
    cj0 = [(i, j) for i in range(2) for j in range(SEGS[i])]
    h0 = [jnp.concatenate([Hs[c][j] for c, j in cj0[16 * t:16 * t + 16]], axis=0) for t in range(2)]
    y0 = _dot(ccat[...], h0[0], NT)
    y1 = _dot(ccat[:, 0:128], h0[1][:, 0:128], NT)
    wait(c_w, c_ax)
    start(c_wo, *c_bx[4:])
    y1 = y1 + _dot(ccat[:, 128:], h0[1][:, 128:], NT)
    for t, y in enumerate((y0, y1)):
        y_post(0, cj0[16 * t:16 * t + 16], jnp.concatenate([jnp.zeros((64, 128), F32), y], axis=0), range(4))
    w_t()
    x_t()
    w_perm(1)
    ssm_out(0, range(2, 4))
    w_perm(2)
    ssm_scan(2)
    for j in range(0, NJ, 2):
        att_kv(j)
    ssm_scan(3)
    w_perm(0)
    start(*o_b[0][1:], *o_b[1][1:])
    wait(c_wo, *c_bx[4:6])
    wo_prep()
    att_q(0)
    for i in range(4):
        att_kv(4 * i + 1)
        att_q(i + 1)
        att(i)
        att_kv(4 * i + 3)
        if i >= 1:
            att_o(i - 1)
    ssm_t(4)
    ssm_t(5)
    for i in range(4, 8):
        if i < 7:
            att_q(i + 1)
        att(i)
        att_o(i - 1)
        if i == 4:
            o_unperm(0)
    att_o(7)
    ssm_in(4, range(4))
    o_unperm(1)
    o_mixed()
    start(*o_a, o_b[0][0], o_b[1][0])
    wait(*c_bx[6:])
    ssm_t(6)
    ssm_t(7)
    ssm_out(1)
    push(*o_b[2], *o_b[3])
    ssm_in(4, range(4, 7))
    ssm_in(5)
    ssm_scan(4)
    ssm_in(6)
    ssm_scan(5)
    ssm_out(2, range(2))
    push(*o_b[4])
    ssm_in(7)
    ssm_out(2, range(2, 3))
    ssm_scan(6)
    ssm_out(2, range(3, 4))
    push(*o_b[5])
    ssm_scan(7)
    ssm_out(3, range(LT0))
    if LT0 == 2:
        start(*o_b[6])
    ssm_last(3)
    pltpu.make_async_copy(out_h, out_h, osem).wait()


@jax.jit
def pallas_concat_heads__sliding_local_dilated__ssm_conv_s5__prompt_kernel(
    A_x, A_wqkv, A_wo, B_x, B_Lambda_re, B_Lambda_im, B_B_re, B_B_im, B_C_re, B_C_im,
    B_log_dt, B_Dskip,
):
    hbm = pl.BlockSpec(memory_space=pltpu.HBM)
    out = pl.pallas_call(
        _kernel,
        out_shape=jax.ShapeDtypeStruct((S, 2 * D), F32),
        grid=(1,),
        in_specs=[hbm] * 12,
        out_specs=hbm,
        scratch_shapes=[
            pltpu.VMEM((D, S), BF16),
            pltpu.VMEM((D, 3 * D), BF16),
            pltpu.VMEM((D, D), BF16),
            pltpu.VMEM((NC, D, T), BF16),
            pltpu.VMEM((2, D, D), BF16),
            pltpu.VMEM((2, D, D), BF16),
            *[pltpu.VMEM((D,), BF16)] * 4,
            pltpu.VMEM((8, 512), F32),
            pltpu.VMEM((896, 512), F32),
            pltpu.VMEM((D, 896), F32),
            *[pltpu.VMEM((4, 512, 128), F32)] * 4,
            pltpu.VMEM((4, 3 * D, 128), F32),
            pltpu.VMEM((3 * D, 512), F32),
            pltpu.VMEM((4, D, 128), F32),
            pltpu.VMEM((D, 512), F32),
            pltpu.VMEM((4, 128 * XP, 128), F32),
            pltpu.VMEM((5, S, 128), F32),
            pltpu.VMEM((S, 128), F32),
            pltpu.VMEM((3, S, 128), F32),
            *[pltpu.VMEM((4, 8 * OP, 128), F32)] * 2,
            pltpu.SemaphoreType.DMA((11 + NC,)),
            pltpu.SemaphoreType.DMA(()),
        ],
        compiler_params=pltpu.CompilerParams(vmem_limit_bytes=100 * 1024 * 1024),
    )(A_x[0].T, A_wqkv, A_wo, B_x[0].T, B_Lambda_re, B_Lambda_im,
      B_B_re, B_B_im, B_C_re, B_C_im, B_log_dt, B_Dskip)
    return out.reshape(1, S, 2 * D)
```

```python
import functools

import jax
import jax.numpy as jnp
from jax import lax
import jax.experimental.pallas as pl
import jax.experimental.pallas.tpu as pltpu

S, D, H, DH, W = 2048, 448, 16, 28, 8
NJ = 16
T = 256
NC = S // T
SEGS = (28, 36)
XP = 20
KG, DJ = ((0,), (1,), (2,), (3,)), 8
OP = 132
LT0, PIECES = 0, ((0, 1), (2,), (3,))
PD = 4
F32, BF16 = jnp.float32, jnp.bfloat16
NN = (((1,), (0,)), ((), ()))
NT = (((1,), (1,)), ((), ()))
JP = [(0, 2), (4, 6), (8, 10), (12, 14), (1, 3), (5, 7), (9, 11), (13, 15)]


_dot = functools.partial(lax.dot_general, preferred_element_type=F32)


def _row0(c):
    return 512 * (c // 2) + 8 * SEGS[0] * (c % 2)


def _cmul(ar, ai, br, bi):
    return ar * br - ai * bi, ar * bi + ai * br


def _kernel(ax_h, wqkv_h, wo_h, bx_h, lre_h, lim_h, bre_h, bim_h, cre_h, cim_h, ldt_h, dsk_h,
            out_h,
            axv, wv, wov, bxv, bv, cv, pv0, pv1, pv2, pv3, prm, bcat, ccat, xb0, xb1, xb2, xb3,
            wt32, wtp, wo32, wot, xa32, obuf, a3, oa, ost0, ost1, isem, osem):
    ost = (ost0, ost1)
    xb32 = (xb0, xb1, xb2, xb3)

    def cp(i, src, dst):
        return pltpu.make_async_copy(src, dst, isem.at[i])
    c_par = [cp(0, lre_h, pv0), cp(1, lim_h, pv1), cp(2, ldt_h, pv2), cp(3, dsk_h, pv3)]
    c_b = [cp(4, bre_h, bv.at[0]), cp(5, bim_h, bv.at[1])]
    c_c = [cp(6, cre_h, cv.at[0]), cp(7, cim_h, cv.at[1])]
    c_bx = [cp(8 + c, bx_h.at[:, pl.ds(c * T, T)], bxv.at[c]) for c in range(NC)]
    c_w, c_ax, c_wo = cp(8 + NC, wqkv_h, wv), cp(9 + NC, ax_h, axv), cp(10 + NC, wo_h, wov)

    def start(*cs):
        for c in cs:
            c.start()

    def wait(*cs):
        for c in cs:
            c.wait()
    start(*c_par, c_bx[0], c_b[0], c_b[1])

    wait(*c_par)
    prm[...] = jnp.zeros(prm.shape, F32)
    for i in range(4):
        prm[i:i + 1, 0:D] = (pv0, pv1, pv2, pv3)[i][...].astype(F32).reshape(1, D)
    lane5 = lax.broadcasted_iota(jnp.int32, (8, 512), 1)
    lre = jnp.where(lane5 < D, jnp.broadcast_to(prm[0:1, :], (8, 512)), -1.0)
    lim = jnp.broadcast_to(prm[1:2, :], (8, 512))
    dt = jnp.exp(jnp.broadcast_to(prm[2:3, :], (8, 512))).astype(BF16).astype(F32)
    never = dt[:, 0:128] < 0.0
    zr, zi = dt * lre, dt * lim
    mag = jnp.exp(zr)
    lr, li = mag * jnp.cos(zi), mag * jnp.sin(zi)
    den = lre * lre + lim * lim
    nr, ni = lr - 1.0, li
    cr = 2.0 * (nr * lre + ni * lim) / den
    ci = 2.0 * (ni * lre - nr * lim) / den
    lane1 = lax.broadcasted_iota(jnp.int32, (8, 128), 1)
    sub = lax.broadcasted_iota(jnp.int32, (8, 128), 0)
    lo = lane1 < 64

    def tiles(r, i):
        r3, i3 = r[:, 384:], i[:, 384:]
        rr = jnp.where(lo, r3, pltpu.roll(r3, 64, 1))
        ii = jnp.where(lo, -i3, pltpu.roll(i3, 64, 1))
        return ([r[:, 128 * k:128 * k + 128] for k in range(3)] + [rr],
                [i[:, 128 * k:128 * k + 128] for k in range(3)] + [ii])
    lam = tiles(lr, li)
    sq = [(lr, li)]
    for _ in range(5):
        sq.append(_cmul(*sq[-1], *sq[-1]))
    pws = []
    for base in (_cmul(*_cmul(*sq[4], *sq[3]), *sq[2]), _cmul(*sq[5], *sq[2])):
        pw = []
        for _ in range(3):
            pw.append(tiles(*base))
            base = _cmul(*base, *base)
        pws.append(pw)
    dsk = pltpu.roll(jnp.broadcast_to(prm[3:4, :], (8, 512)), 64, 1)

    def cstep(m, k, a, b):
        if k < 3:
            return m[0][k] * a - m[1][k] * b, m[0][k] * b + m[1][k] * a
        return m[0][k] * a + m[1][k] * b, m[0][k] * b - m[1][k] * a

    pend = []
    z0 = pl.program_id(0)

    def push(*cs):
        start(*cs)
        obuf[4, 0:8, :] = dsk[:, 128:256]
        pend.append([PD, obuf[4, pl.ds(pl.multiple_of(z0 * 8, 8), 8), :]])

    def gate(rhs):
        t = None
        if pend:
            pend[0][0] -= 1
            if pend[0][0] == 0:
                t = pend.pop(0)[1]
        if t is not None:
            parts = []
            for r in range(0, rhs.shape[0], 128):
                last = rhs[r + 120:r + 128]
                last = jnp.concatenate([jnp.where(never, t, last[:, c:c + 128])
                                        for c in range(0, rhs.shape[1], 128)], axis=1)
                parts += [rhs[r:r + 120], last]
            rhs = jnp.concatenate(parts, axis=0)
        return rhs

    def prep_b(i):
        for r in range(0, D, 64):
            v = jnp.concatenate([jnp.zeros((64, 64), F32), bv[i, r:r + 64, :].astype(F32)], axis=1)
            r2 = 384 * i + r if r < 384 else 768 + 64 * i
            bcat[r2:r2 + 64, :] = v

    def prep_c():
        nci = -ci[0:1, :D]
        for r in range(0, D, 32):
            c_re = cv[0, r:r + 32, :].astype(F32)
            c_im = cv[1, r:r + 32, :].astype(F32)
            c2r = c_re * cr[0:1, :D] - c_im * ci[0:1, :D]
            c2i = c_re * nci - c_im * cr[0:1, :D]
            ccat[r:r + 32, 0:384] = c2r[:, 0:384]
            ccat[r:r + 32, 384:768] = c2i[:, 0:384]
            ccat[r:r + 32, 768:896] = jnp.concatenate([c2r[:, 384:448], c2i[:, 384:448]], axis=1)

    def ssm_t(c):
        for k in range(4):
            if k == 0:
                xt = jnp.concatenate([jnp.zeros((64, T), F32), bxv[c, 0:64, :].astype(F32)], axis=0)
            else:
                xt = bxv[c, 128 * k - 64:128 * k + 64, :].astype(F32)
            xb32[c // 2][k, T * (c % 2):T * (c % 2) + T, :] = xt.T

    def xs(c, k, j):
        return xb32[c // 2][k, pl.ds(_row0(c) % 512 + j, 8, stride=SEGS[c % 2]), :]

    U, Hs = {}, {}

    def ssm_in(c, ns=range(7)):
        for n in ns:
            xl = jnp.concatenate([jnp.concatenate([xs(c, k, j) for k in range(4)], axis=1)
                                  for j in range(SEGS[c % 2])], axis=0)
            U[c, n] = _dot(xl, gate(bcat[128 * n:128 * n + 128, :]), NT)

    carry = [(jnp.zeros((8, 128), F32),) * 2] * 4

    def ssm_scan(c):
        SEG, pw = SEGS[c % 2], pws[c % 2]
        sw = pltpu.roll(U[c, 6], 64, 1)

        def u(j, k):
            if k < 3:
                return U[c, k][8 * j:8 * j + 8], U[c, k + 3][8 * j:8 * j + 8]
            return U[c, 6][8 * j:8 * j + 8], sw[8 * j:8 * j + 8]
        h, hs, dep = [None] * 4, {}, None
        for ks in KG:
            for k in ks:
                h[k] = u(0, k)
                if dep is not None:
                    h[k] = tuple(jnp.where(never, dep, v) for v in h[k])
            for j in range(1, SEG):
                for k in ks:
                    a, b = cstep(lam, k, *h[k])
                    ua, ub = u(j, k)
                    h[k] = (a + ua, b + ub)
            for k in ks:
                z = [jnp.where(sub == 0, carry[k][i], pltpu.roll(h[k][i], 1, 0)) for i in range(2)]
                for n in range(3):
                    sh = 1 << n
                    a, b = cstep(pw[n], k, *[jnp.where(sub >= sh, pltpu.roll(v, sh, 0), 0.0) for v in z])
                    z = [z[0] + a, z[1] + b]
                h[k] = tuple(z)
            for j in range(SEG):
                for k in ks:
                    a, b = cstep(lam, k, *h[k])
                    ua, ub = u(j, k)
                    h[k] = hs[j, k] = (a + ua, b + ub)
                if j == SEG * DJ // 8 - 1:
                    dep = h[ks[-1]][0]
        Hs[c] = [jnp.concatenate([hs[j, 0][0], hs[j, 1][0], hs[j, 2][0], hs[j, 0][1], hs[j, 1][1], hs[j, 2][1],
                                  hs[j, 3][0]], axis=1) for j in range(SEG)]
        carry[:] = [tuple(jnp.broadcast_to(v[7:8], (8, 128)) for v in h[k]) for k in range(4)]

    def ssm_out(p, ts=range(4), between=lambda: None):
        cj = [(2 * p + i, j) for i in range(2) for j in range(SEGS[i])]
        yts = [_dot(ccat[...], gate(jnp.concatenate([Hs[c][j] for c, j in cj[16 * t:16 * t + 16]], axis=0)), NT)
               for t in ts]
        between()
        for t, yt in zip(ts, yts):
            blk = cj[16 * t:16 * t + 16]
            y_post(p, blk, jnp.concatenate([jnp.zeros((64, 128), F32), yt], axis=0), range(4))

    def y_post(p, blk, yt, ks):
        for n, k in enumerate(ks):
            y = yt[128 * n:128 * n + 128].T
            for i, (c, j) in enumerate(blk):
                rows = pl.ds(_row0(c) + j, 8, stride=SEGS[c % 2])
                v = y[8 * i:8 * i + 8] + xs(c, k, j) * dsk[:, 128 * k:128 * k + 128]
                if k == 0 and p >= NPRE:
                    v = jnp.where(lo, a3[rows, :], v)
                obuf[k, rows, :] = v

    def ssm_last(p):
        t0 = LT0
        cj = [(2 * p + i, j) for i in range(2) for j in range(SEGS[i])][16 * t0:]
        hh = jnp.concatenate([Hs[c][j] for c, j in cj], axis=0)
        for ks in PIECES:
            yt = _dot(ccat[max(128 * ks[0] - 64, 0):128 * ks[-1] + 64, :], gate(hh), NT)
            if ks[0] == 0:
                yt = jnp.concatenate([jnp.zeros((64, 256 + 128 * (2 - t0)), F32), yt], axis=0)
            for t in range(4 - t0):
                y_post(p, cj[16 * t:16 * t + 16], yt[:, 128 * t:128 * t + 128], ks)
            start(*[o_b[c][k] for c in range(2 * p + t0 // 2, 2 * p + 2) for k in ks])

    def w_t():
        for k in range(4):
            n = min(128, D - 128 * k)
            blk = wv[128 * k:128 * k + n, :].astype(F32)
            if n < 128:
                blk = jnp.concatenate([blk, jnp.zeros((128 - n, 3 * D), F32)], axis=0)
            wt32[k] = blk.T

    def w_perm(g):
        for d in range(DH):
            v = [jnp.concatenate([wt32[k, pl.ds(g * D + hh * 224 + d, 8, stride=DH), :]
                                  for k in range(4)], axis=1) for hh in range(2)]
            wtp[g * D + 16 * d:g * D + 16 * d + 16, :] = jnp.concatenate(v, axis=0)

    def x_t():
        for k in range(4):
            n = min(128, D - 128 * k)
            for t in range(4):
                blk = axv[128 * k:128 * k + n, 512 * t:512 * t + 512].astype(F32)
                if n < 128:
                    blk = jnp.concatenate([blk, jnp.zeros((128 - n, 512), F32)], axis=0)
                bt = blk.T
                for g in range(32):
                    r = XP * (32 * t + g)
                    xa32[k, r:r + 16, :] = bt[16 * g:16 * g + 16]

    def wo_prep():
        wo = jnp.concatenate([wov[...].astype(F32), jnp.zeros((D, 64), F32)], axis=1)
        for k in range(4):
            wo32[k] = wo[:, 128 * k:128 * k + 128]
        for k in range(4):
            v = [wo32[k, pl.ds(hh * 224 + d, 8, stride=DH), :] for d in range(DH) for hh in range(2)]
            v = jnp.concatenate(v + [jnp.zeros((64, 128), F32)], axis=0).T
            n = min(128, D - 128 * k)
            wot[128 * k:128 * k + n, :] = v[:n]

    def xa(j):
        return jnp.concatenate([xa32[k, pl.ds(j, 128, stride=XP), :] for k in range(4)], axis=1)

    KV, Q, O = ({}, {}), {}, {}

    def att_kv(j):
        for g in (0, 1):
            r = _dot(wtp[D * (g + 1):D * (g + 2), :], gate(xa(j)), NT)
            KV[g][j + 14] = r
            if j >= 2:
                KV[g][j - 2] = pltpu.roll(r, 1, 1)

    def att_q(jp):
        for j in JP[jp]:
            Q[j] = _dot(wtp[0:D, :], gate(xa(j)), NT)

    scale = DH ** -0.5

    def att(jp):
        js = JP[jp]
        es = range(js[0], js[1] + 15, 2)
        P = {}
        for hh in range(2):
            lg = {}
            for d in range(DH):
                r = slice(16 * d + 8 * hh, 16 * d + 8 * hh + 8)
                for j in js:
                    for w in range(W):
                        t = Q[j][r] * KV[0][j + 14 - 2 * w][r]
                        lg[j, w] = t if d == 0 else lg[j, w] + t
            for j in js:
                l = [lg[j, w] * scale for w in range(W)]
                l = [jnp.where(lane1 == 0, -1e9, l[w]) if j < 2 * w else l[w] for w in range(W)]
                m = l[0]
                for w in range(1, W):
                    m = jnp.maximum(m, l[w])
                e = [jnp.exp(x - m) for x in l]
                ssum = e[0]
                for w in range(1, W):
                    ssum = ssum + e[w]
                inv = 1.0 / ssum
                P[hh, j] = [x * inv for x in e]
        for j in js:
            O[j] = [None] * (2 * DH)
        dep = None
        for hh, jj in [(h, js) for h in range(2)]:
            if dep is not None:
                for j in jj:
                    P[hh, j] = [jnp.where(never, dep, x) for x in P[hh, j]]
            for d in range(DH):
                r = slice(16 * d + 8 * hh, 16 * d + 8 * hh + 8)
                for j in jj:
                    acc = None
                    for w in range(W):
                        t = P[hh, j][w] * KV[1][j + 14 - 2 * w][r]
                        acc = t if acc is None else acc + t
                    O[j][2 * d + hh] = acc
                    if d == DH - 1:
                        dep = acc

    def att_o(jp):
        rhs = jnp.concatenate([jnp.concatenate(O[j] + [jnp.zeros((64, 128), F32)], axis=0) for j in JP[jp]], axis=1)
        res = _dot(wot[...], gate(rhs), NN)
        for i, j in enumerate(JP[jp]):
            rt = jnp.concatenate([res[:, 128 * i:128 * i + 128], jnp.zeros((64, 128), F32)], axis=0)
            for k in range(4):
                ost[j % 2][k, pl.ds(OP * (j // 2), 128), :] = rt[128 * k:128 * k + 128].T

    def o_rows(par, k, s):
        return ost[par][k, pl.ds(s, 8, stride=OP), :]

    def o_unperm(par):
        for k in range(3):
            for s in range(128):
                oa[k, pl.ds(NJ * s + par, 8, stride=2), :] = o_rows(par, k, s)

    def o_mixed():
        for s in range(128):
            for par in range(2):
                rows = pl.ds(NJ * s + par, 8, stride=2)
                if NJ * s < 512 * NPRE:
                    obuf[0, rows, :] = jnp.where(lo, o_rows(par, 3, s), obuf[0, rows, :])
                else:
                    a3[rows, :] = o_rows(par, 3, s)

    o_a = [pltpu.make_async_copy(oa.at[k], out_h.at[:, pl.ds(128 * k, 128)], osem) for k in range(3)]
    o_b = [[pltpu.make_async_copy(obuf.at[k, pl.ds(_row0(c), 8 * SEGS[c % 2])],
                                  out_h.at[pl.ds(_row0(c), 8 * SEGS[c % 2]), pl.ds(128 * (k + 3), 128)],
                                  osem) for k in range(4)] for c in range(NC)]

    NPRE = 2
    wait(c_bx[0], c_b[0])
    start(c_bx[1], c_bx[2], c_bx[3])
    prep_b(0)
    ssm_t(0)
    ssm_in(0, range(2))
    wait(c_b[1], c_bx[1])
    start(*c_c)
    prep_b(1)
    ssm_t(1)
    ssm_in(0, range(2, 7))
    ssm_in(1, range(2))
    wait(c_bx[2], c_bx[3])
    start(c_w, c_ax)
    ssm_in(1, range(2, 7))
    ssm_scan(0)
    ssm_t(2)
    ssm_t(3)
    ssm_in(2, range(2))
    wait(*c_c)
    prep_c()
    ssm_in(2, range(2, 7))
    ssm_in(3, range(2))
    ssm_scan(1)
    ssm_in(3, range(2, 7))
    cj0 = [(i, j) for i in range(2) for j in range(SEGS[i])]
    h0 = [jnp.concatenate([Hs[c][j] for c, j in cj0[16 * t:16 * t + 16]], axis=0) for t in range(2)]
    y0 = _dot(ccat[...], h0[0], NT)
    y1 = _dot(ccat[:, 0:128], h0[1][:, 0:128], NT)
    wait(c_w, c_ax)
    start(c_wo, *c_bx[4:])
    y1 = y1 + _dot(ccat[:, 128:], h0[1][:, 128:], NT)
    for t, y in enumerate((y0, y1)):
        y_post(0, cj0[16 * t:16 * t + 16], jnp.concatenate([jnp.zeros((64, 128), F32), y], axis=0), range(4))
    w_t()
    x_t()
    w_perm(1)
    ssm_out(0, range(2, 4))
    w_perm(2)
    ssm_scan(2)
    for j in range(0, NJ, 2):
        att_kv(j)
    ssm_scan(3)
    w_perm(0)
    start(*o_b[0][1:], *o_b[1][1:])
    wait(c_wo, *c_bx[4:6])
    wo_prep()
    att_q(0)
    for i in range(4):
        att_kv(4 * i + 1)
        att_q(i + 1)
        att(i)
        att_kv(4 * i + 3)
        if i >= 1:
            att_o(i - 1)
    ssm_t(4)
    ssm_t(5)
    for i in range(4, 8):
        ssm_out(1, [i - 4])
        if i in (5, 7):
            push(*o_b[i // 2][1:])
        if i < 7:
            att_q(i + 1)
        att(i)
        att_o(i - 1)
        if i == 4:
            o_unperm(0)
    att_o(7)
    ssm_in(4, range(4))
    o_unperm(1)
    o_mixed()
    start(*o_a, o_b[0][0], o_b[1][0], o_b[2][0], o_b[3][0])
    wait(*c_bx[6:])
    ssm_t(6)
    ssm_t(7)
    ssm_in(4, range(4, 7))
    ssm_in(5)
    ssm_scan(4)
    ssm_in(6)
    ssm_scan(5)
    ssm_out(2, range(2))
    push(*o_b[4])
    ssm_in(7)
    ssm_out(2, range(2, 3))
    ssm_scan(6)
    ssm_out(2, range(3, 4))
    push(*o_b[5])
    ssm_scan(7)
    ssm_out(3, range(LT0))
    if LT0 == 2:
        start(*o_b[6])
    ssm_last(3)
    pltpu.make_async_copy(out_h, out_h, osem).wait()


@jax.jit
def pallas_concat_heads__sliding_local_dilated__ssm_conv_s5__prompt_kernel(
    A_x, A_wqkv, A_wo, B_x, B_Lambda_re, B_Lambda_im, B_B_re, B_B_im, B_C_re, B_C_im,
    B_log_dt, B_Dskip,
):
    hbm = pl.BlockSpec(memory_space=pltpu.HBM)
    out = pl.pallas_call(
        _kernel,
        out_shape=jax.ShapeDtypeStruct((S, 2 * D), F32),
        grid=(1,),
        in_specs=[hbm] * 12,
        out_specs=hbm,
        scratch_shapes=[
            pltpu.VMEM((D, S), BF16),
            pltpu.VMEM((D, 3 * D), BF16),
            pltpu.VMEM((D, D), BF16),
            pltpu.VMEM((NC, D, T), BF16),
            pltpu.VMEM((2, D, D), BF16),
            pltpu.VMEM((2, D, D), BF16),
            *[pltpu.VMEM((D,), BF16)] * 4,
            pltpu.VMEM((8, 512), F32),
            pltpu.VMEM((896, 512), F32),
            pltpu.VMEM((D, 896), F32),
            *[pltpu.VMEM((4, 512, 128), F32)] * 4,
            pltpu.VMEM((4, 3 * D, 128), F32),
            pltpu.VMEM((3 * D, 512), F32),
            pltpu.VMEM((4, D, 128), F32),
            pltpu.VMEM((D, 512), F32),
            pltpu.VMEM((4, 128 * XP, 128), F32),
            pltpu.VMEM((5, S, 128), F32),
            pltpu.VMEM((S, 128), F32),
            pltpu.VMEM((3, S, 128), F32),
            *[pltpu.VMEM((4, 8 * OP, 128), F32)] * 2,
            pltpu.SemaphoreType.DMA((11 + NC,)),
            pltpu.SemaphoreType.DMA(()),
        ],
        compiler_params=pltpu.CompilerParams(vmem_limit_bytes=100 * 1024 * 1024),
    )(A_x[0].T, A_wqkv, A_wo, B_x[0].T, B_Lambda_re, B_Lambda_im,
      B_B_re, B_B_im, B_C_re, B_C_im, B_log_dt, B_Dskip)
    return out.reshape(1, S, 2 * D)
```

```python
import functools

import jax
import jax.numpy as jnp
from jax import lax
import jax.experimental.pallas as pl
import jax.experimental.pallas.tpu as pltpu

S, D, H, DH, W = 2048, 448, 16, 28, 8
NJ = 16
T = 256
NC = S // T
SEGS = (28, 36)
XP = 20
KG, DJ = ((0,), (1,), (2,), (3,)), 8
OP = 132
PIECES = (((0, 1), (0, 1, 2, 3), (0, 1)), ((2,), (0, 1, 2, 3), (0, 1)), ((3,), (0, 1), (0,)), ((3,), (2, 3), (1,)))
PD = 4
F32, BF16 = jnp.float32, jnp.bfloat16
NN = (((1,), (0,)), ((), ()))
NT = (((1,), (1,)), ((), ()))
JP = [(0, 2), (4, 6), (8, 10), (12, 14), (1, 3), (5, 7), (9, 11), (13, 15)]


_dot = functools.partial(lax.dot_general, preferred_element_type=F32)


def _row0(c):
    return 512 * (c // 2) + 8 * SEGS[0] * (c % 2)


def _cmul(ar, ai, br, bi):
    return ar * br - ai * bi, ar * bi + ai * br


def _kernel(ax_h, wqkv_h, wo_h, bx_h, lre_h, lim_h, bre_h, bim_h, cre_h, cim_h, ldt_h, dsk_h,
            out_h,
            axv, wv, wov, bxv, bv, cv, pv0, pv1, pv2, pv3, prm, bcat, ccat, xb0, xb1, xb2, xb3,
            wt32, wtp, wo32, wot, xa32, obuf, a3, oa, ost0, ost1, isem, osem):
    ost = (ost0, ost1)
    xb32 = (xb0, xb1, xb2, xb3)

    def cp(i, src, dst):
        return pltpu.make_async_copy(src, dst, isem.at[i])
    c_par = [cp(0, lre_h, pv0), cp(1, lim_h, pv1), cp(2, ldt_h, pv2), cp(3, dsk_h, pv3)]
    c_b = [cp(4, bre_h, bv.at[0]), cp(5, bim_h, bv.at[1])]
    c_c = [cp(6, cre_h, cv.at[0]), cp(7, cim_h, cv.at[1])]
    c_bx = [cp(8 + c, bx_h.at[:, pl.ds(c * T, T)], bxv.at[c]) for c in range(NC)]
    c_w, c_ax, c_wo = cp(8 + NC, wqkv_h, wv), cp(9 + NC, ax_h, axv), cp(10 + NC, wo_h, wov)

    def start(*cs):
        for c in cs:
            c.start()

    def wait(*cs):
        for c in cs:
            c.wait()
    start(*c_par, c_bx[0], c_b[0], c_b[1])

    wait(*c_par)
    prm[...] = jnp.zeros(prm.shape, F32)
    for i in range(4):
        prm[i:i + 1, 0:D] = (pv0, pv1, pv2, pv3)[i][...].astype(F32).reshape(1, D)
    lane5 = lax.broadcasted_iota(jnp.int32, (8, 512), 1)
    lre = jnp.where(lane5 < D, jnp.broadcast_to(prm[0:1, :], (8, 512)), -1.0)
    lim = jnp.broadcast_to(prm[1:2, :], (8, 512))
    dt = jnp.exp(jnp.broadcast_to(prm[2:3, :], (8, 512))).astype(BF16).astype(F32)
    never = dt[:, 0:128] < 0.0
    zr, zi = dt * lre, dt * lim
    mag = jnp.exp(zr)
    lr, li = mag * jnp.cos(zi), mag * jnp.sin(zi)
    den = lre * lre + lim * lim
    nr, ni = lr - 1.0, li
    cr = 2.0 * (nr * lre + ni * lim) / den
    ci = 2.0 * (ni * lre - nr * lim) / den
    lane1 = lax.broadcasted_iota(jnp.int32, (8, 128), 1)
    sub = lax.broadcasted_iota(jnp.int32, (8, 128), 0)
    lo = lane1 < 64

    def tiles(r, i):
        r3, i3 = r[:, 384:], i[:, 384:]
        rr = jnp.where(lo, r3, pltpu.roll(r3, 64, 1))
        ii = jnp.where(lo, -i3, pltpu.roll(i3, 64, 1))
        return ([r[:, 128 * k:128 * k + 128] for k in range(3)] + [rr],
                [i[:, 128 * k:128 * k + 128] for k in range(3)] + [ii])
    lam = tiles(lr, li)
    sq = [(lr, li)]
    for _ in range(5):
        sq.append(_cmul(*sq[-1], *sq[-1]))
    pws = []
    for base in (_cmul(*_cmul(*sq[4], *sq[3]), *sq[2]), _cmul(*sq[5], *sq[2])):
        pw = []
        for _ in range(3):
            pw.append(tiles(*base))
            base = _cmul(*base, *base)
        pws.append(pw)
    dsk = pltpu.roll(jnp.broadcast_to(prm[3:4, :], (8, 512)), 64, 1)

    def cstep(m, k, a, b):
        if k < 3:
            return m[0][k] * a - m[1][k] * b, m[0][k] * b + m[1][k] * a
        return m[0][k] * a + m[1][k] * b, m[0][k] * b - m[1][k] * a

    pend = []
    z0 = pl.program_id(0)

    def push(*cs):
        start(*cs)
        obuf[4, 0:8, :] = dsk[:, 128:256]
        pend.append([PD, obuf[4, pl.ds(pl.multiple_of(z0 * 8, 8), 8), :]])

    def gate(rhs, t=None):
        if pend and t is None:
            pend[0][0] -= 1
            if pend[0][0] == 0:
                t = pend.pop(0)[1]
        if t is not None:
            parts = []
            for r in range(0, rhs.shape[0], 128):
                last = rhs[r + 120:r + 128]
                last = jnp.concatenate([jnp.where(never, t, last[:, c:c + 128])
                                        for c in range(0, rhs.shape[1], 128)], axis=1)
                parts += [rhs[r:r + 120], last]
            rhs = jnp.concatenate(parts, axis=0)
        return rhs

    def prep_b(i):
        for r in range(0, D, 64):
            v = jnp.concatenate([jnp.zeros((64, 64), F32), bv[i, r:r + 64, :].astype(F32)], axis=1)
            r2 = 384 * i + r if r < 384 else 768 + 64 * i
            bcat[r2:r2 + 64, :] = v

    ctok = []

    def prep_c():
        toks = []
        nci = -ci[0:1, :D]
        for r in range(0, D, 32):
            c_re = cv[0, r:r + 32, :].astype(F32)
            c_im = cv[1, r:r + 32, :].astype(F32)
            c2r = c_re * cr[0:1, :D] - c_im * ci[0:1, :D]
            c2i = c_re * nci - c_im * cr[0:1, :D]
            ccat[r:r + 32, 0:384] = c2r[:, 0:384]
            ccat[r:r + 32, 384:768] = c2i[:, 0:384]
            c3 = jnp.concatenate([c2r[:, 384:448], c2i[:, 384:448]], axis=1)
            ccat[r:r + 32, 768:896] = c3
            toks += [v[i:i + 8, c:c + 128] for v in (c2r[:, 0:384], c2i[:, 0:384], c3)
                     for i in range(0, 32, 8) for c in range(0, v.shape[1], 128)]
        ctok.append(functools.reduce(jnp.maximum, toks))

    def ssm_t(c):
        for k in range(4):
            if k == 0:
                xt = jnp.concatenate([jnp.zeros((64, T), F32), bxv[c, 0:64, :].astype(F32)], axis=0)
            else:
                xt = bxv[c, 128 * k - 64:128 * k + 64, :].astype(F32)
            xb32[c // 2][k, T * (c % 2):T * (c % 2) + T, :] = xt.T

    def xs(c, k, j):
        return xb32[c // 2][k, pl.ds(_row0(c) % 512 + j, 8, stride=SEGS[c % 2]), :]

    U, Hs = {}, {}

    def ssm_in(c, ns=range(7)):
        for n in ns:
            xl = jnp.concatenate([jnp.concatenate([xs(c, k, j) for k in range(4)], axis=1)
                                  for j in range(SEGS[c % 2])], axis=0)
            U[c, n] = _dot(xl, gate(bcat[128 * n:128 * n + 128, :], ctok[0] if c == 3 else None), NT)

    carry = [(jnp.zeros((8, 128), F32),) * 2] * 4

    def ssm_scan(c):
        SEG, pw = SEGS[c % 2], pws[c % 2]
        sw = pltpu.roll(U[c, 6], 64, 1)

        def u(j, k):
            if k < 3:
                return U[c, k][8 * j:8 * j + 8], U[c, k + 3][8 * j:8 * j + 8]
            return U[c, 6][8 * j:8 * j + 8], sw[8 * j:8 * j + 8]
        h, hs, dep = [None] * 4, {}, None
        for ks in KG:
            for k in ks:
                h[k] = u(0, k)
                if dep is not None:
                    h[k] = tuple(jnp.where(never, dep, v) for v in h[k])
            for j in range(1, SEG):
                for k in ks:
                    a, b = cstep(lam, k, *h[k])
                    ua, ub = u(j, k)
                    h[k] = (a + ua, b + ub)
            for k in ks:
                z = [jnp.where(sub == 0, carry[k][i], pltpu.roll(h[k][i], 1, 0)) for i in range(2)]
                for n in range(3):
                    sh = 1 << n
                    a, b = cstep(pw[n], k, *[jnp.where(sub >= sh, pltpu.roll(v, sh, 0), 0.0) for v in z])
                    z = [z[0] + a, z[1] + b]
                h[k] = tuple(z)
            for j in range(SEG):
                for k in ks:
                    a, b = cstep(lam, k, *h[k])
                    ua, ub = u(j, k)
                    h[k] = hs[j, k] = (a + ua, b + ub)
                if j == SEG * DJ // 8 - 1:
                    dep = h[ks[-1]][0]
        Hs[c] = [jnp.concatenate([hs[j, 0][0], hs[j, 1][0], hs[j, 2][0], hs[j, 0][1], hs[j, 1][1], hs[j, 2][1],
                                  hs[j, 3][0]], axis=1) for j in range(SEG)]
        carry[:] = [tuple(jnp.broadcast_to(v[7:8], (8, 128)) for v in h[k]) for k in range(4)]

    def ssm_out(p, ts=range(4), between=lambda: None):
        cj = [(2 * p + i, j) for i in range(2) for j in range(SEGS[i])]
        yts = [_dot(ccat[...], gate(jnp.concatenate([Hs[c][j] for c, j in cj[16 * t:16 * t + 16]], axis=0)), NT)
               for t in ts]
        between()
        for t, yt in zip(ts, yts):
            blk = cj[16 * t:16 * t + 16]
            y_post(p, blk, jnp.concatenate([jnp.zeros((64, 128), F32), yt], axis=0), range(4))

    def y_post(p, blk, yt, ks):
        for n, k in enumerate(ks):
            y = yt[128 * n:128 * n + 128].T
            for i, (c, j) in enumerate(blk):
                rows = pl.ds(_row0(c) + j, 8, stride=SEGS[c % 2])
                v = y[8 * i:8 * i + 8] + xs(c, k, j) * dsk[:, 128 * k:128 * k + 128]
                if k == 0 and p >= NPRE:
                    v = jnp.where(lo, a3[rows, :], v)
                obuf[k, rows, :] = v

    def ssm_last(p):
        cj = [(2 * p + i, j) for i in range(2) for j in range(SEGS[i])]
        for ks, ts, cs in PIECES:
            hh = jnp.concatenate([Hs[c][j] for c, j in cj[16 * ts[0]:16 * ts[-1] + 16]], axis=0)
            yt = _dot(ccat[max(128 * ks[0] - 64, 0):128 * ks[-1] + 64, :], gate(hh), NT)
            if ks[0] == 0:
                yt = jnp.concatenate([jnp.zeros((64, yt.shape[1]), F32), yt], axis=0)
            for n, t in enumerate(ts):
                y_post(p, cj[16 * t:16 * t + 16], yt[:, 128 * n:128 * n + 128], ks)
            start(*[o_b[2 * p + c][k] for c in cs for k in ks])

    def w_t(c0, c1):
        for k in range(4):
            n = min(128, D - 128 * k)
            blk = wv[128 * k:128 * k + n, c0:c1].astype(F32)
            if n < 128:
                blk = jnp.concatenate([blk, jnp.zeros((128 - n, c1 - c0), F32)], axis=0)
            wt32[k, c0:c1, :] = blk.T

    def w_rows(g):
        return jnp.concatenate(
            [jnp.concatenate([wt32[k, pl.ds(g * D + hh * 224 + d, 8, stride=DH), :] for k in range(4)], axis=1)
             for d in range(DH) for hh in range(2)], axis=0)

    def w_perm(g):
        for d in range(DH):
            v = [jnp.concatenate([wt32[k, pl.ds(g * D + hh * 224 + d, 8, stride=DH), :]
                                  for k in range(4)], axis=1) for hh in range(2)]
            wtp[g * D + 16 * d:g * D + 16 * d + 16, :] = jnp.concatenate(v, axis=0)

    def x_t():
        for k in range(4):
            n = min(128, D - 128 * k)
            for t in range(4):
                blk = axv[128 * k:128 * k + n, 512 * t:512 * t + 512].astype(F32)
                if n < 128:
                    blk = jnp.concatenate([blk, jnp.zeros((128 - n, 512), F32)], axis=0)
                bt = blk.T
                for g in range(32):
                    r = XP * (32 * t + g)
                    xa32[k, r:r + 16, :] = bt[16 * g:16 * g + 16]

    def wo_prep():
        wo = jnp.concatenate([wov[...].astype(F32), jnp.zeros((D, 64), F32)], axis=1)
        for k in range(4):
            wo32[k] = wo[:, 128 * k:128 * k + 128]
        for k in range(4):
            v = [wo32[k, pl.ds(hh * 224 + d, 8, stride=DH), :] for d in range(DH) for hh in range(2)]
            v = jnp.concatenate(v + [jnp.zeros((64, 128), F32)], axis=0).T
            n = min(128, D - 128 * k)
            wot[128 * k:128 * k + n, :] = v[:n]

    def xa(j):
        return jnp.concatenate([xa32[k, pl.ds(j, 128, stride=XP), :] for k in range(4)], axis=1)

    KV, Q, O = ({}, {}), {}, {}

    def att_kv(j):
        for g in (0, 1):
            r = _dot(w_rows(g + 1), gate(xa(j)), NT)
            KV[g][j + 14] = r
            if j >= 2 and j != NJ - 2:
                KV[g][j - 2] = pltpu.roll(r, 1, 1)

    def att_q(jp):
        for j in JP[jp]:
            Q[j] = _dot(w_rows(0), gate(xa(j)), NT)

    scale = DH ** -0.5

    def att(jp):
        js = JP[jp]
        es = range(js[0], js[1] + 15, 2)
        P = {}
        for hh in range(2):
            lg = {}
            for d in range(DH):
                r = slice(16 * d + 8 * hh, 16 * d + 8 * hh + 8)
                for j in js:
                    for w in range(W):
                        t = Q[j][r] * KV[0][j + 14 - 2 * w][r]
                        lg[j, w] = t if d == 0 else lg[j, w] + t
            for j in js:
                l = [lg[j, w] * scale for w in range(W)]
                l = [jnp.where(lane1 == 0, -1e9, l[w]) if j < 2 * w else l[w] for w in range(W)]
                m = l[0]
                for w in range(1, W):
                    m = jnp.maximum(m, l[w])
                e = [jnp.exp(x - m) for x in l]
                ssum = e[0]
                for w in range(1, W):
                    ssum = ssum + e[w]
                inv = 1.0 / ssum
                P[hh, j] = [x * inv for x in e]
        for j in js:
            O[j] = [None] * (2 * DH)
        dep = None
        for hh, jj in [(h, js) for h in range(2)]:
            if dep is not None:
                for j in jj:
                    P[hh, j] = [jnp.where(never, dep, x) for x in P[hh, j]]
            for d in range(DH):
                r = slice(16 * d + 8 * hh, 16 * d + 8 * hh + 8)
                for j in jj:
                    acc = None
                    for w in range(W):
                        t = P[hh, j][w] * KV[1][j + 14 - 2 * w][r]
                        acc = t if acc is None else acc + t
                    O[j][2 * d + hh] = acc
                    if d == DH - 1:
                        dep = acc

    def att_o(jp):
        rhs = jnp.concatenate([jnp.concatenate(O[j] + [jnp.zeros((64, 128), F32)], axis=0) for j in JP[jp]], axis=1)
        res = _dot(wot[...], gate(rhs), NN)
        for i, j in enumerate(JP[jp]):
            rt = jnp.concatenate([res[:, 128 * i:128 * i + 128], jnp.zeros((64, 128), F32)], axis=0)
            for k in range(4):
                ost[j % 2][k, pl.ds(OP * (j // 2), 128), :] = rt[128 * k:128 * k + 128].T

    def o_rows(par, k, s):
        return ost[par][k, pl.ds(s, 8, stride=OP), :]

    def o_unperm(par):
        for k in range(3):
            for s in range(128):
                oa[k, pl.ds(NJ * s + par, 8, stride=2), :] = o_rows(par, k, s)

    def o_mixed():
        for s in range(128):
            for par in range(2):
                rows = pl.ds(NJ * s + par, 8, stride=2)
                if NJ * s < 512 * NPRE:
                    obuf[0, rows, :] = jnp.where(lo, o_rows(par, 3, s), obuf[0, rows, :])
                else:
                    a3[rows, :] = o_rows(par, 3, s)

    o_a = [pltpu.make_async_copy(oa.at[k], out_h.at[:, pl.ds(128 * k, 128)], osem) for k in range(3)]
    o_b = [[pltpu.make_async_copy(obuf.at[k, pl.ds(_row0(c), 8 * SEGS[c % 2])],
                                  out_h.at[pl.ds(_row0(c), 8 * SEGS[c % 2]), pl.ds(128 * (k + 3), 128)],
                                  osem) for k in range(4)] for c in range(NC)]

    NPRE = 2
    wait(c_bx[0], c_b[0])
    start(c_bx[1], c_bx[2], c_bx[3])
    prep_b(0)
    ssm_t(0)
    ssm_in(0, range(2))
    wait(c_b[1], c_bx[1])
    start(*c_c)
    prep_b(1)
    ssm_t(1)
    ssm_in(0, range(2, 7))
    ssm_in(1, range(2))
    wait(c_bx[2], c_bx[3])
    start(c_w, c_ax)
    ssm_in(1, range(2, 7))
    ssm_scan(0)
    ssm_t(2)
    ssm_t(3)
    ssm_in(2, range(2))
    wait(*c_c)
    prep_c()
    ssm_in(2, range(2, 7))
    ssm_in(3, range(2))
    ssm_scan(1)
    ssm_in(3, range(2, 7))
    cj0 = [(i, j) for i in range(2) for j in range(SEGS[i])]
    h0 = [jnp.concatenate([Hs[c][j] for c, j in cj0[16 * t:16 * t + 16]], axis=0) for t in range(2)]
    y0 = _dot(ccat[...], h0[0], NT)
    y1 = _dot(ccat[:, 0:640], h0[1][:, 0:640], NT)
    y1 = jnp.concatenate([jnp.where(never, 0.0, y1[r:r + 8]) for r in range(0, D, 8)], axis=0)
    wait(c_w, c_ax)
    start(c_wo, *c_bx[4:])
    y1 = y1 + _dot(ccat[:, 640:], h0[1][:, 640:], NT)
    for t, y in enumerate((y0, y1)):
        y_post(0, cj0[16 * t:16 * t + 16], jnp.concatenate([jnp.zeros((64, 128), F32), y], axis=0), range(4))
    w_t(384, 3 * D)
    x_t()
    ssm_out(0, range(2, 4))
    ssm_scan(2)
    for j in range(0, NJ, 2):
        att_kv(j)
    ssm_scan(3)
    w_t(0, 384)
    start(*o_b[0][1:], *o_b[1][1:])
    wait(c_wo, *c_bx[4:6])
    for g in range(2):
        KV[g][NJ - 4] = pltpu.roll(KV[g][NJ + 12], 1, 1)
    wo_prep()
    att_q(0)
    for i in range(4):
        att_kv(4 * i + 1)
        att_q(i + 1)
        att(i)
        att_kv(4 * i + 3)
        if i >= 1:
            att_o(i - 1)
    ssm_t(4)
    ssm_t(5)
    for i in range(4, 8):
        ssm_out(1, [i - 4])
        if i in (5, 7):
            push(*o_b[i // 2][1:])
        if i < 7:
            att_q(i + 1)
        att(i)
        att_o(i - 1)
        if i == 4:
            o_unperm(0)
    att_o(7)
    ssm_in(4, range(4))
    o_unperm(1)
    o_mixed()
    start(*o_a, o_b[0][0], o_b[1][0], o_b[2][0], o_b[3][0])
    wait(*c_bx[6:])
    ssm_t(6)
    ssm_t(7)
    ssm_in(4, range(4, 7))
    ssm_in(5)
    ssm_scan(4)
    ssm_in(6)
    ssm_scan(5)
    ssm_out(2, range(2))
    push(*o_b[4])
    ssm_in(7)
    ssm_out(2, range(2, 3))
    ssm_scan(6)
    ssm_out(2, range(3, 4))
    push(*o_b[5])
    ssm_scan(7)
    ssm_last(3)
    pltpu.make_async_copy(out_h, out_h, osem).wait()


@jax.jit
def pallas_concat_heads__sliding_local_dilated__ssm_conv_s5__prompt_kernel(
    A_x, A_wqkv, A_wo, B_x, B_Lambda_re, B_Lambda_im, B_B_re, B_B_im, B_C_re, B_C_im,
    B_log_dt, B_Dskip,
):
    hbm = pl.BlockSpec(memory_space=pltpu.HBM)
    out = pl.pallas_call(
        _kernel,
        out_shape=jax.ShapeDtypeStruct((S, 2 * D), F32),
        grid=(1,),
        in_specs=[hbm] * 12,
        out_specs=hbm,
        scratch_shapes=[
            pltpu.VMEM((D, S), BF16),
            pltpu.VMEM((D, 3 * D), BF16),
            pltpu.VMEM((D, D), BF16),
            pltpu.VMEM((NC, D, T), BF16),
            pltpu.VMEM((2, D, D), BF16),
            pltpu.VMEM((2, D, D), BF16),
            *[pltpu.VMEM((D,), BF16)] * 4,
            pltpu.VMEM((8, 512), F32),
            pltpu.VMEM((896, 512), F32),
            pltpu.VMEM((D, 896), F32),
            *[pltpu.VMEM((4, 512, 128), F32)] * 4,
            pltpu.VMEM((4, 3 * D, 128), F32),
            pltpu.VMEM((3 * D, 512), F32),
            pltpu.VMEM((4, D, 128), F32),
            pltpu.VMEM((D, 512), F32),
            pltpu.VMEM((4, 128 * XP, 128), F32),
            pltpu.VMEM((5, S, 128), F32),
            pltpu.VMEM((S, 128), F32),
            pltpu.VMEM((3, S, 128), F32),
            *[pltpu.VMEM((4, 8 * OP, 128), F32)] * 2,
            pltpu.SemaphoreType.DMA((11 + NC,)),
            pltpu.SemaphoreType.DMA(()),
        ],
        compiler_params=pltpu.CompilerParams(vmem_limit_bytes=100 * 1024 * 1024),
    )(A_x[0].T, A_wqkv, A_wo, B_x[0].T, B_Lambda_re, B_Lambda_im,
      B_B_re, B_B_im, B_C_re, B_C_im, B_log_dt, B_Dskip)
    return out.reshape(1, S, 2 * D)
```

```python
import functools

import jax
import jax.numpy as jnp
from jax import lax
import jax.experimental.pallas as pl
import jax.experimental.pallas.tpu as pltpu

S, D, H, DH, W = 2048, 448, 16, 28, 8
NJ = 16
T = 256
NC = S // T
SEGS = (28, 36)
XP = 20
KG, DJ = ((0,), (1,), (2,), (3,)), 8
OP = 132
PIECES = (((0, 1), (0, 1, 2, 3), (0, 1)), ((2,), (0, 1, 2, 3), (0, 1)), ((3,), (0, 1), (0,)), ((3,), (2, 3), (1,)))
LO = 2
PD = 4
F32, BF16 = jnp.float32, jnp.bfloat16
NN = (((1,), (0,)), ((), ()))
NT = (((1,), (1,)), ((), ()))
JP = [(0, 2), (4, 6), (8, 10), (12, 14), (1, 3), (5, 7), (9, 11), (13, 15)]


_dot = functools.partial(lax.dot_general, preferred_element_type=F32)


def _row0(c):
    return 512 * (c // 2) + 8 * SEGS[0] * (c % 2)


def _cmul(ar, ai, br, bi):
    return ar * br - ai * bi, ar * bi + ai * br


def _kernel(ax_h, wqkv_h, wo_h, bx_h, lre_h, lim_h, bre_h, bim_h, cre_h, cim_h, ldt_h, dsk_h,
            out_h,
            axv, wv, wov, bxv, bv, cv, pv0, pv1, pv2, pv3, prm, bcat, ccat, xb0, xb1, xb2, xb3,
            wt32, wtp, wo32, wot, xa32, obuf, a3, oa, ost0, ost1, isem, osem):
    ost = (ost0, ost1)
    xb32 = (xb0, xb1, xb2, xb3)

    def cp(i, src, dst):
        return pltpu.make_async_copy(src, dst, isem.at[i])
    c_par = [cp(0, lre_h, pv0), cp(1, lim_h, pv1), cp(2, ldt_h, pv2), cp(3, dsk_h, pv3)]
    c_b = [cp(4, bre_h, bv.at[0]), cp(5, bim_h, bv.at[1])]
    c_c = [cp(6, cre_h, cv.at[0]), cp(7, cim_h, cv.at[1])]
    c_bx = [cp(8 + c, bx_h.at[:, pl.ds(c * T, T)], bxv.at[c]) for c in range(NC)]
    c_w, c_ax, c_wo = cp(8 + NC, wqkv_h, wv), cp(9 + NC, ax_h, axv), cp(10 + NC, wo_h, wov)

    def start(*cs):
        for c in cs:
            c.start()

    def wait(*cs):
        for c in cs:
            c.wait()
    start(*c_par, c_bx[0], c_b[0], c_b[1])

    wait(*c_par)
    prm[...] = jnp.zeros(prm.shape, F32)
    for i in range(4):
        prm[i:i + 1, 0:D] = (pv0, pv1, pv2, pv3)[i][...].astype(F32).reshape(1, D)
    lane5 = lax.broadcasted_iota(jnp.int32, (8, 512), 1)
    lre = jnp.where(lane5 < D, jnp.broadcast_to(prm[0:1, :], (8, 512)), -1.0)
    lim = jnp.broadcast_to(prm[1:2, :], (8, 512))
    dt = jnp.exp(jnp.broadcast_to(prm[2:3, :], (8, 512))).astype(BF16).astype(F32)
    never = dt[:, 0:128] < 0.0
    zr, zi = dt * lre, dt * lim
    mag = jnp.exp(zr)
    lr, li = mag * jnp.cos(zi), mag * jnp.sin(zi)
    den = lre * lre + lim * lim
    nr, ni = lr - 1.0, li
    cr = 2.0 * (nr * lre + ni * lim) / den
    ci = 2.0 * (ni * lre - nr * lim) / den
    lane1 = lax.broadcasted_iota(jnp.int32, (8, 128), 1)
    sub = lax.broadcasted_iota(jnp.int32, (8, 128), 0)
    lo = lane1 < 64

    def tiles(r, i):
        r3, i3 = r[:, 384:], i[:, 384:]
        rr = jnp.where(lo, r3, pltpu.roll(r3, 64, 1))
        ii = jnp.where(lo, -i3, pltpu.roll(i3, 64, 1))
        return ([r[:, 128 * k:128 * k + 128] for k in range(3)] + [rr],
                [i[:, 128 * k:128 * k + 128] for k in range(3)] + [ii])
    lam = tiles(lr, li)
    sq = [(lr, li)]
    for _ in range(5):
        sq.append(_cmul(*sq[-1], *sq[-1]))
    pws = []
    for base in (_cmul(*_cmul(*sq[4], *sq[3]), *sq[2]), _cmul(*sq[5], *sq[2])):
        pw = []
        for _ in range(3):
            pw.append(tiles(*base))
            base = _cmul(*base, *base)
        pws.append(pw)
    dsk = pltpu.roll(jnp.broadcast_to(prm[3:4, :], (8, 512)), 64, 1)

    def cstep(m, k, a, b):
        if k < 3:
            return m[0][k] * a - m[1][k] * b, m[0][k] * b + m[1][k] * a
        return m[0][k] * a + m[1][k] * b, m[0][k] * b - m[1][k] * a

    pend = []
    z0 = pl.program_id(0)

    def push(*cs):
        start(*cs)
        obuf[4, 0:8, :] = dsk[:, 128:256]
        pend.append([PD, obuf[4, pl.ds(pl.multiple_of(z0 * 8, 8), 8), :]])

    def gate(rhs, t=None):
        if pend and t is None:
            pend[0][0] -= 1
            if pend[0][0] == 0:
                t = pend.pop(0)[1]
        if t is not None:
            parts = []
            for r in range(0, rhs.shape[0], 128):
                last = rhs[r + 120:r + 128]
                last = jnp.concatenate([jnp.where(never, t, last[:, c:c + 128])
                                        for c in range(0, rhs.shape[1], 128)], axis=1)
                parts += [rhs[r:r + 120], last]
            rhs = jnp.concatenate(parts, axis=0)
        return rhs

    def prep_b(i):
        for r in range(0, D, 64):
            v = jnp.concatenate([jnp.zeros((64, 64), F32), bv[i, r:r + 64, :].astype(F32)], axis=1)
            r2 = 384 * i + r if r < 384 else 768 + 64 * i
            bcat[r2:r2 + 64, :] = v

    ctok = []

    def prep_c():
        toks = []
        nci = -ci[0:1, :D]
        for r in range(0, D, 32):
            c_re = cv[0, r:r + 32, :].astype(F32)
            c_im = cv[1, r:r + 32, :].astype(F32)
            c2r = c_re * cr[0:1, :D] - c_im * ci[0:1, :D]
            c2i = c_re * nci - c_im * cr[0:1, :D]
            ccat[r:r + 32, 0:384] = c2r[:, 0:384]
            ccat[r:r + 32, 384:768] = c2i[:, 0:384]
            c3 = jnp.concatenate([c2r[:, 384:448], c2i[:, 384:448]], axis=1)
            ccat[r:r + 32, 768:896] = c3
            toks += [v[i:i + 8, c:c + 128] for v in (c2r[:, 0:384], c2i[:, 0:384], c3)
                     for i in range(0, 32, 8) for c in range(0, v.shape[1], 128)]
        ctok.append(functools.reduce(jnp.maximum, toks))

    def ssm_t(c):
        for k in range(4):
            if k == 0:
                xt = jnp.concatenate([jnp.zeros((64, T), F32), bxv[c, 0:64, :].astype(F32)], axis=0)
            else:
                xt = bxv[c, 128 * k - 64:128 * k + 64, :].astype(F32)
            xb32[c // 2][k, T * (c % 2):T * (c % 2) + T, :] = xt.T

    def xs(c, k, j):
        return xb32[c // 2][k, pl.ds(_row0(c) % 512 + j, 8, stride=SEGS[c % 2]), :]

    U, Hs = {}, {}

    def ssm_in(c, ns=range(7)):
        for n in ns:
            xl = jnp.concatenate([jnp.concatenate([xs(c, k, j) for k in range(4)], axis=1)
                                  for j in range(SEGS[c % 2])], axis=0)
            U[c, n] = _dot(xl, gate(bcat[128 * n:128 * n + 128, :], ctok[0] if c == 3 else None), NT)

    carry = [(jnp.zeros((8, 128), F32),) * 2] * 4

    def ssm_scan(c):
        SEG, pw = SEGS[c % 2], pws[c % 2]
        sw = pltpu.roll(U[c, 6], 64, 1)

        def u(j, k):
            if k < 3:
                return U[c, k][8 * j:8 * j + 8], U[c, k + 3][8 * j:8 * j + 8]
            return U[c, 6][8 * j:8 * j + 8], sw[8 * j:8 * j + 8]
        h, hs, dep = [None] * 4, {}, None
        for ks in KG:
            for k in ks:
                h[k] = u(0, k)
                if dep is not None:
                    h[k] = tuple(jnp.where(never, dep, v) for v in h[k])
            for j in range(1, SEG):
                for k in ks:
                    a, b = cstep(lam, k, *h[k])
                    ua, ub = u(j, k)
                    h[k] = (a + ua, b + ub)
            for k in ks:
                z = [jnp.where(sub == 0, carry[k][i], pltpu.roll(h[k][i], 1, 0)) for i in range(2)]
                for n in range(3):
                    sh = 1 << n
                    a, b = cstep(pw[n], k, *[jnp.where(sub >= sh, pltpu.roll(v, sh, 0), 0.0) for v in z])
                    z = [z[0] + a, z[1] + b]
                h[k] = tuple(z)
            for j in range(SEG):
                for k in ks:
                    a, b = cstep(lam, k, *h[k])
                    ua, ub = u(j, k)
                    h[k] = hs[j, k] = (a + ua, b + ub)
                if j == SEG * DJ // 8 - 1:
                    dep = h[ks[-1]][0]
        Hs[c] = [jnp.concatenate([hs[j, 0][0], hs[j, 1][0], hs[j, 2][0], hs[j, 0][1], hs[j, 1][1], hs[j, 2][1],
                                  hs[j, 3][0]], axis=1) for j in range(SEG)]
        carry[:] = [tuple(jnp.broadcast_to(v[7:8], (8, 128)) for v in h[k]) for k in range(4)]

    def ssm_out(p, ts=range(4), between=lambda: None):
        cj = [(2 * p + i, j) for i in range(2) for j in range(SEGS[i])]
        yts = [_dot(ccat[...], gate(jnp.concatenate([Hs[c][j] for c, j in cj[16 * t:16 * t + 16]], axis=0)), NT)
               for t in ts]
        between()
        for t, yt in zip(ts, yts):
            blk = cj[16 * t:16 * t + 16]
            y_post(p, blk, jnp.concatenate([jnp.zeros((64, 128), F32), yt], axis=0), range(4))

    def y_post(p, blk, yt, ks):
        for n, k in enumerate(ks):
            y = yt[128 * n:128 * n + 128].T
            for i, (c, j) in enumerate(blk):
                rows = pl.ds(_row0(c) + j, 8, stride=SEGS[c % 2])
                v = y[8 * i:8 * i + 8] + xs(c, k, j) * dsk[:, 128 * k:128 * k + 128]
                if k == 0 and p >= NPRE:
                    v = jnp.where(lo, a3[rows, :], v)
                obuf[k, rows, :] = v

    def ssm_last(p):
        cj = [(2 * p + i, j) for i in range(2) for j in range(SEGS[i])]
        for ks, ts, cs in PIECES:
            hh = jnp.concatenate([Hs[c][j] for c, j in cj[16 * ts[0]:16 * ts[-1] + 16]], axis=0)
            yt = _dot(ccat[max(128 * ks[0] - 64, 0):128 * ks[-1] + 64, :], gate(hh), NT)
            if ks[0] == 0:
                yt = jnp.concatenate([jnp.zeros((64, yt.shape[1]), F32), yt], axis=0)
            for n, t in enumerate(ts):
                y_post(p, cj[16 * t:16 * t + 16], yt[:, 128 * n:128 * n + 128], ks)
            start(*[o_b[2 * p + c][k] for c in cs for k in ks])

    def w_t(c0, c1):
        for k in range(4):
            n = min(128, D - 128 * k)
            blk = wv[128 * k:128 * k + n, c0:c1].astype(F32)
            if n < 128:
                blk = jnp.concatenate([blk, jnp.zeros((128 - n, c1 - c0), F32)], axis=0)
            wt32[k, c0:c1, :] = blk.T

    def w_rows(g):
        return jnp.concatenate(
            [jnp.concatenate([wt32[k, pl.ds(g * D + hh * 224 + d, 8, stride=DH), :] for k in range(4)], axis=1)
             for d in range(DH) for hh in range(2)], axis=0)

    def w_perm(g):
        for d in range(DH):
            v = [jnp.concatenate([wt32[k, pl.ds(g * D + hh * 224 + d, 8, stride=DH), :]
                                  for k in range(4)], axis=1) for hh in range(2)]
            wtp[g * D + 16 * d:g * D + 16 * d + 16, :] = jnp.concatenate(v, axis=0)

    def x_t():
        for k in range(4):
            n = min(128, D - 128 * k)
            for t in range(4):
                blk = axv[128 * k:128 * k + n, 512 * t:512 * t + 512].astype(F32)
                if n < 128:
                    blk = jnp.concatenate([blk, jnp.zeros((128 - n, 512), F32)], axis=0)
                bt = blk.T
                for g in range(32):
                    r = XP * (32 * t + g)
                    xa32[k, r:r + 16, :] = bt[16 * g:16 * g + 16]

    def wo_prep():
        wo = jnp.concatenate([wov[...].astype(F32), jnp.zeros((D, 64), F32)], axis=1)
        for k in range(4):
            wo32[k] = wo[:, 128 * k:128 * k + 128]
        for k in range(4):
            v = [wo32[k, pl.ds(hh * 224 + d, 8, stride=DH), :] for d in range(DH) for hh in range(2)]
            v = jnp.concatenate(v + [jnp.zeros((64, 128), F32)], axis=0).T
            n = min(128, D - 128 * k)
            wot[128 * k:128 * k + n, :] = v[:n]

    def xa(j):
        return jnp.concatenate([xa32[k, pl.ds(j, 128, stride=XP), :] for k in range(4)], axis=1)

    KV, Q, O = ({}, {}), {}, {}

    def att_kv(j):
        for g in (0, 1):
            r = _dot(w_rows(g + 1), gate(xa(j)), NT)
            KV[g][j + 14] = r
            if j >= 2 and j != NJ - 2:
                KV[g][j - 2] = pltpu.roll(r, 1, 1)

    def att_q(jp):
        for j in JP[jp]:
            Q[j] = _dot(w_rows(0), gate(xa(j)), NT)

    scale = DH ** -0.5

    PP = {}

    def att_l(jp):
        js = JP[jp]
        es = range(js[0], js[1] + 15, 2)
        P = {}
        for hh in range(2):
            lg = {}
            for d in range(DH):
                r = slice(16 * d + 8 * hh, 16 * d + 8 * hh + 8)
                for j in js:
                    for w in range(W):
                        t = Q[j][r] * KV[0][j + 14 - 2 * w][r]
                        lg[j, w] = t if d == 0 else lg[j, w] + t
            for j in js:
                l = [lg[j, w] * scale for w in range(W)]
                l = [jnp.where(lane1 == 0, -1e9, l[w]) if j < 2 * w else l[w] for w in range(W)]
                m = l[0]
                for w in range(1, W):
                    m = jnp.maximum(m, l[w])
                e = [jnp.exp(x - m) for x in l]
                ssum = e[0]
                for w in range(1, W):
                    ssum = ssum + e[w]
                inv = 1.0 / ssum
                P[hh, j] = [x * inv for x in e]
        PP[jp] = P

    def att_v(jp):
        js, P = JP[jp], PP[jp]
        for j in js:
            O[j] = [None] * (2 * DH)
        dep = None
        for hh, jj in [(h, js) for h in range(2)]:
            if dep is not None:
                for j in jj:
                    P[hh, j] = [jnp.where(never, dep, x) for x in P[hh, j]]
            for d in range(DH):
                r = slice(16 * d + 8 * hh, 16 * d + 8 * hh + 8)
                for j in jj:
                    acc = None
                    for w in range(W):
                        t = P[hh, j][w] * KV[1][j + 14 - 2 * w][r]
                        acc = t if acc is None else acc + t
                    O[j][2 * d + hh] = acc
                    if d == DH - 1:
                        dep = acc

    def att_o(jp):
        rhs = jnp.concatenate([jnp.concatenate(O[j] + [jnp.zeros((64, 128), F32)], axis=0) for j in JP[jp]], axis=1)
        res = _dot(wot[...], gate(rhs), NN)
        for i, j in enumerate(JP[jp]):
            rt = jnp.concatenate([res[:, 128 * i:128 * i + 128], jnp.zeros((64, 128), F32)], axis=0)
            for k in range(4):
                ost[j % 2][k, pl.ds(OP * (j // 2), 128), :] = rt[128 * k:128 * k + 128].T

    def o_rows(par, k, s):
        return ost[par][k, pl.ds(s, 8, stride=OP), :]

    def o_unperm(par):
        for k in range(3):
            for s in range(128):
                oa[k, pl.ds(NJ * s + par, 8, stride=2), :] = o_rows(par, k, s)

    def o_mixed():
        for s in range(128):
            for par in range(2):
                rows = pl.ds(NJ * s + par, 8, stride=2)
                if NJ * s < 512 * NPRE:
                    obuf[0, rows, :] = jnp.where(lo, o_rows(par, 3, s), obuf[0, rows, :])
                else:
                    a3[rows, :] = o_rows(par, 3, s)

    o_a = [pltpu.make_async_copy(oa.at[k], out_h.at[:, pl.ds(128 * k, 128)], osem) for k in range(3)]
    o_b = [[pltpu.make_async_copy(obuf.at[k, pl.ds(_row0(c), 8 * SEGS[c % 2])],
                                  out_h.at[pl.ds(_row0(c), 8 * SEGS[c % 2]), pl.ds(128 * (k + 3), 128)],
                                  osem) for k in range(4)] for c in range(NC)]

    NPRE = 2
    wait(c_bx[0], c_b[0])
    start(c_bx[1], c_bx[2], c_bx[3])
    prep_b(0)
    ssm_t(0)
    ssm_in(0, range(2))
    wait(c_b[1], c_bx[1])
    start(*c_c)
    prep_b(1)
    ssm_t(1)
    ssm_in(0, range(2, 7))
    ssm_in(1, range(2))
    wait(c_bx[2], c_bx[3])
    start(c_w, c_ax)
    ssm_in(1, range(2, 7))
    ssm_scan(0)
    ssm_t(2)
    ssm_t(3)
    ssm_in(2, range(2))
    wait(*c_c)
    prep_c()
    ssm_in(2, range(2, 7))
    ssm_in(3, range(2))
    ssm_scan(1)
    ssm_in(3, range(2, 7))
    cj0 = [(i, j) for i in range(2) for j in range(SEGS[i])]
    h0 = [jnp.concatenate([Hs[c][j] for c, j in cj0[16 * t:16 * t + 16]], axis=0) for t in range(2)]
    y0 = _dot(ccat[...], h0[0], NT)
    y1 = _dot(ccat[:, 0:640], h0[1][:, 0:640], NT)
    y1 = jnp.concatenate([jnp.where(never, 0.0, y1[r:r + 8]) for r in range(0, D, 8)], axis=0)
    wait(c_w, c_ax)
    start(c_wo, *c_bx[4:])
    y1 = y1 + _dot(ccat[:, 640:], h0[1][:, 640:], NT)
    for t, y in enumerate((y0, y1)):
        y_post(0, cj0[16 * t:16 * t + 16], jnp.concatenate([jnp.zeros((64, 128), F32), y], axis=0), range(4))
    w_t(384, 3 * D)
    x_t()
    ssm_out(0, range(2, 4))
    ssm_scan(2)
    for j in range(0, NJ, 2):
        att_kv(j)
    ssm_scan(3)
    w_t(0, 384)
    start(*o_b[0][1:], *o_b[1][1:])
    wait(c_wo, *c_bx[4:6])
    for g in range(2):
        KV[g][NJ - 4] = pltpu.roll(KV[g][NJ + 12], 1, 1)
    wo_prep()
    att_q(0)
    for i in range(4):
        att_kv(4 * i + 1)
        att_q(i + 1)
        att_l(i)
        att_v(i)
        att_kv(4 * i + 3)
        if i >= LO:
            att_o(i - LO)
    ssm_t(4)
    ssm_t(5)
    for i in range(4, 8):
        if i < 7:
            att_q(i + 1)
        ssm_out(1, [i - 4])
        if i in (5, 7):
            push(*o_b[i // 2][1:])
        att_l(i)
        att_v(i)
        att_o(i - LO)
        if i - LO == 3:
            o_unperm(0)
    for i in range(8 - LO, 8):
        att_o(i)
    ssm_in(4, range(4))
    o_unperm(1)
    o_mixed()
    start(*o_a, o_b[0][0], o_b[1][0], o_b[2][0], o_b[3][0])
    wait(*c_bx[6:])
    ssm_t(6)
    ssm_t(7)
    ssm_in(4, range(4, 7))
    ssm_in(5)
    ssm_scan(4)
    ssm_in(6)
    ssm_scan(5)
    ssm_out(2, range(2))
    push(*o_b[4])
    ssm_in(7)
    ssm_out(2, range(2, 3))
    ssm_scan(6)
    ssm_out(2, range(3, 4))
    push(*o_b[5])
    ssm_scan(7)
    ssm_last(3)
    pltpu.make_async_copy(out_h, out_h, osem).wait()


@jax.jit
def pallas_concat_heads__sliding_local_dilated__ssm_conv_s5__prompt_kernel(
    A_x, A_wqkv, A_wo, B_x, B_Lambda_re, B_Lambda_im, B_B_re, B_B_im, B_C_re, B_C_im,
    B_log_dt, B_Dskip,
):
    hbm = pl.BlockSpec(memory_space=pltpu.HBM)
    out = pl.pallas_call(
        _kernel,
        out_shape=jax.ShapeDtypeStruct((S, 2 * D), F32),
        grid=(1,),
        in_specs=[hbm] * 12,
        out_specs=hbm,
        scratch_shapes=[
            pltpu.VMEM((D, S), BF16),
            pltpu.VMEM((D, 3 * D), BF16),
            pltpu.VMEM((D, D), BF16),
            pltpu.VMEM((NC, D, T), BF16),
            pltpu.VMEM((2, D, D), BF16),
            pltpu.VMEM((2, D, D), BF16),
            *[pltpu.VMEM((D,), BF16)] * 4,
            pltpu.VMEM((8, 512), F32),
            pltpu.VMEM((896, 512), F32),
            pltpu.VMEM((D, 896), F32),
            *[pltpu.VMEM((4, 512, 128), F32)] * 4,
            pltpu.VMEM((4, 3 * D, 128), F32),
            pltpu.VMEM((3 * D, 512), F32),
            pltpu.VMEM((4, D, 128), F32),
            pltpu.VMEM((D, 512), F32),
            pltpu.VMEM((4, 128 * XP, 128), F32),
            pltpu.VMEM((5, S, 128), F32),
            pltpu.VMEM((S, 128), F32),
            pltpu.VMEM((3, S, 128), F32),
            *[pltpu.VMEM((4, 8 * OP, 128), F32)] * 2,
            pltpu.SemaphoreType.DMA((11 + NC,)),
            pltpu.SemaphoreType.DMA(()),
        ],
        compiler_params=pltpu.CompilerParams(vmem_limit_bytes=100 * 1024 * 1024),
    )(A_x[0].T, A_wqkv, A_wo, B_x[0].T, B_Lambda_re, B_Lambda_im,
      B_B_re, B_B_im, B_C_re, B_C_im, B_log_dt, B_Dskip)
    return out.reshape(1, S, 2 * D)
```

```python
import functools

import jax
import jax.numpy as jnp
from jax import lax
import jax.experimental.pallas as pl
import jax.experimental.pallas.tpu as pltpu

S, D, H, DH, W = 2048, 448, 16, 28, 8
NJ = 16
T = 256
NC = S // T
SEGS = (28, 36)
XP = 20
KG, DJ = ((0,), (1,), (2,), (3,)), 8
OP = 132
PIECES = (((0, 1), (0, 1, 2, 3), (0, 1)), ((2,), (0, 1, 2, 3), (0, 1)), ((3,), (0, 1), (0,)), ((3,), (2, 3), (1,)))
LO = 2
PD = 4
F32, BF16 = jnp.float32, jnp.bfloat16
NN = (((1,), (0,)), ((), ()))
NT = (((1,), (1,)), ((), ()))
JP = [(0, 2), (4, 6), (8, 10), (12, 14), (1, 3), (5, 7), (9, 11), (13, 15)]


_dot = functools.partial(lax.dot_general, preferred_element_type=F32)


def _row0(c):
    return 512 * (c // 2) + 8 * SEGS[0] * (c % 2)


def _cmul(ar, ai, br, bi):
    return ar * br - ai * bi, ar * bi + ai * br


def _kernel(ax_h, wqkv_h, wo_h, bx_h, lre_h, lim_h, bre_h, bim_h, cre_h, cim_h, ldt_h, dsk_h,
            out_h,
            axv, wv, wov, bxv, bv, cv, pv0, pv1, pv2, pv3, prm, bcat, ccat, xb0, xb1, xb2, xb3,
            wt32, wtp, wo32, wot, xa32, obuf, a3, oa, ost0, ost1, isem, osem):
    ost = (ost0, ost1)
    xb32 = (xb0, xb1, xb2, xb3)

    def cp(i, src, dst):
        return pltpu.make_async_copy(src, dst, isem.at[i])
    c_par = [cp(0, lre_h, pv0), cp(1, lim_h, pv1), cp(2, ldt_h, pv2), cp(3, dsk_h, pv3)]
    c_b = [cp(4, bre_h, bv.at[0]), cp(5, bim_h, bv.at[1])]
    c_c = [cp(6, cre_h, cv.at[0]), cp(7, cim_h, cv.at[1])]
    c_bx = [cp(8 + c, bx_h.at[:, pl.ds(c * T, T)], bxv.at[c]) for c in range(NC)]
    c_w, c_ax, c_wo = cp(8 + NC, wqkv_h, wv), cp(9 + NC, ax_h, axv), cp(10 + NC, wo_h, wov)

    def start(*cs):
        for c in cs:
            c.start()

    def wait(*cs):
        for c in cs:
            c.wait()
    start(*c_par, c_bx[0], c_b[0], c_b[1])

    wait(*c_par)
    prm[...] = jnp.zeros(prm.shape, F32)
    for i in range(4):
        prm[i:i + 1, 0:D] = (pv0, pv1, pv2, pv3)[i][...].astype(F32).reshape(1, D)
    lane5 = lax.broadcasted_iota(jnp.int32, (8, 512), 1)
    lre = jnp.where(lane5 < D, jnp.broadcast_to(prm[0:1, :], (8, 512)), -1.0)
    lim = jnp.broadcast_to(prm[1:2, :], (8, 512))
    dt = jnp.exp(jnp.broadcast_to(prm[2:3, :], (8, 512))).astype(BF16).astype(F32)
    never = dt[:, 0:128] < 0.0
    zr, zi = dt * lre, dt * lim
    mag = jnp.exp(zr)
    lr, li = mag * jnp.cos(zi), mag * jnp.sin(zi)
    den = lre * lre + lim * lim
    nr, ni = lr - 1.0, li
    cr = 2.0 * (nr * lre + ni * lim) / den
    ci = 2.0 * (ni * lre - nr * lim) / den
    lane1 = lax.broadcasted_iota(jnp.int32, (8, 128), 1)
    sub = lax.broadcasted_iota(jnp.int32, (8, 128), 0)
    lo = lane1 < 64

    def tiles(r, i):
        r3, i3 = r[:, 384:], i[:, 384:]
        rr = jnp.where(lo, r3, pltpu.roll(r3, 64, 1))
        ii = jnp.where(lo, -i3, pltpu.roll(i3, 64, 1))
        return ([r[:, 128 * k:128 * k + 128] for k in range(3)] + [rr],
                [i[:, 128 * k:128 * k + 128] for k in range(3)] + [ii])
    lam = tiles(lr, li)
    sq = [(lr, li)]
    for _ in range(5):
        sq.append(_cmul(*sq[-1], *sq[-1]))
    pws = []
    for base in (_cmul(*_cmul(*sq[4], *sq[3]), *sq[2]), _cmul(*sq[5], *sq[2])):
        pw = []
        for _ in range(3):
            pw.append(tiles(*base))
            base = _cmul(*base, *base)
        pws.append(pw)
    dsk = pltpu.roll(jnp.broadcast_to(prm[3:4, :], (8, 512)), 64, 1)

    def cstep(m, k, a, b):
        if k < 3:
            return m[0][k] * a - m[1][k] * b, m[0][k] * b + m[1][k] * a
        return m[0][k] * a + m[1][k] * b, m[0][k] * b - m[1][k] * a

    pend = []
    z0 = pl.program_id(0)

    def push(*cs):
        start(*cs)
        obuf[4, 0:8, :] = dsk[:, 128:256]
        pend.append([PD, obuf[4, pl.ds(pl.multiple_of(z0 * 8, 8), 8), :]])

    def gate(rhs, t=None):
        if pend and t is None:
            pend[0][0] -= 1
            if pend[0][0] == 0:
                t = pend.pop(0)[1]
        if t is not None:
            parts = []
            for r in range(0, rhs.shape[0], 128):
                last = rhs[r + 120:r + 128]
                last = jnp.concatenate([jnp.where(never, t, last[:, c:c + 128])
                                        for c in range(0, rhs.shape[1], 128)], axis=1)
                parts += [rhs[r:r + 120], last]
            rhs = jnp.concatenate(parts, axis=0)
        return rhs

    def prep_b(i):
        for r in range(0, D, 64):
            v = jnp.concatenate([jnp.zeros((64, 64), F32), bv[i, r:r + 64, :].astype(F32)], axis=1)
            r2 = 384 * i + r if r < 384 else 768 + 64 * i
            bcat[r2:r2 + 64, :] = v

    ctok = []

    def prep_c():
        toks = []
        nci = -ci[0:1, :D]
        for r in range(0, D, 32):
            c_re = cv[0, r:r + 32, :].astype(F32)
            c_im = cv[1, r:r + 32, :].astype(F32)
            c2r = c_re * cr[0:1, :D] - c_im * ci[0:1, :D]
            c2i = c_re * nci - c_im * cr[0:1, :D]
            ccat[r:r + 32, 0:384] = c2r[:, 0:384]
            ccat[r:r + 32, 384:768] = c2i[:, 0:384]
            c3 = jnp.concatenate([c2r[:, 384:448], c2i[:, 384:448]], axis=1)
            ccat[r:r + 32, 768:896] = c3
            toks += [v[i:i + 8, c:c + 128] for v in (c2r[:, 0:384], c2i[:, 0:384], c3)
                     for i in range(0, 32, 8) for c in range(0, v.shape[1], 128)]
        ctok.append(functools.reduce(jnp.maximum, toks))

    def ssm_t(c):
        for k in range(4):
            if k == 0:
                xt = jnp.concatenate([jnp.zeros((64, T), F32), bxv[c, 0:64, :].astype(F32)], axis=0)
            else:
                xt = bxv[c, 128 * k - 64:128 * k + 64, :].astype(F32)
            xb32[c // 2][k, T * (c % 2):T * (c % 2) + T, :] = xt.T

    def xs(c, k, j):
        return xb32[c // 2][k, pl.ds(_row0(c) % 512 + j, 8, stride=SEGS[c % 2]), :]

    U, Hs = {}, {}

    def ssm_in(c, ns=range(7)):
        for n in ns:
            xl = jnp.concatenate([jnp.concatenate([xs(c, k, j) for k in range(4)], axis=1)
                                  for j in range(SEGS[c % 2])], axis=0)
            U[c, n] = _dot(xl, gate(bcat[128 * n:128 * n + 128, :], ctok[0] if c == 3 else None), NT)

    carry = [(jnp.zeros((8, 128), F32),) * 2] * 4

    def ssm_scan(c):
        SEG, pw = SEGS[c % 2], pws[c % 2]
        sw = pltpu.roll(U[c, 6], 64, 1)

        def u(j, k):
            if k < 3:
                return U[c, k][8 * j:8 * j + 8], U[c, k + 3][8 * j:8 * j + 8]
            return U[c, 6][8 * j:8 * j + 8], sw[8 * j:8 * j + 8]
        h, hs, dep = [None] * 4, {}, None
        for ks in KG:
            for k in ks:
                h[k] = u(0, k)
                if dep is not None:
                    h[k] = tuple(jnp.where(never, dep, v) for v in h[k])
            for j in range(1, SEG):
                for k in ks:
                    a, b = cstep(lam, k, *h[k])
                    ua, ub = u(j, k)
                    h[k] = (a + ua, b + ub)
            for k in ks:
                z = [jnp.where(sub == 0, carry[k][i], pltpu.roll(h[k][i], 1, 0)) for i in range(2)]
                for n in range(3):
                    sh = 1 << n
                    a, b = cstep(pw[n], k, *[jnp.where(sub >= sh, pltpu.roll(v, sh, 0), 0.0) for v in z])
                    z = [z[0] + a, z[1] + b]
                h[k] = tuple(z)
            for j in range(SEG):
                for k in ks:
                    a, b = cstep(lam, k, *h[k])
                    ua, ub = u(j, k)
                    h[k] = hs[j, k] = (a + ua, b + ub)
                if j == SEG * DJ // 8 - 1:
                    dep = h[ks[-1]][0]
        Hs[c] = [jnp.concatenate([hs[j, 0][0], hs[j, 1][0], hs[j, 2][0], hs[j, 0][1], hs[j, 1][1], hs[j, 2][1],
                                  hs[j, 3][0]], axis=1) for j in range(SEG)]
        carry[:] = [tuple(jnp.broadcast_to(v[7:8], (8, 128)) for v in h[k]) for k in range(4)]

    def ssm_out(p, ts=range(4), between=lambda: None):
        cj = [(2 * p + i, j) for i in range(2) for j in range(SEGS[i])]
        yts = [_dot(ccat[...], gate(jnp.concatenate([Hs[c][j] for c, j in cj[16 * t:16 * t + 16]], axis=0)), NT)
               for t in ts]
        between()
        for t, yt in zip(ts, yts):
            blk = cj[16 * t:16 * t + 16]
            y_post(p, blk, jnp.concatenate([jnp.zeros((64, 128), F32), yt], axis=0), range(4))

    def y_post(p, blk, yt, ks):
        for n, k in enumerate(ks):
            y = yt[128 * n:128 * n + 128].T
            for i, (c, j) in enumerate(blk):
                rows = pl.ds(_row0(c) + j, 8, stride=SEGS[c % 2])
                v = y[8 * i:8 * i + 8] + xs(c, k, j) * dsk[:, 128 * k:128 * k + 128]
                if k == 0 and p >= NPRE:
                    v = jnp.where(lo, a3[rows, :], v)
                obuf[k, rows, :] = v

    def ssm_last(p):
        cj = [(2 * p + i, j) for i in range(2) for j in range(SEGS[i])]
        for ks, ts, cs in PIECES:
            hh = jnp.concatenate([Hs[c][j] for c, j in cj[16 * ts[0]:16 * ts[-1] + 16]], axis=0)
            yt = _dot(ccat[max(128 * ks[0] - 64, 0):128 * ks[-1] + 64, :], gate(hh), NT)
            if ks[0] == 0:
                yt = jnp.concatenate([jnp.zeros((64, yt.shape[1]), F32), yt], axis=0)
            for n, t in enumerate(ts):
                y_post(p, cj[16 * t:16 * t + 16], yt[:, 128 * n:128 * n + 128], ks)
            start(*[o_b[2 * p + c][k] for c in cs for k in ks])

    def w_t(c0, c1):
        for k in range(4):
            n = min(128, D - 128 * k)
            blk = wv[128 * k:128 * k + n, c0:c1].astype(F32)
            if n < 128:
                blk = jnp.concatenate([blk, jnp.zeros((128 - n, c1 - c0), F32)], axis=0)
            wt32[k, c0:c1, :] = blk.T

    def w_rows(g):
        return jnp.concatenate(
            [jnp.concatenate([wt32[k, pl.ds(g * D + hh * 224 + d, 8, stride=DH), :] for k in range(4)], axis=1)
             for d in range(DH) for hh in range(2)], axis=0)

    def w_perm(g):
        for d in range(DH):
            v = [jnp.concatenate([wt32[k, pl.ds(g * D + hh * 224 + d, 8, stride=DH), :]
                                  for k in range(4)], axis=1) for hh in range(2)]
            wtp[g * D + 16 * d:g * D + 16 * d + 16, :] = jnp.concatenate(v, axis=0)

    def x_t():
        for k in range(4):
            n = min(128, D - 128 * k)
            for t in range(4):
                blk = axv[128 * k:128 * k + n, 512 * t:512 * t + 512].astype(F32)
                if n < 128:
                    blk = jnp.concatenate([blk, jnp.zeros((128 - n, 512), F32)], axis=0)
                bt = blk.T
                for g in range(32):
                    r = XP * (32 * t + g)
                    xa32[k, r:r + 16, :] = bt[16 * g:16 * g + 16]

    def wo_prep():
        wo = jnp.concatenate([wov[...].astype(F32), jnp.zeros((D, 64), F32)], axis=1)
        for k in range(4):
            wo32[k] = wo[:, 128 * k:128 * k + 128]
        for k in range(4):
            v = [wo32[k, pl.ds(hh * 224 + d, 8, stride=DH), :] for d in range(DH) for hh in range(2)]
            v = jnp.concatenate(v + [jnp.zeros((64, 128), F32)], axis=0).T
            n = min(128, D - 128 * k)
            wot[128 * k:128 * k + n, :] = v[:n]

    def xa(j):
        return jnp.concatenate([xa32[k, pl.ds(j, 128, stride=XP), :] for k in range(4)], axis=1)

    KV, Q, O = ({}, {}), {}, {}

    def att_kv(j, gs=(0, 1)):
        for g in gs:
            r = _dot(w_rows(g + 1), gate(xa(j)), NT)
            KV[g][j + 14] = r
            if j >= 2 and j != NJ - 2:
                KV[g][j - 2] = pltpu.roll(r, 1, 1)

    def att_q(*js):
        for j in js:
            Q[j] = _dot(w_rows(0), gate(xa(j)), NT)

    scale = DH ** -0.5

    PP = {}

    def att_l(jp):
        js = JP[jp]
        es = range(js[0], js[1] + 15, 2)
        P = {}
        for hh in range(2):
            lg = {}
            for d in range(DH):
                r = slice(16 * d + 8 * hh, 16 * d + 8 * hh + 8)
                for j in js:
                    for w in range(W):
                        t = Q[j][r] * KV[0][j + 14 - 2 * w][r]
                        lg[j, w] = t if d == 0 else lg[j, w] + t
            for j in js:
                l = [lg[j, w] * scale for w in range(W)]
                l = [jnp.where(lane1 == 0, -1e9, l[w]) if j < 2 * w else l[w] for w in range(W)]
                m = l[0]
                for w in range(1, W):
                    m = jnp.maximum(m, l[w])
                e = [jnp.exp(x - m) for x in l]
                ssum = e[0]
                for w in range(1, W):
                    ssum = ssum + e[w]
                inv = 1.0 / ssum
                P[hh, j] = [x * inv for x in e]
        PP[jp] = P

    def att_v(jp):
        js, P = JP[jp], PP[jp]
        for j in js:
            O[j] = [None] * (2 * DH)
        dep = None
        for hh, jj in [(h, js) for h in range(2)]:
            if dep is not None:
                for j in jj:
                    P[hh, j] = [jnp.where(never, dep, x) for x in P[hh, j]]
            for d in range(DH):
                r = slice(16 * d + 8 * hh, 16 * d + 8 * hh + 8)
                for j in jj:
                    acc = None
                    for w in range(W):
                        t = P[hh, j][w] * KV[1][j + 14 - 2 * w][r]
                        acc = t if acc is None else acc + t
                    O[j][2 * d + hh] = acc
                    if d == DH - 1:
                        dep = acc

    def att_o(jp):
        rhs = jnp.concatenate([jnp.concatenate(O[j] + [jnp.zeros((64, 128), F32)], axis=0) for j in JP[jp]], axis=1)
        res = _dot(wot[...], gate(rhs), NN)
        for i, j in enumerate(JP[jp]):
            rt = jnp.concatenate([res[:, 128 * i:128 * i + 128], jnp.zeros((64, 128), F32)], axis=0)
            for k in range(4):
                ost[j % 2][k, pl.ds(OP * (j // 2), 128), :] = rt[128 * k:128 * k + 128].T

    def o_rows(par, k, s):
        return ost[par][k, pl.ds(s, 8, stride=OP), :]

    def o_unperm(par):
        for k in range(3):
            for s in range(128):
                oa[k, pl.ds(NJ * s + par, 8, stride=2), :] = o_rows(par, k, s)

    def o_mixed():
        for s in range(128):
            for par in range(2):
                rows = pl.ds(NJ * s + par, 8, stride=2)
                if NJ * s < 512 * NPRE:
                    obuf[0, rows, :] = jnp.where(lo, o_rows(par, 3, s), obuf[0, rows, :])
                else:
                    a3[rows, :] = o_rows(par, 3, s)

    o_a = [pltpu.make_async_copy(oa.at[k], out_h.at[:, pl.ds(128 * k, 128)], osem) for k in range(3)]
    o_b = [[pltpu.make_async_copy(obuf.at[k, pl.ds(_row0(c), 8 * SEGS[c % 2])],
                                  out_h.at[pl.ds(_row0(c), 8 * SEGS[c % 2]), pl.ds(128 * (k + 3), 128)],
                                  osem) for k in range(4)] for c in range(NC)]

    NPRE = 2
    wait(c_bx[0], c_b[0])
    start(c_bx[1], c_bx[2], c_bx[3])
    prep_b(0)
    ssm_t(0)
    ssm_in(0, range(2))
    wait(c_b[1], c_bx[1])
    start(*c_c)
    prep_b(1)
    ssm_t(1)
    ssm_in(0, range(2, 7))
    ssm_in(1, range(2))
    wait(c_bx[2], c_bx[3])
    start(c_w, c_ax)
    ssm_in(1, range(2, 7))
    ssm_scan(0)
    ssm_t(2)
    ssm_t(3)
    ssm_in(2, range(2))
    wait(*c_c)
    prep_c()
    ssm_in(2, range(2, 7))
    ssm_in(3, range(2))
    ssm_scan(1)
    ssm_in(3, range(2, 7))
    cj0 = [(i, j) for i in range(2) for j in range(SEGS[i])]
    h0 = [jnp.concatenate([Hs[c][j] for c, j in cj0[16 * t:16 * t + 16]], axis=0) for t in range(2)]
    y0 = _dot(ccat[...], h0[0], NT)
    y1 = _dot(ccat[:, 0:640], h0[1][:, 0:640], NT)
    y1 = jnp.concatenate([jnp.where(never, 0.0, y1[r:r + 8]) for r in range(0, D, 8)], axis=0)
    wait(c_w, c_ax)
    start(c_wo, *c_bx[4:])
    y1 = y1 + _dot(ccat[:, 640:], h0[1][:, 640:], NT)
    for t, y in enumerate((y0, y1)):
        y_post(0, cj0[16 * t:16 * t + 16], jnp.concatenate([jnp.zeros((64, 128), F32), y], axis=0), range(4))
    w_t(384, 3 * D)
    x_t()
    ssm_out(0, range(2, 4))
    ssm_scan(2)
    for j in range(0, NJ, 2):
        att_kv(j)
    ssm_scan(3)
    w_t(0, 384)
    start(*o_b[0][1:], *o_b[1][1:])
    wait(c_wo, *c_bx[4:6])
    for g in range(2):
        KV[g][NJ - 4] = pltpu.roll(KV[g][NJ + 12], 1, 1)
    wo_prep()
    att_kv(1, (1,))
    att_q(0)
    att_q(2)
    att_kv(1, (0,))
    att_q(4)
    att_q(6)
    att_l(0)
    att_v(0)
    att_kv(3, (0,))
    att_kv(3, (1,))
    att_kv(5, (0,))
    att_kv(5, (1,))
    att_q(8)
    att_q(10)
    att_l(1)
    att_v(1)
    att_kv(7, (0,))
    att_kv(7, (1,))
    att_kv(9, (0,))
    att_kv(9, (1,))
    att_q(12)
    att_q(14)
    att_l(2)
    att_v(2)
    att_kv(11, (0,))
    att_kv(11, (1,))
    att_o(0)
    att_kv(13, (0,))
    att_kv(13, (1,))
    att_q(1)
    att_q(3)
    att_l(3)
    att_v(3)
    att_kv(15, (0,))
    att_kv(15, (1,))
    att_o(1)
    ssm_t(4)
    ssm_t(5)
    att_q(5)
    att_q(7)
    ssm_out(1, [0])
    att_l(4)
    att_v(4)
    att_o(2)
    att_q(9)
    att_q(11)
    ssm_out(1, [1])
    push(*o_b[2][1:])
    att_l(5)
    att_v(5)
    att_o(3)
    o_unperm(0)
    att_q(13)
    att_q(15)
    ssm_out(1, [2])
    att_l(6)
    att_v(6)
    att_o(4)
    ssm_out(1, [3])
    push(*o_b[3][1:])
    att_l(7)
    att_v(7)
    att_o(5)
    att_o(6)
    att_o(7)
    ssm_in(4, [0])
    ssm_in(4, [1])
    ssm_in(4, [2])
    ssm_in(4, [3])
    o_unperm(1)
    o_mixed()
    start(*o_a, o_b[0][0], o_b[1][0], o_b[2][0], o_b[3][0])
    wait(*c_bx[6:])
    ssm_t(6)
    ssm_t(7)
    ssm_in(4, range(4, 7))
    ssm_in(5)
    ssm_scan(4)
    ssm_in(6)
    ssm_scan(5)
    ssm_out(2, range(2))
    push(*o_b[4])
    ssm_in(7)
    ssm_out(2, range(2, 3))
    ssm_scan(6)
    ssm_out(2, range(3, 4))
    push(*o_b[5])
    ssm_scan(7)
    ssm_last(3)
    pltpu.make_async_copy(out_h, out_h, osem).wait()


@jax.jit
def pallas_concat_heads__sliding_local_dilated__ssm_conv_s5__prompt_kernel(
    A_x, A_wqkv, A_wo, B_x, B_Lambda_re, B_Lambda_im, B_B_re, B_B_im, B_C_re, B_C_im,
    B_log_dt, B_Dskip,
):
    hbm = pl.BlockSpec(memory_space=pltpu.HBM)
    out = pl.pallas_call(
        _kernel,
        out_shape=jax.ShapeDtypeStruct((S, 2 * D), F32),
        grid=(1,),
        in_specs=[hbm] * 12,
        out_specs=hbm,
        scratch_shapes=[
            pltpu.VMEM((D, S), BF16),
            pltpu.VMEM((D, 3 * D), BF16),
            pltpu.VMEM((D, D), BF16),
            pltpu.VMEM((NC, D, T), BF16),
            pltpu.VMEM((2, D, D), BF16),
            pltpu.VMEM((2, D, D), BF16),
            *[pltpu.VMEM((D,), BF16)] * 4,
            pltpu.VMEM((8, 512), F32),
            pltpu.VMEM((896, 512), F32),
            pltpu.VMEM((D, 896), F32),
            *[pltpu.VMEM((4, 512, 128), F32)] * 4,
            pltpu.VMEM((4, 3 * D, 128), F32),
            pltpu.VMEM((3 * D, 512), F32),
            pltpu.VMEM((4, D, 128), F32),
            pltpu.VMEM((D, 512), F32),
            pltpu.VMEM((4, 128 * XP, 128), F32),
            pltpu.VMEM((5, S, 128), F32),
            pltpu.VMEM((S, 128), F32),
            pltpu.VMEM((3, S, 128), F32),
            *[pltpu.VMEM((4, 8 * OP, 128), F32)] * 2,
            pltpu.SemaphoreType.DMA((11 + NC,)),
            pltpu.SemaphoreType.DMA(()),
        ],
        compiler_params=pltpu.CompilerParams(vmem_limit_bytes=100 * 1024 * 1024),
    )(A_x[0].T, A_wqkv, A_wo, B_x[0].T, B_Lambda_re, B_Lambda_im,
      B_B_re, B_B_im, B_C_re, B_C_im, B_log_dt, B_Dskip)
    return out.reshape(1, S, 2 * D)
```

```python
import functools

import jax
import jax.numpy as jnp
from jax import lax
import jax.experimental.pallas as pl
import jax.experimental.pallas.tpu as pltpu

S, D, H, DH, W = 2048, 448, 16, 28, 8
NJ = 16
T = 256
NC = S // T
SEGS = (28, 36)
XP = 20
KG, DJ = ((0,), (1,), (2,), (3,)), 8
OP = 132
PIECES = (((0, 1), (0, 1, 2, 3), (0, 1)), ((2,), (0, 1, 2, 3), (0, 1)), ((3,), (0, 1), (0,)), ((3,), (2, 3), (1,)))
LO = 2
PD = 4
F32, BF16 = jnp.float32, jnp.bfloat16
NN = (((1,), (0,)), ((), ()))
NT = (((1,), (1,)), ((), ()))
JP = [(0, 2), (4, 6), (8, 10), (12, 14), (1, 3), (5, 7), (9, 11), (13, 15)]


_dot = functools.partial(lax.dot_general, preferred_element_type=F32)


def _row0(c):
    return 512 * (c // 2) + 8 * SEGS[0] * (c % 2)


def _cmul(ar, ai, br, bi):
    return ar * br - ai * bi, ar * bi + ai * br


def _kernel(ax_h, wqkv_h, wo_h, bx_h, lre_h, lim_h, bre_h, bim_h, cre_h, cim_h, ldt_h, dsk_h,
            out_h,
            axv, wv, wov, bxv, bv, cv, pv0, pv1, pv2, pv3, prm, bcat, ccat, xb0, xb1, xb2, xb3,
            wt32, wtp, wo32, wot, xa32, obuf, a3, oa, ost0, ost1, isem, osem):
    ost = (ost0, ost1)
    xb32 = (xb0, xb1, xb2, xb3)

    def cp(i, src, dst):
        return pltpu.make_async_copy(src, dst, isem.at[i])
    c_par = [cp(0, lre_h, pv0), cp(1, lim_h, pv1), cp(2, ldt_h, pv2), cp(3, dsk_h, pv3)]
    c_b = [cp(4, bre_h, bv.at[0]), cp(5, bim_h, bv.at[1])]
    c_c = [cp(6, cre_h, cv.at[0]), cp(7, cim_h, cv.at[1])]
    c_bx = [cp(8 + c, bx_h.at[:, pl.ds(c * T, T)], bxv.at[c]) for c in range(NC)]
    c_w, c_ax, c_wo = cp(8 + NC, wqkv_h, wv), cp(9 + NC, ax_h, axv), cp(10 + NC, wo_h, wov)

    def start(*cs):
        for c in cs:
            c.start()

    def wait(*cs):
        for c in cs:
            c.wait()
    start(*c_par, c_bx[0], c_b[0], c_b[1])

    wait(*c_par, c_bx[0])
    prm[...] = jnp.zeros(prm.shape, F32)
    for i in range(4):
        prm[i:i + 1, 0:D] = (pv0, pv1, pv2, pv3)[i][...].astype(F32).reshape(1, D)
    lane5 = lax.broadcasted_iota(jnp.int32, (8, 512), 1)
    lre = jnp.where(lane5 < D, jnp.broadcast_to(prm[0:1, :], (8, 512)), -1.0)
    lim = jnp.broadcast_to(prm[1:2, :], (8, 512))
    dt = jnp.exp(jnp.broadcast_to(prm[2:3, :], (8, 512))).astype(BF16).astype(F32)
    never = dt[:, 0:128] < 0.0
    zr, zi = dt * lre, dt * lim
    mag = jnp.exp(zr)
    lr, li = mag * jnp.cos(zi), mag * jnp.sin(zi)
    den = lre * lre + lim * lim
    nr, ni = lr - 1.0, li
    cr = 2.0 * (nr * lre + ni * lim) / den
    ci = 2.0 * (ni * lre - nr * lim) / den
    lane1 = lax.broadcasted_iota(jnp.int32, (8, 128), 1)
    sub = lax.broadcasted_iota(jnp.int32, (8, 128), 0)
    lo = lane1 < 64

    def tiles(r, i):
        r3, i3 = r[:, 384:], i[:, 384:]
        rr = jnp.where(lo, r3, pltpu.roll(r3, 64, 1))
        ii = jnp.where(lo, -i3, pltpu.roll(i3, 64, 1))
        return ([r[:, 128 * k:128 * k + 128] for k in range(3)] + [rr],
                [i[:, 128 * k:128 * k + 128] for k in range(3)] + [ii])
    lam = tiles(lr, li)
    sq = [(lr, li)]
    for _ in range(5):
        sq.append(_cmul(*sq[-1], *sq[-1]))
    pws = []
    for base in (_cmul(*_cmul(*sq[4], *sq[3]), *sq[2]), _cmul(*sq[5], *sq[2])):
        pw = []
        for _ in range(3):
            pw.append(tiles(*base))
            base = _cmul(*base, *base)
        pws.append(pw)
    dsk = pltpu.roll(jnp.broadcast_to(prm[3:4, :], (8, 512)), 64, 1)

    def cstep(m, k, a, b):
        if k < 3:
            return m[0][k] * a - m[1][k] * b, m[0][k] * b + m[1][k] * a
        return m[0][k] * a + m[1][k] * b, m[0][k] * b - m[1][k] * a

    pend = []
    z0 = pl.program_id(0)

    def push(*cs):
        start(*cs)
        obuf[4, 0:8, :] = dsk[:, 128:256]
        pend.append([PD, obuf[4, pl.ds(pl.multiple_of(z0 * 8, 8), 8), :]])

    def gate(rhs, t=None):
        if pend and t is None:
            pend[0][0] -= 1
            if pend[0][0] == 0:
                t = pend.pop(0)[1]
        if t is not None:
            parts = []
            for r in range(0, rhs.shape[0], 128):
                last = rhs[r + 120:r + 128]
                last = jnp.concatenate([jnp.where(never, t, last[:, c:c + 128])
                                        for c in range(0, rhs.shape[1], 128)], axis=1)
                parts += [rhs[r:r + 120], last]
            rhs = jnp.concatenate(parts, axis=0)
        return rhs

    def prep_b(i):
        for r in range(0, D, 64):
            v = jnp.concatenate([jnp.zeros((64, 64), F32), bv[i, r:r + 64, :].astype(F32)], axis=1)
            r2 = 384 * i + r if r < 384 else 768 + 64 * i
            bcat[r2:r2 + 64, :] = v

    ctok = []

    def prep_c():
        toks = []
        nci = -ci[0:1, :D]
        for r in range(0, D, 32):
            c_re = cv[0, r:r + 32, :].astype(F32)
            c_im = cv[1, r:r + 32, :].astype(F32)
            c2r = c_re * cr[0:1, :D] - c_im * ci[0:1, :D]
            c2i = c_re * nci - c_im * cr[0:1, :D]
            ccat[r:r + 32, 0:384] = c2r[:, 0:384]
            ccat[r:r + 32, 384:768] = c2i[:, 0:384]
            c3 = jnp.concatenate([c2r[:, 384:448], c2i[:, 384:448]], axis=1)
            ccat[r:r + 32, 768:896] = c3
            toks += [v[i:i + 8, c:c + 128] for v in (c2r[:, 0:384], c2i[:, 0:384], c3)
                     for i in range(0, 32, 8) for c in range(0, v.shape[1], 128)]
        ctok.append(functools.reduce(jnp.maximum, toks))

    def ssm_t(c):
        for k in range(4):
            if k == 0:
                xt = jnp.concatenate([jnp.zeros((64, T), F32), bxv[c, 0:64, :].astype(F32)], axis=0)
            else:
                xt = bxv[c, 128 * k - 64:128 * k + 64, :].astype(F32)
            xb32[c // 2][k, T * (c % 2):T * (c % 2) + T, :] = xt.T

    def xs(c, k, j):
        return xb32[c // 2][k, pl.ds(_row0(c) % 512 + j, 8, stride=SEGS[c % 2]), :]

    U, Hs = {}, {}

    def ssm_in(c, ns=range(7)):
        for n in ns:
            xl = jnp.concatenate([jnp.concatenate([xs(c, k, j) for k in range(4)], axis=1)
                                  for j in range(SEGS[c % 2])], axis=0)
            U[c, n] = _dot(xl, gate(bcat[128 * n:128 * n + 128, :], ctok[0] if c == 3 and n >= 3 else None), NT)

    carry = [(jnp.zeros((8, 128), F32),) * 2] * 4

    def ssm_scan(c):
        SEG, pw = SEGS[c % 2], pws[c % 2]
        sw = pltpu.roll(U[c, 6], 64, 1)

        def u(j, k):
            if k < 3:
                return U[c, k][8 * j:8 * j + 8], U[c, k + 3][8 * j:8 * j + 8]
            return U[c, 6][8 * j:8 * j + 8], sw[8 * j:8 * j + 8]
        h, hs, dep = [None] * 4, {}, None
        for ks in KG:
            for k in ks:
                h[k] = u(0, k)
                if dep is not None:
                    h[k] = tuple(jnp.where(never, dep, v) for v in h[k])
            for j in range(1, SEG):
                for k in ks:
                    a, b = cstep(lam, k, *h[k])
                    ua, ub = u(j, k)
                    h[k] = (a + ua, b + ub)
            for k in ks:
                z = [jnp.where(sub == 0, carry[k][i], pltpu.roll(h[k][i], 1, 0)) for i in range(2)]
                for n in range(3):
                    sh = 1 << n
                    a, b = cstep(pw[n], k, *[jnp.where(sub >= sh, pltpu.roll(v, sh, 0), 0.0) for v in z])
                    z = [z[0] + a, z[1] + b]
                h[k] = tuple(z)
            for j in range(SEG):
                for k in ks:
                    a, b = cstep(lam, k, *h[k])
                    ua, ub = u(j, k)
                    h[k] = hs[j, k] = (a + ua, b + ub)
                if j == SEG * DJ // 8 - 1:
                    dep = h[ks[-1]][0]
        Hs[c] = [jnp.concatenate([hs[j, 0][0], hs[j, 1][0], hs[j, 2][0], hs[j, 0][1], hs[j, 1][1], hs[j, 2][1],
                                  hs[j, 3][0]], axis=1) for j in range(SEG)]
        carry[:] = [tuple(jnp.broadcast_to(v[7:8], (8, 128)) for v in h[k]) for k in range(4)]

    def ssm_out(p, ts=range(4), between=lambda: None):
        cj = [(2 * p + i, j) for i in range(2) for j in range(SEGS[i])]
        yts = [_dot(ccat[...], gate(jnp.concatenate([Hs[c][j] for c, j in cj[16 * t:16 * t + 16]], axis=0)), NT)
               for t in ts]
        between()
        for t, yt in zip(ts, yts):
            blk = cj[16 * t:16 * t + 16]
            y_post(p, blk, jnp.concatenate([jnp.zeros((64, 128), F32), yt], axis=0), range(4))

    def y_post(p, blk, yt, ks):
        for n, k in enumerate(ks):
            y = yt[128 * n:128 * n + 128].T
            for i, (c, j) in enumerate(blk):
                rows = pl.ds(_row0(c) + j, 8, stride=SEGS[c % 2])
                v = y[8 * i:8 * i + 8] + xs(c, k, j) * dsk[:, 128 * k:128 * k + 128]
                if k == 0 and p >= NPRE:
                    v = jnp.where(lo, a3[rows, :], v)
                obuf[k, rows, :] = v

    def ssm_last(p):
        cj = [(2 * p + i, j) for i in range(2) for j in range(SEGS[i])]
        for ks, ts, cs in PIECES:
            hh = jnp.concatenate([Hs[c][j] for c, j in cj[16 * ts[0]:16 * ts[-1] + 16]], axis=0)
            yt = _dot(ccat[max(128 * ks[0] - 64, 0):128 * ks[-1] + 64, :], gate(hh), NT)
            if ks[0] == 0:
                yt = jnp.concatenate([jnp.zeros((64, yt.shape[1]), F32), yt], axis=0)
            for n, t in enumerate(ts):
                y_post(p, cj[16 * t:16 * t + 16], yt[:, 128 * n:128 * n + 128], ks)
            start(*[o_b[2 * p + c][k] for c in cs for k in ks])

    def w_t(c0, c1):
        for k in range(4):
            n = min(128, D - 128 * k)
            blk = wv[128 * k:128 * k + n, c0:c1].astype(F32)
            if n < 128:
                blk = jnp.concatenate([blk, jnp.zeros((128 - n, c1 - c0), F32)], axis=0)
            wt32[k, c0:c1, :] = blk.T

    def w_rows(g):
        return jnp.concatenate(
            [jnp.concatenate([wt32[k, pl.ds(g * D + hh * 224 + d, 8, stride=DH), :] for k in range(4)], axis=1)
             for d in range(DH) for hh in range(2)], axis=0)

    def w_perm(g):
        for d in range(DH):
            v = [jnp.concatenate([wt32[k, pl.ds(g * D + hh * 224 + d, 8, stride=DH), :]
                                  for k in range(4)], axis=1) for hh in range(2)]
            wtp[g * D + 16 * d:g * D + 16 * d + 16, :] = jnp.concatenate(v, axis=0)

    def x_t():
        for k in range(4):
            n = min(128, D - 128 * k)
            for t in range(4):
                blk = axv[128 * k:128 * k + n, 512 * t:512 * t + 512].astype(F32)
                if n < 128:
                    blk = jnp.concatenate([blk, jnp.zeros((128 - n, 512), F32)], axis=0)
                bt = blk.T
                for g in range(32):
                    r = XP * (32 * t + g)
                    xa32[k, r:r + 16, :] = bt[16 * g:16 * g + 16]

    def wo_prep():
        wo = jnp.concatenate([wov[...].astype(F32), jnp.zeros((D, 64), F32)], axis=1)
        for k in range(4):
            wo32[k] = wo[:, 128 * k:128 * k + 128]
        for k in range(4):
            v = [wo32[k, pl.ds(hh * 224 + d, 8, stride=DH), :] for d in range(DH) for hh in range(2)]
            v = jnp.concatenate(v + [jnp.zeros((64, 128), F32)], axis=0).T
            n = min(128, D - 128 * k)
            wot[128 * k:128 * k + n, :] = v[:n]

    def xa(j):
        return jnp.concatenate([xa32[k, pl.ds(j, 128, stride=XP), :] for k in range(4)], axis=1)

    KV, Q, O = ({}, {}), {}, {}

    def att_kv(j, gs=(0, 1)):
        for g in gs:
            r = _dot(w_rows(g + 1), gate(xa(j)), NT)
            KV[g][j + 14] = r
            if j >= 2 and j != NJ - 2:
                KV[g][j - 2] = pltpu.roll(r, 1, 1)

    def att_q(*js):
        for j in js:
            Q[j] = _dot(w_rows(0), gate(xa(j)), NT)

    scale = DH ** -0.5

    PP = {}

    def att_l(jp):
        js = JP[jp]
        es = range(js[0], js[1] + 15, 2)
        P = {}
        for hh in range(2):
            lg = {}
            for d in range(DH):
                r = slice(16 * d + 8 * hh, 16 * d + 8 * hh + 8)
                for j in js:
                    for w in range(W):
                        t = Q[j][r] * KV[0][j + 14 - 2 * w][r]
                        lg[j, w] = t if d == 0 else lg[j, w] + t
            for j in js:
                l = [lg[j, w] * scale for w in range(W)]
                l = [jnp.where(lane1 == 0, -1e9, l[w]) if j < 2 * w else l[w] for w in range(W)]
                m = l[0]
                for w in range(1, W):
                    m = jnp.maximum(m, l[w])
                e = [jnp.exp(x - m) for x in l]
                ssum = e[0]
                for w in range(1, W):
                    ssum = ssum + e[w]
                inv = 1.0 / ssum
                P[hh, j] = [x * inv for x in e]
        PP[jp] = P

    def att_v(jp):
        js, P = JP[jp], PP[jp]
        for j in js:
            O[j] = [None] * (2 * DH)
        dep = None
        for hh, jj in [(h, js) for h in range(2)]:
            if dep is not None:
                for j in jj:
                    P[hh, j] = [jnp.where(never, dep, x) for x in P[hh, j]]
            for d in range(DH):
                r = slice(16 * d + 8 * hh, 16 * d + 8 * hh + 8)
                for j in jj:
                    acc = None
                    for w in range(W):
                        t = P[hh, j][w] * KV[1][j + 14 - 2 * w][r]
                        acc = t if acc is None else acc + t
                    O[j][2 * d + hh] = acc
                    if d == DH - 1:
                        dep = acc

    def att_o(jp):
        rhs = jnp.concatenate([jnp.concatenate(O[j] + [jnp.zeros((64, 128), F32)], axis=0) for j in JP[jp]], axis=1)
        res = _dot(wot[...], gate(rhs), NN)
        for i, j in enumerate(JP[jp]):
            rt = jnp.concatenate([res[:, 128 * i:128 * i + 128], jnp.zeros((64, 128), F32)], axis=0)
            for k in range(4):
                ost[j % 2][k, pl.ds(OP * (j // 2), 128), :] = rt[128 * k:128 * k + 128].T

    def o_rows(par, k, s):
        return ost[par][k, pl.ds(s, 8, stride=OP), :]

    def o_unperm(par):
        for k in range(3):
            for s in range(128):
                oa[k, pl.ds(NJ * s + par, 8, stride=2), :] = o_rows(par, k, s)

    def o_mixed():
        for s in range(128):
            for par in range(2):
                rows = pl.ds(NJ * s + par, 8, stride=2)
                if NJ * s < 512 * NPRE:
                    obuf[0, rows, :] = jnp.where(lo, o_rows(par, 3, s), obuf[0, rows, :])
                else:
                    a3[rows, :] = o_rows(par, 3, s)

    o_a = [pltpu.make_async_copy(oa.at[k], out_h.at[:, pl.ds(128 * k, 128)], osem) for k in range(3)]
    o_b = [[pltpu.make_async_copy(obuf.at[k, pl.ds(_row0(c), 8 * SEGS[c % 2])],
                                  out_h.at[pl.ds(_row0(c), 8 * SEGS[c % 2]), pl.ds(128 * (k + 3), 128)],
                                  osem) for k in range(4)] for c in range(NC)]

    NPRE = 2
    ssm_t(0)
    wait(c_b[0])
    start(c_bx[1], c_bx[2], c_bx[3])
    prep_b(0)
    ssm_in(0, range(2))
    wait(c_b[1], c_bx[1])
    start(*c_c, c_w)
    prep_b(1)
    ssm_t(1)
    ssm_in(0, range(2, 7))
    ssm_in(1, range(2))
    wait(c_bx[2], c_bx[3])
    start(c_ax)
    ssm_in(1, range(2, 7))
    ssm_scan(0)
    ssm_t(2)
    ssm_t(3)
    ssm_in(2, range(7))
    wait(*c_c, c_w)
    w_t(384, 3 * D)
    prep_c()
    ssm_in(2, range(7, 7))
    ssm_in(3, range(2))
    ssm_scan(1)
    ssm_in(3, range(2, 7))
    cj0 = [(i, j) for i in range(2) for j in range(SEGS[i])]
    h0 = [jnp.concatenate([Hs[c][j] for c, j in cj0[16 * t:16 * t + 16]], axis=0) for t in range(2)]
    y0 = _dot(ccat[...], h0[0], NT)
    y1 = _dot(ccat[:, 0:640], h0[1][:, 0:640], NT)
    y1 = jnp.concatenate([jnp.where(never, 0.0, y1[r:r + 8]) for r in range(0, D, 8)], axis=0)
    wait(c_ax)
    start(c_wo, *c_bx[4:])
    y1 = y1 + _dot(ccat[:, 640:], h0[1][:, 640:], NT)
    for t, y in enumerate((y0, y1)):
        y_post(0, cj0[16 * t:16 * t + 16], jnp.concatenate([jnp.zeros((64, 128), F32), y], axis=0), range(4))
    x_t()
    ssm_out(0, range(2, 4))
    ssm_scan(2)
    for j in range(0, NJ, 2):
        att_kv(j)
    ssm_scan(3)
    w_t(0, 384)
    start(*o_b[0][1:], *o_b[1][1:])
    wait(c_wo, *c_bx[4:6])
    for g in range(2):
        KV[g][NJ - 4] = pltpu.roll(KV[g][NJ + 12], 1, 1)
    wo_prep()
    att_kv(1, (1,))
    att_q(0)
    att_q(2)
    att_kv(1, (0,))
    att_q(4)
    att_q(6)
    att_l(0)
    att_v(0)
    att_kv(3, (0,))
    att_kv(3, (1,))
    att_kv(5, (0,))
    att_kv(5, (1,))
    att_q(8)
    att_q(10)
    att_l(1)
    att_v(1)
    att_kv(7, (0,))
    att_kv(7, (1,))
    att_kv(9, (0,))
    att_kv(9, (1,))
    att_q(12)
    att_q(14)
    att_l(2)
    att_v(2)
    att_kv(11, (0,))
    att_kv(11, (1,))
    att_o(0)
    att_kv(13, (0,))
    att_kv(13, (1,))
    att_q(1)
    att_q(3)
    att_l(3)
    att_v(3)
    att_kv(15, (0,))
    att_kv(15, (1,))
    att_o(1)
    ssm_t(4)
    ssm_t(5)
    att_q(5)
    att_q(7)
    ssm_out(1, [0])
    att_l(4)
    att_v(4)
    att_o(2)
    att_q(9)
    att_q(11)
    ssm_out(1, [1])
    push(*o_b[2][1:])
    att_l(5)
    att_v(5)
    att_o(3)
    o_unperm(0)
    att_q(13)
    att_q(15)
    ssm_out(1, [2])
    att_l(6)
    att_v(6)
    att_o(4)
    ssm_out(1, [3])
    push(*o_b[3][1:])
    att_l(7)
    att_v(7)
    att_o(5)
    att_o(6)
    att_o(7)
    ssm_in(4, [0])
    ssm_in(4, [1])
    ssm_in(4, [2])
    ssm_in(4, [3])
    o_unperm(1)
    o_mixed()
    start(*o_a, o_b[0][0], o_b[1][0], o_b[2][0], o_b[3][0])
    wait(*c_bx[6:])
    ssm_t(6)
    ssm_t(7)
    ssm_in(4, range(4, 7))
    ssm_in(5)
    ssm_scan(4)
    ssm_in(6)
    ssm_scan(5)
    ssm_out(2, range(2))
    push(*o_b[4])
    ssm_in(7)
    ssm_out(2, range(2, 3))
    ssm_scan(6)
    ssm_out(2, range(3, 4))
    push(*o_b[5])
    ssm_scan(7)
    ssm_last(3)
    pltpu.make_async_copy(out_h, out_h, osem).wait()


@jax.jit
def pallas_concat_heads__sliding_local_dilated__ssm_conv_s5__prompt_kernel(
    A_x, A_wqkv, A_wo, B_x, B_Lambda_re, B_Lambda_im, B_B_re, B_B_im, B_C_re, B_C_im,
    B_log_dt, B_Dskip,
):
    hbm = pl.BlockSpec(memory_space=pltpu.HBM)
    out = pl.pallas_call(
        _kernel,
        out_shape=jax.ShapeDtypeStruct((S, 2 * D), F32),
        grid=(1,),
        in_specs=[hbm] * 12,
        out_specs=hbm,
        scratch_shapes=[
            pltpu.VMEM((D, S), BF16),
            pltpu.VMEM((D, 3 * D), BF16),
            pltpu.VMEM((D, D), BF16),
            pltpu.VMEM((NC, D, T), BF16),
            pltpu.VMEM((2, D, D), BF16),
            pltpu.VMEM((2, D, D), BF16),
            *[pltpu.VMEM((D,), BF16)] * 4,
            pltpu.VMEM((8, 512), F32),
            pltpu.VMEM((896, 512), F32),
            pltpu.VMEM((D, 896), F32),
            *[pltpu.VMEM((4, 512, 128), F32)] * 4,
            pltpu.VMEM((4, 3 * D, 128), F32),
            pltpu.VMEM((3 * D, 512), F32),
            pltpu.VMEM((4, D, 128), F32),
            pltpu.VMEM((D, 512), F32),
            pltpu.VMEM((4, 128 * XP, 128), F32),
            pltpu.VMEM((5, S, 128), F32),
            pltpu.VMEM((S, 128), F32),
            pltpu.VMEM((3, S, 128), F32),
            *[pltpu.VMEM((4, 8 * OP, 128), F32)] * 2,
            pltpu.SemaphoreType.DMA((11 + NC,)),
            pltpu.SemaphoreType.DMA(()),
        ],
        compiler_params=pltpu.CompilerParams(vmem_limit_bytes=100 * 1024 * 1024),
    )(A_x[0].T, A_wqkv, A_wo, B_x[0].T, B_Lambda_re, B_Lambda_im,
      B_B_re, B_B_im, B_C_re, B_C_im, B_log_dt, B_Dskip)
    return out.reshape(1, S, 2 * D)
```

```python
import functools

import jax
import jax.numpy as jnp
from jax import lax
import jax.experimental.pallas as pl
import jax.experimental.pallas.tpu as pltpu

S, D, H, DH, W = 2048, 448, 16, 28, 8
NJ = 16
T = 256
NC = S // T
SEGS = (28, 36)
XP = 20
KG, DJ = ((0,), (1,), (2,), (3,)), 8
OP = 132
PIECES = (((0, 1), (0, 1, 2, 3), (0, 1)), ((2,), (0, 1, 2, 3), (0, 1)), ((3,), (0, 1), (0,)), ((3,), (2, 3), (1,)))
LO = 2
PD = 4
F32, BF16 = jnp.float32, jnp.bfloat16
NN = (((1,), (0,)), ((), ()))
NT = (((1,), (1,)), ((), ()))
JP = [(0, 2), (4, 6), (8, 10), (12, 14), (1, 3), (5, 7), (9, 11), (13, 15)]


_dot = functools.partial(lax.dot_general, preferred_element_type=F32)


def _row0(c):
    return 512 * (c // 2) + 8 * SEGS[0] * (c % 2)


def _cmul(ar, ai, br, bi):
    return ar * br - ai * bi, ar * bi + ai * br


def _kernel(ax_h, wqkv_h, wo_h, bx_h, lre_h, lim_h, bre_h, bim_h, cre_h, cim_h, ldt_h, dsk_h,
            out_h,
            axv, wv, wov, bxv, bv, cv, pv0, pv1, pv2, pv3, prm, bcat, ccat, xb0, xb1, xb2, xb3,
            wt32, wtp, wo32, wot, xa32, obuf, a3, oa, ost0, ost1, isem, osem):
    ost = (ost0, ost1)
    xb32 = (xb0, xb1, xb2, xb3)

    def cp(i, src, dst):
        return pltpu.make_async_copy(src, dst, isem.at[i])
    c_par = [cp(0, lre_h, pv0), cp(1, lim_h, pv1), cp(2, ldt_h, pv2), cp(3, dsk_h, pv3)]
    c_b = [cp(4, bre_h, bv.at[0]), cp(5, bim_h, bv.at[1])]
    c_c = [cp(6, cre_h, cv.at[0]), cp(7, cim_h, cv.at[1])]
    c_bx = [cp(8 + c, bx_h.at[:, pl.ds(c * T, T)], bxv.at[c]) for c in range(NC)]
    c_w, c_ax, c_wo = cp(8 + NC, wqkv_h, wv), cp(9 + NC, ax_h, axv), cp(10 + NC, wo_h, wov)

    def start(*cs):
        for c in cs:
            c.start()

    def wait(*cs):
        for c in cs:
            c.wait()
    start(*c_par, c_bx[0], c_b[0], c_b[1])

    wait(*c_par, c_bx[0])
    prm[...] = jnp.zeros(prm.shape, F32)
    for i in range(4):
        prm[i:i + 1, 0:D] = (pv0, pv1, pv2, pv3)[i][...].astype(F32).reshape(1, D)
    lane5 = lax.broadcasted_iota(jnp.int32, (8, 512), 1)
    lre = jnp.where(lane5 < D, jnp.broadcast_to(prm[0:1, :], (8, 512)), -1.0)
    lim = jnp.broadcast_to(prm[1:2, :], (8, 512))
    dt = jnp.exp(jnp.broadcast_to(prm[2:3, :], (8, 512))).astype(BF16).astype(F32)
    never = dt[:, 0:128] < 0.0
    zr, zi = dt * lre, dt * lim
    mag = jnp.exp(zr)
    lr, li = mag * jnp.cos(zi), mag * jnp.sin(zi)
    den = lre * lre + lim * lim
    nr, ni = lr - 1.0, li
    cr = 2.0 * (nr * lre + ni * lim) / den
    ci = 2.0 * (ni * lre - nr * lim) / den
    lane1 = lax.broadcasted_iota(jnp.int32, (8, 128), 1)
    sub = lax.broadcasted_iota(jnp.int32, (8, 128), 0)
    lo = lane1 < 64

    def tiles(r, i):
        r3, i3 = r[:, 384:], i[:, 384:]
        rr = jnp.where(lo, r3, pltpu.roll(r3, 64, 1))
        ii = jnp.where(lo, -i3, pltpu.roll(i3, 64, 1))
        return ([r[:, 128 * k:128 * k + 128] for k in range(3)] + [rr],
                [i[:, 128 * k:128 * k + 128] for k in range(3)] + [ii])
    lam = tiles(lr, li)
    sq = [(lr, li)]
    for _ in range(5):
        sq.append(_cmul(*sq[-1], *sq[-1]))
    pws = []
    for base in (_cmul(*_cmul(*sq[4], *sq[3]), *sq[2]), _cmul(*sq[5], *sq[2])):
        pw = []
        for _ in range(3):
            pw.append(tiles(*base))
            base = _cmul(*base, *base)
        pws.append(pw)
    dsk = pltpu.roll(jnp.broadcast_to(prm[3:4, :], (8, 512)), 64, 1)

    def cstep(m, k, a, b):
        if k < 3:
            return m[0][k] * a - m[1][k] * b, m[0][k] * b + m[1][k] * a
        return m[0][k] * a + m[1][k] * b, m[0][k] * b - m[1][k] * a

    pend = []
    z0 = pl.program_id(0)

    def push(*cs):
        start(*cs)
        obuf[4, 0:8, :] = dsk[:, 128:256]
        pend.append([PD, obuf[4, pl.ds(pl.multiple_of(z0 * 8, 8), 8), :]])

    def gate(rhs, t=None):
        if pend and t is None:
            pend[0][0] -= 1
            if pend[0][0] == 0:
                t = pend.pop(0)[1]
        if t is not None:
            parts = []
            for r in range(0, rhs.shape[0], 128):
                last = rhs[r + 120:r + 128]
                last = jnp.concatenate([jnp.where(never, t, last[:, c:c + 128])
                                        for c in range(0, rhs.shape[1], 128)], axis=1)
                parts += [rhs[r:r + 120], last]
            rhs = jnp.concatenate(parts, axis=0)
        return rhs

    def prep_b(i):
        for r in range(0, D, 64):
            v = jnp.concatenate([jnp.zeros((64, 64), F32), bv[i, r:r + 64, :].astype(F32)], axis=1)
            r2 = 384 * i + r if r < 384 else 768 + 64 * i
            bcat[r2:r2 + 64, :] = v

    ctok = []

    def prep_c():
        toks = []
        nci = -ci[0:1, :D]
        for r in range(0, D, 32):
            c_re = cv[0, r:r + 32, :].astype(F32)
            c_im = cv[1, r:r + 32, :].astype(F32)
            c2r = c_re * cr[0:1, :D] - c_im * ci[0:1, :D]
            c2i = c_re * nci - c_im * cr[0:1, :D]
            ccat[r:r + 32, 0:384] = c2r[:, 0:384]
            ccat[r:r + 32, 384:768] = c2i[:, 0:384]
            c3 = jnp.concatenate([c2r[:, 384:448], c2i[:, 384:448]], axis=1)
            ccat[r:r + 32, 768:896] = c3
            toks += [v[i:i + 8, c:c + 128] for v in (c2r[:, 0:384], c2i[:, 0:384], c3)
                     for i in range(0, 32, 8) for c in range(0, v.shape[1], 128)]
        ctok.append(functools.reduce(jnp.maximum, toks))

    def ssm_t(c):
        for k in range(4):
            if k == 0:
                xt = jnp.concatenate([jnp.zeros((64, T), F32), bxv[c, 0:64, :].astype(F32)], axis=0)
            else:
                xt = bxv[c, 128 * k - 64:128 * k + 64, :].astype(F32)
            xb32[c // 2][k, T * (c % 2):T * (c % 2) + T, :] = xt.T

    def xs(c, k, j):
        return xb32[c // 2][k, pl.ds(_row0(c) % 512 + j, 8, stride=SEGS[c % 2]), :]

    U, Hs = {}, {}

    def ssm_in(c, ns=range(7)):
        for n in ns:
            xl = jnp.concatenate([jnp.concatenate([xs(c, k, j) for k in range(4)], axis=1)
                                  for j in range(SEGS[c % 2])], axis=0)
            U[c, n] = _dot(xl, gate(bcat[128 * n:128 * n + 128, :], ctok[0] if c == 3 and n >= 3 else None), NT)

    carry = [(jnp.zeros((8, 128), F32),) * 2] * 4

    def ssm_scan(c):
        SEG, pw = SEGS[c % 2], pws[c % 2]
        sw = pltpu.roll(U[c, 6], 64, 1)

        def u(j, k):
            if k < 3:
                return U[c, k][8 * j:8 * j + 8], U[c, k + 3][8 * j:8 * j + 8]
            return U[c, 6][8 * j:8 * j + 8], sw[8 * j:8 * j + 8]
        h, hs, dep = [None] * 4, {}, None
        for ks in KG:
            for k in ks:
                h[k] = u(0, k)
                if dep is not None:
                    h[k] = tuple(jnp.where(never, dep, v) for v in h[k])
            for j in range(1, SEG):
                for k in ks:
                    a, b = cstep(lam, k, *h[k])
                    ua, ub = u(j, k)
                    h[k] = (a + ua, b + ub)
            for k in ks:
                z = [jnp.where(sub == 0, carry[k][i], pltpu.roll(h[k][i], 1, 0)) for i in range(2)]
                for n in range(3):
                    sh = 1 << n
                    a, b = cstep(pw[n], k, *[jnp.where(sub >= sh, pltpu.roll(v, sh, 0), 0.0) for v in z])
                    z = [z[0] + a, z[1] + b]
                h[k] = tuple(z)
            for j in range(SEG):
                for k in ks:
                    a, b = cstep(lam, k, *h[k])
                    ua, ub = u(j, k)
                    h[k] = hs[j, k] = (a + ua, b + ub)
                if j == SEG * DJ // 8 - 1:
                    dep = h[ks[-1]][0]
        Hs[c] = [jnp.concatenate([hs[j, 0][0], hs[j, 1][0], hs[j, 2][0], hs[j, 0][1], hs[j, 1][1], hs[j, 2][1],
                                  hs[j, 3][0]], axis=1) for j in range(SEG)]
        carry[:] = [tuple(jnp.broadcast_to(v[7:8], (8, 128)) for v in h[k]) for k in range(4)]

    def ssm_out(p, ts=range(4), between=lambda: None):
        cj = [(2 * p + i, j) for i in range(2) for j in range(SEGS[i])]
        yts = [_dot(ccat[...], gate(jnp.concatenate([Hs[c][j] for c, j in cj[16 * t:16 * t + 16]], axis=0)), NT)
               for t in ts]
        between()
        for t, yt in zip(ts, yts):
            blk = cj[16 * t:16 * t + 16]
            y_post(p, blk, jnp.concatenate([jnp.zeros((64, 128), F32), yt], axis=0), range(4))

    def y_post(p, blk, yt, ks):
        for n, k in enumerate(ks):
            y = yt[128 * n:128 * n + 128].T
            for i, (c, j) in enumerate(blk):
                rows = pl.ds(_row0(c) + j, 8, stride=SEGS[c % 2])
                v = y[8 * i:8 * i + 8] + xs(c, k, j) * dsk[:, 128 * k:128 * k + 128]
                if k == 0 and p >= NPRE:
                    v = jnp.where(lo, a3[rows, :], v)
                obuf[k, rows, :] = v

    def ssm_last(p):
        cj = [(2 * p + i, j) for i in range(2) for j in range(SEGS[i])]
        for ks, ts, cs in PIECES:
            hh = jnp.concatenate([Hs[c][j] for c, j in cj[16 * ts[0]:16 * ts[-1] + 16]], axis=0)
            yt = _dot(ccat[max(128 * ks[0] - 64, 0):128 * ks[-1] + 64, :], gate(hh), NT)
            if ks[0] == 0:
                yt = jnp.concatenate([jnp.zeros((64, yt.shape[1]), F32), yt], axis=0)
            for n, t in enumerate(ts):
                y_post(p, cj[16 * t:16 * t + 16], yt[:, 128 * n:128 * n + 128], ks)
            start(*[o_b[2 * p + c][k] for c in cs for k in ks])

    def w_t(c0, c1):
        for k in range(4):
            n = min(128, D - 128 * k)
            blk = wv[128 * k:128 * k + n, c0:c1].astype(F32)
            if n < 128:
                blk = jnp.concatenate([blk, jnp.zeros((128 - n, c1 - c0), F32)], axis=0)
            wt32[k, c0:c1, :] = blk.T

    def w_rows(g):
        return jnp.concatenate(
            [jnp.concatenate([wt32[k, pl.ds(g * D + hh * 224 + d, 8, stride=DH), :] for k in range(4)], axis=1)
             for d in range(DH) for hh in range(2)], axis=0)

    def w_perm(g):
        for d in range(DH):
            v = [jnp.concatenate([wt32[k, pl.ds(g * D + hh * 224 + d, 8, stride=DH), :]
                                  for k in range(4)], axis=1) for hh in range(2)]
            wtp[g * D + 16 * d:g * D + 16 * d + 16, :] = jnp.concatenate(v, axis=0)

    def x_t():
        for k in range(4):
            n = min(128, D - 128 * k)
            for t in range(4):
                blk = axv[128 * k:128 * k + n, 512 * t:512 * t + 512].astype(F32)
                if n < 128:
                    blk = jnp.concatenate([blk, jnp.zeros((128 - n, 512), F32)], axis=0)
                bt = blk.T
                for g in range(32):
                    r = XP * (32 * t + g)
                    xa32[k, r:r + 16, :] = bt[16 * g:16 * g + 16]

    def wo_prep():
        wo = jnp.concatenate([wov[...].astype(F32), jnp.zeros((D, 64), F32)], axis=1)
        for k in range(4):
            wo32[k] = wo[:, 128 * k:128 * k + 128]
        for k in range(4):
            v = [wo32[k, pl.ds(hh * 224 + d, 8, stride=DH), :] for d in range(DH) for hh in range(2)]
            v = jnp.concatenate(v + [jnp.zeros((64, 128), F32)], axis=0).T
            n = min(128, D - 128 * k)
            wot[128 * k:128 * k + n, :] = v[:n]

    def xa(j):
        return jnp.concatenate([xa32[k, pl.ds(j, 128, stride=XP), :] for k in range(4)], axis=1)

    KV, Q, O = ({}, {}), {}, {}

    def att_kv(j, gs=(0, 1)):
        for g in gs:
            r = _dot(w_rows(g + 1), gate(xa(j)), NT)
            KV[g][j + 14] = r
            if j >= 2 and j != NJ - 2:
                KV[g][j - 2] = pltpu.roll(r, 1, 1)

    def att_q(*js):
        for j in js:
            Q[j] = _dot(w_rows(0), gate(xa(j)), NT)

    scale = DH ** -0.5

    PP = {}

    def att_l(jp):
        js = JP[jp]
        es = range(js[0], js[1] + 15, 2)
        P = {}
        for hh in range(2):
            lg = {}
            for d in range(DH):
                r = slice(16 * d + 8 * hh, 16 * d + 8 * hh + 8)
                for j in js:
                    for w in range(W):
                        t = Q[j][r] * KV[0][j + 14 - 2 * w][r]
                        lg[j, w] = t if d == 0 else lg[j, w] + t
            for j in js:
                l = [lg[j, w] * scale for w in range(W)]
                l = [jnp.where(lane1 == 0, -1e9, l[w]) if j < 2 * w else l[w] for w in range(W)]
                m = l[0]
                for w in range(1, W):
                    m = jnp.maximum(m, l[w])
                e = [jnp.exp(x - m) for x in l]
                ssum = e[0]
                for w in range(1, W):
                    ssum = ssum + e[w]
                inv = 1.0 / ssum
                P[hh, j] = [x * inv for x in e]
        PP[jp] = P

    def att_v(jp):
        js, P = JP[jp], PP[jp]
        for j in js:
            O[j] = [None] * (2 * DH)
        dep = None
        for hh, jj in [(h, js) for h in range(2)]:
            if dep is not None:
                for j in jj:
                    P[hh, j] = [jnp.where(never, dep, x) for x in P[hh, j]]
            for d in range(DH):
                r = slice(16 * d + 8 * hh, 16 * d + 8 * hh + 8)
                for j in jj:
                    acc = None
                    for w in range(W):
                        t = P[hh, j][w] * KV[1][j + 14 - 2 * w][r]
                        acc = t if acc is None else acc + t
                    O[j][2 * d + hh] = acc
                    if d == DH - 1:
                        dep = acc

    def att_o(jp):
        rhs = jnp.concatenate([jnp.concatenate(O[j] + [jnp.zeros((64, 128), F32)], axis=0) for j in JP[jp]], axis=1)
        res = _dot(wot[...], gate(rhs), NN)
        for i, j in enumerate(JP[jp]):
            rt = jnp.concatenate([res[:, 128 * i:128 * i + 128], jnp.zeros((64, 128), F32)], axis=0)
            for k in range(4):
                ost[j % 2][k, pl.ds(OP * (j // 2), 128), :] = rt[128 * k:128 * k + 128].T

    def o_rows(par, k, s):
        return ost[par][k, pl.ds(s, 8, stride=OP), :]

    def o_unperm(par):
        for k in range(3):
            for s in range(128):
                oa[k, pl.ds(NJ * s + par, 8, stride=2), :] = o_rows(par, k, s)

    def o_mixed():
        for s in range(128):
            for par in range(2):
                rows = pl.ds(NJ * s + par, 8, stride=2)
                if NJ * s < 512 * NPRE:
                    obuf[0, rows, :] = jnp.where(lo, o_rows(par, 3, s), obuf[0, rows, :])
                else:
                    a3[rows, :] = o_rows(par, 3, s)

    o_a = [pltpu.make_async_copy(oa.at[k], out_h.at[:, pl.ds(128 * k, 128)], osem) for k in range(3)]
    o_b = [[pltpu.make_async_copy(obuf.at[k, pl.ds(_row0(c), 8 * SEGS[c % 2])],
                                  out_h.at[pl.ds(_row0(c), 8 * SEGS[c % 2]), pl.ds(128 * (k + 3), 128)],
                                  osem) for k in range(4)] for c in range(NC)]

    NPRE = 2
    ssm_t(0)
    wait(c_b[0])
    start(c_bx[1], c_bx[2], c_bx[3])
    prep_b(0)
    ssm_in(0, range(2))
    wait(c_b[1], c_bx[1])
    start(*c_c, c_w)
    prep_b(1)
    ssm_t(1)
    ssm_in(0, range(2, 7))
    ssm_in(1, range(2))
    wait(c_bx[2], c_bx[3])
    ssm_in(1, range(2, 7))
    axv[0:16, 0:128] = U[1, 5][0:16].astype(BF16)
    start(c_ax)
    ssm_scan(0)
    ssm_t(2)
    ssm_t(3)
    ssm_in(2, range(7))
    wait(*c_c, c_w)
    w_t(384, 3 * D)
    prep_c()
    ssm_in(2, range(7, 7))
    ssm_in(3, range(2))
    ssm_scan(1)
    ssm_in(3, range(2, 7))
    cj0 = [(i, j) for i in range(2) for j in range(SEGS[i])]
    h0 = [jnp.concatenate([Hs[c][j] for c, j in cj0[16 * t:16 * t + 16]], axis=0) for t in range(3)]
    y0 = _dot(ccat[...], h0[0], NT)
    ym = _dot(ccat[...], h0[1], NT)
    y1 = _dot(ccat[:, 0:256], h0[2][:, 0:256], NT)
    y1 = jnp.concatenate([jnp.where(never, 0.0, y1[r:r + 8]) for r in range(0, D, 8)], axis=0)
    wait(c_ax)
    start(c_wo, *c_bx[4:])
    y1 = y1 + _dot(ccat[:, 256:], h0[2][:, 256:], NT)
    for t, y in enumerate((y0, ym, y1)):
        y_post(0, cj0[16 * t:16 * t + 16], jnp.concatenate([jnp.zeros((64, 128), F32), y], axis=0), range(4))
    x_t()
    ssm_out(0, range(3, 4))
    ssm_scan(2)
    for j in range(0, NJ, 2):
        att_kv(j)
    ssm_scan(3)
    w_t(0, 384)
    start(*o_b[0][1:], *o_b[1][1:])
    wait(c_wo, *c_bx[4:6])
    for g in range(2):
        KV[g][NJ - 4] = pltpu.roll(KV[g][NJ + 12], 1, 1)
    wo_prep()
    att_kv(1, (1,))
    att_q(0)
    att_q(2)
    att_kv(1, (0,))
    att_q(4)
    att_q(6)
    att_l(0)
    att_v(0)
    att_kv(3, (0,))
    att_kv(3, (1,))
    att_kv(5, (0,))
    att_kv(5, (1,))
    att_q(8)
    att_q(10)
    att_l(1)
    att_v(1)
    att_kv(7, (0,))
    att_kv(7, (1,))
    att_kv(9, (0,))
    att_kv(9, (1,))
    att_q(12)
    att_q(14)
    att_l(2)
    att_v(2)
    att_kv(11, (0,))
    att_kv(11, (1,))
    att_o(0)
    att_kv(13, (0,))
    att_kv(13, (1,))
    att_q(1)
    att_q(3)
    att_l(3)
    att_v(3)
    att_kv(15, (0,))
    att_kv(15, (1,))
    att_o(1)
    ssm_t(4)
    ssm_t(5)
    att_q(5)
    att_q(7)
    ssm_out(1, [0])
    att_l(4)
    att_v(4)
    att_o(2)
    att_q(9)
    att_q(11)
    ssm_out(1, [1])
    push(*o_b[2][1:])
    att_l(5)
    att_v(5)
    att_o(3)
    o_unperm(0)
    att_q(13)
    att_q(15)
    ssm_out(1, [2])
    att_l(6)
    att_v(6)
    att_o(4)
    ssm_out(1, [3])
    push(*o_b[3][1:])
    att_l(7)
    att_v(7)
    att_o(5)
    att_o(6)
    att_o(7)
    ssm_in(4, [0])
    ssm_in(4, [1])
    ssm_in(4, [2])
    ssm_in(4, [3])
    o_unperm(1)
    o_mixed()
    start(*o_a, o_b[0][0], o_b[1][0], o_b[2][0], o_b[3][0])
    wait(*c_bx[6:])
    ssm_t(6)
    ssm_t(7)
    ssm_in(4, range(4, 7))
    ssm_in(5)
    ssm_scan(4)
    ssm_in(6)
    ssm_scan(5)
    ssm_out(2, range(2))
    push(*o_b[4])
    ssm_in(7)
    ssm_out(2, range(2, 3))
    ssm_scan(6)
    ssm_out(2, range(3, 4))
    push(*o_b[5])
    ssm_scan(7)
    ssm_last(3)
    pltpu.make_async_copy(out_h, out_h, osem).wait()


@jax.jit
def pallas_concat_heads__sliding_local_dilated__ssm_conv_s5__prompt_kernel(
    A_x, A_wqkv, A_wo, B_x, B_Lambda_re, B_Lambda_im, B_B_re, B_B_im, B_C_re, B_C_im,
    B_log_dt, B_Dskip,
):
    hbm = pl.BlockSpec(memory_space=pltpu.HBM)
    out = pl.pallas_call(
        _kernel,
        out_shape=jax.ShapeDtypeStruct((S, 2 * D), F32),
        grid=(1,),
        in_specs=[hbm] * 12,
        out_specs=hbm,
        scratch_shapes=[
            pltpu.VMEM((D, S), BF16),
            pltpu.VMEM((D, 3 * D), BF16),
            pltpu.VMEM((D, D), BF16),
            pltpu.VMEM((NC, D, T), BF16),
            pltpu.VMEM((2, D, D), BF16),
            pltpu.VMEM((2, D, D), BF16),
            *[pltpu.VMEM((D,), BF16)] * 4,
            pltpu.VMEM((8, 512), F32),
            pltpu.VMEM((896, 512), F32),
            pltpu.VMEM((D, 896), F32),
            *[pltpu.VMEM((4, 512, 128), F32)] * 4,
            pltpu.VMEM((4, 3 * D, 128), F32),
            pltpu.VMEM((3 * D, 512), F32),
            pltpu.VMEM((4, D, 128), F32),
            pltpu.VMEM((D, 512), F32),
            pltpu.VMEM((4, 128 * XP, 128), F32),
            pltpu.VMEM((5, S, 128), F32),
            pltpu.VMEM((S, 128), F32),
            pltpu.VMEM((3, S, 128), F32),
            *[pltpu.VMEM((4, 8 * OP, 128), F32)] * 2,
            pltpu.SemaphoreType.DMA((11 + NC,)),
            pltpu.SemaphoreType.DMA(()),
        ],
        compiler_params=pltpu.CompilerParams(vmem_limit_bytes=100 * 1024 * 1024),
    )(A_x[0].T, A_wqkv, A_wo, B_x[0].T, B_Lambda_re, B_Lambda_im,
      B_B_re, B_B_im, B_C_re, B_C_im, B_log_dt, B_Dskip)
    return out.reshape(1, S, 2 * D)
```

```python
import functools

import jax
import jax.numpy as jnp
from jax import lax
import jax.experimental.pallas as pl
import jax.experimental.pallas.tpu as pltpu

S, D, H, DH, W = 2048, 448, 16, 28, 8
NJ = 16
T = 256
NC = S // T
SEGS = (28, 36)
XP = 20
KG, DJ = ((0,), (1,), (2,), (3,)), 8
OP = 132
PIECES = (((0, 1), (0, 1, 2, 3), (0, 1)), ((2,), (0, 1, 2, 3), (0, 1)), ((3,), (0, 1), (0,)), ((3,), (2, 3), (1,)))
PD = 4
F32, BF16 = jnp.float32, jnp.bfloat16
NN = (((1,), (0,)), ((), ()))
NT = (((1,), (1,)), ((), ()))
JP = [(0, 2), (4, 6), (8, 10), (12, 14), (1, 3), (5, 7), (9, 11), (13, 15)]


_dot = functools.partial(lax.dot_general, preferred_element_type=F32)


def _row0(c):
    return 512 * (c // 2) + 8 * SEGS[0] * (c % 2)


def _cmul(ar, ai, br, bi):
    return ar * br - ai * bi, ar * bi + ai * br


def _kernel(ax_h, wqkv_h, wo_h, bx_h, lre_h, lim_h, bre_h, bim_h, cre_h, cim_h, ldt_h, dsk_h,
            out_h,
            axv, wv, wov, bxv, bv, cv, pv0, pv1, pv2, pv3, prm, bcat, ccat, xb0, xb1, xb2, xb3,
            wt32, wo32, wot, xa32, obuf, a3, oa, ost0, ost1, isem, osem):
    ost = (ost0, ost1)
    xb32 = (xb0, xb1, xb2, xb3)

    def cp(i, src, dst):
        return pltpu.make_async_copy(src, dst, isem.at[i])
    c_par = [cp(0, lre_h, pv0), cp(1, lim_h, pv1), cp(2, ldt_h, pv2), cp(3, dsk_h, pv3)]
    c_b = [cp(4, bre_h, bv.at[0]), cp(5, bim_h, bv.at[1])]
    c_c = [cp(6, cre_h, cv.at[0]), cp(7, cim_h, cv.at[1])]
    c_bx = [cp(8 + c, bx_h.at[:, pl.ds(c * T, T)], bxv.at[c]) for c in range(NC)]
    c_w, c_ax, c_wo = cp(8 + NC, wqkv_h, wv), cp(9 + NC, ax_h, axv), cp(10 + NC, wo_h, wov)

    def start(*cs):
        for c in cs:
            c.start()

    def wait(*cs):
        for c in cs:
            c.wait()
    start(*c_par, c_bx[0], c_b[0], c_b[1])

    wait(*c_par, c_bx[0])
    prm[...] = jnp.zeros(prm.shape, F32)
    for i in range(4):
        prm[i:i + 1, 0:D] = (pv0, pv1, pv2, pv3)[i][...].astype(F32).reshape(1, D)
    lane5 = lax.broadcasted_iota(jnp.int32, (8, 512), 1)
    lre = jnp.where(lane5 < D, jnp.broadcast_to(prm[0:1, :], (8, 512)), -1.0)
    lim = jnp.broadcast_to(prm[1:2, :], (8, 512))
    dt = jnp.exp(jnp.broadcast_to(prm[2:3, :], (8, 512))).astype(BF16).astype(F32)
    never = dt[:, 0:128] < 0.0
    zr, zi = dt * lre, dt * lim
    mag = jnp.exp(zr)
    lr, li = mag * jnp.cos(zi), mag * jnp.sin(zi)
    den = lre * lre + lim * lim
    nr, ni = lr - 1.0, li
    cr = 2.0 * (nr * lre + ni * lim) / den
    ci = 2.0 * (ni * lre - nr * lim) / den
    lane1 = lax.broadcasted_iota(jnp.int32, (8, 128), 1)
    sub = lax.broadcasted_iota(jnp.int32, (8, 128), 0)
    lo = lane1 < 64

    def tiles(r, i):
        r3, i3 = r[:, 384:], i[:, 384:]
        rr = jnp.where(lo, r3, pltpu.roll(r3, 64, 1))
        ii = jnp.where(lo, -i3, pltpu.roll(i3, 64, 1))
        return ([r[:, 128 * k:128 * k + 128] for k in range(3)] + [rr],
                [i[:, 128 * k:128 * k + 128] for k in range(3)] + [ii])
    lam = tiles(lr, li)
    sq = [(lr, li)]
    for _ in range(5):
        sq.append(_cmul(*sq[-1], *sq[-1]))
    pws = []
    for base in (_cmul(*_cmul(*sq[4], *sq[3]), *sq[2]), _cmul(*sq[5], *sq[2])):
        pw = []
        for _ in range(3):
            pw.append(tiles(*base))
            base = _cmul(*base, *base)
        pws.append(pw)
    dsk = pltpu.roll(jnp.broadcast_to(prm[3:4, :], (8, 512)), 64, 1)

    def cstep(m, k, a, b):
        if k < 3:
            return m[0][k] * a - m[1][k] * b, m[0][k] * b + m[1][k] * a
        return m[0][k] * a + m[1][k] * b, m[0][k] * b - m[1][k] * a

    pend = []
    z0 = pl.program_id(0)

    def push(*cs):
        start(*cs)
        obuf[4, 0:8, :] = dsk[:, 128:256]
        pend.append([PD, obuf[4, pl.ds(pl.multiple_of(z0 * 8, 8), 8), :]])

    def gate(rhs, t=None):
        if pend and t is None:
            pend[0][0] -= 1
            if pend[0][0] == 0:
                t = pend.pop(0)[1]
        if t is not None:
            parts = []
            for r in range(0, rhs.shape[0], 128):
                last = rhs[r + 120:r + 128]
                last = jnp.concatenate([jnp.where(never, t, last[:, c:c + 128])
                                        for c in range(0, rhs.shape[1], 128)], axis=1)
                parts += [rhs[r:r + 120], last]
            rhs = jnp.concatenate(parts, axis=0)
        return rhs

    def prep_b(i):
        for r in range(0, D, 64):
            v = jnp.concatenate([jnp.zeros((64, 64), F32), bv[i, r:r + 64, :].astype(F32)], axis=1)
            r2 = 384 * i + r if r < 384 else 768 + 64 * i
            bcat[r2:r2 + 64, :] = v

    ctok = []

    def prep_c():
        toks = []
        nci = -ci[0:1, :D]
        for r in range(0, D, 32):
            c_re = cv[0, r:r + 32, :].astype(F32)
            c_im = cv[1, r:r + 32, :].astype(F32)
            c2r = c_re * cr[0:1, :D] - c_im * ci[0:1, :D]
            c2i = c_re * nci - c_im * cr[0:1, :D]
            ccat[r:r + 32, 0:384] = c2r[:, 0:384]
            ccat[r:r + 32, 384:768] = c2i[:, 0:384]
            c3 = jnp.concatenate([c2r[:, 384:448], c2i[:, 384:448]], axis=1)
            ccat[r:r + 32, 768:896] = c3
            toks += [v[i:i + 8, c:c + 128] for v in (c2r[:, 0:384], c2i[:, 0:384], c3)
                     for i in range(0, 32, 8) for c in range(0, v.shape[1], 128)]
        ctok.append(functools.reduce(jnp.maximum, toks))

    def ssm_t(c):
        for k in range(4):
            if k == 0:
                xt = jnp.concatenate([jnp.zeros((64, T), F32), bxv[c, 0:64, :].astype(F32)], axis=0)
            else:
                xt = bxv[c, 128 * k - 64:128 * k + 64, :].astype(F32)
            xb32[c // 2][k, T * (c % 2):T * (c % 2) + T, :] = xt.T

    def xs(c, k, j):
        return xb32[c // 2][k, pl.ds(_row0(c) % 512 + j, 8, stride=SEGS[c % 2]), :]

    U, Hs = {}, {}

    def ssm_in(c, ns=range(7)):
        for n in ns:
            xl = jnp.concatenate([jnp.concatenate([xs(c, k, j) for k in range(4)], axis=1)
                                  for j in range(SEGS[c % 2])], axis=0)
            U[c, n] = _dot(xl, gate(bcat[128 * n:128 * n + 128, :], ctok[0] if c == 3 and n >= 3 else None), NT)

    carry = [(jnp.zeros((8, 128), F32),) * 2] * 4

    def ssm_scan(c):
        SEG, pw = SEGS[c % 2], pws[c % 2]
        sw = pltpu.roll(U[c, 6], 64, 1)

        def u(j, k):
            if k < 3:
                return U[c, k][8 * j:8 * j + 8], U[c, k + 3][8 * j:8 * j + 8]
            return U[c, 6][8 * j:8 * j + 8], sw[8 * j:8 * j + 8]
        h, hs, dep = [None] * 4, {}, None
        for ks in KG:
            for k in ks:
                h[k] = u(0, k)
                if dep is not None:
                    h[k] = tuple(jnp.where(never, dep, v) for v in h[k])
            for j in range(1, SEG):
                for k in ks:
                    a, b = cstep(lam, k, *h[k])
                    ua, ub = u(j, k)
                    h[k] = (a + ua, b + ub)
            for k in ks:
                z = [jnp.where(sub == 0, carry[k][i], pltpu.roll(h[k][i], 1, 0)) for i in range(2)]
                for n in range(3):
                    sh = 1 << n
                    a, b = cstep(pw[n], k, *[jnp.where(sub >= sh, pltpu.roll(v, sh, 0), 0.0) for v in z])
                    z = [z[0] + a, z[1] + b]
                h[k] = tuple(z)
            for j in range(SEG):
                for k in ks:
                    a, b = cstep(lam, k, *h[k])
                    ua, ub = u(j, k)
                    h[k] = hs[j, k] = (a + ua, b + ub)
                if j == SEG * DJ // 8 - 1:
                    dep = h[ks[-1]][0]
        Hs[c] = [jnp.concatenate([hs[j, 0][0], hs[j, 1][0], hs[j, 2][0], hs[j, 0][1], hs[j, 1][1], hs[j, 2][1],
                                  hs[j, 3][0]], axis=1) for j in range(SEG)]
        carry[:] = [tuple(jnp.broadcast_to(v[7:8], (8, 128)) for v in h[k]) for k in range(4)]

    def ssm_out(p, ts=range(4), between=lambda: None):
        cj = [(2 * p + i, j) for i in range(2) for j in range(SEGS[i])]
        yts = [_dot(ccat[...], gate(jnp.concatenate([Hs[c][j] for c, j in cj[16 * t:16 * t + 16]], axis=0)), NT)
               for t in ts]
        between()
        for t, yt in zip(ts, yts):
            blk = cj[16 * t:16 * t + 16]
            y_post(p, blk, jnp.concatenate([jnp.zeros((64, 128), F32), yt], axis=0), range(4))

    def y_post(p, blk, yt, ks):
        for n, k in enumerate(ks):
            y = yt[128 * n:128 * n + 128].T
            for i, (c, j) in enumerate(blk):
                rows = pl.ds(_row0(c) + j, 8, stride=SEGS[c % 2])
                v = y[8 * i:8 * i + 8] + xs(c, k, j) * dsk[:, 128 * k:128 * k + 128]
                if k == 0 and p >= NPRE:
                    v = jnp.where(lo, a3[rows, :], v)
                obuf[k, rows, :] = v

    def ssm_last(p):
        cj = [(2 * p + i, j) for i in range(2) for j in range(SEGS[i])]
        for ks, ts, cs in PIECES:
            hh = jnp.concatenate([Hs[c][j] for c, j in cj[16 * ts[0]:16 * ts[-1] + 16]], axis=0)
            yt = _dot(ccat[max(128 * ks[0] - 64, 0):128 * ks[-1] + 64, :], gate(hh), NT)
            if ks[0] == 0:
                yt = jnp.concatenate([jnp.zeros((64, yt.shape[1]), F32), yt], axis=0)
            for n, t in enumerate(ts):
                y_post(p, cj[16 * t:16 * t + 16], yt[:, 128 * n:128 * n + 128], ks)
            start(*[o_b[2 * p + c][k] for c in cs for k in ks])

    def w_t(c0, c1):
        for k in range(4):
            n = min(128, D - 128 * k)
            blk = wv[128 * k:128 * k + n, c0:c1].astype(F32)
            if n < 128:
                blk = jnp.concatenate([blk, jnp.zeros((128 - n, c1 - c0), F32)], axis=0)
            wt32[k, c0:c1, :] = blk.T

    def w_rows(g):
        return jnp.concatenate(
            [jnp.concatenate([wt32[k, pl.ds(g * D + hh * 224 + d, 8, stride=DH), :] for k in range(4)], axis=1)
             for d in range(DH) for hh in range(2)], axis=0)

    def w_perm(g):
        for d in range(DH):
            v = [jnp.concatenate([wt32[k, pl.ds(g * D + hh * 224 + d, 8, stride=DH), :]
                                  for k in range(4)], axis=1) for hh in range(2)]
            wtp[g * D + 16 * d:g * D + 16 * d + 16, :] = jnp.concatenate(v, axis=0)

    def x_t():
        for k in range(4):
            n = min(128, D - 128 * k)
            for t in range(4):
                blk = axv[128 * k:128 * k + n, 512 * t:512 * t + 512].astype(F32)
                if n < 128:
                    blk = jnp.concatenate([blk, jnp.zeros((128 - n, 512), F32)], axis=0)
                bt = blk.T
                for g in range(32):
                    r = XP * (32 * t + g)
                    xa32[k, r:r + 16, :] = bt[16 * g:16 * g + 16]

    def wo_prep():
        wo = jnp.concatenate([wov[...].astype(F32), jnp.zeros((D, 64), F32)], axis=1)
        for k in range(4):
            wo32[k] = wo[:, 128 * k:128 * k + 128]
        for k in range(4):
            v = [wo32[k, pl.ds(hh * 224 + d, 8, stride=DH), :] for d in range(DH) for hh in range(2)]
            v = jnp.concatenate(v + [jnp.zeros((64, 128), F32)], axis=0).T
            n = min(128, D - 128 * k)
            wot[128 * k:128 * k + n, :] = v[:n]

    def xa(j):
        return jnp.concatenate([xa32[k, pl.ds(j, 128, stride=XP), :] for k in range(4)], axis=1)

    KV, Q, O = ({}, {}), {}, {}

    def att_kv(j, gs=(0, 1)):
        for g in gs:
            r = _dot(w_rows(g + 1), gate(xa(j)), NT)
            KV[g][j + 14] = r
            if j >= 2 and j != NJ - 2:
                KV[g][j - 2] = pltpu.roll(r, 1, 1)

    def att_q(*js):
        for j in js:
            Q[j] = _dot(w_rows(0), gate(xa(j)), NT)

    scale = DH ** -0.5

    PP = {}

    def att_l(jp):
        js = JP[jp]
        es = range(js[0], js[1] + 15, 2)
        P = {}
        for hh in range(2):
            lg = {}
            for d in range(DH):
                r = slice(16 * d + 8 * hh, 16 * d + 8 * hh + 8)
                for j in js:
                    for w in range(W):
                        t = Q[j][r] * KV[0][j + 14 - 2 * w][r]
                        lg[j, w] = t if d == 0 else lg[j, w] + t
            for j in js:
                l = [lg[j, w] * scale for w in range(W)]
                l = [jnp.where(lane1 == 0, -1e9, l[w]) if j < 2 * w else l[w] for w in range(W)]
                m = l[0]
                for w in range(1, W):
                    m = jnp.maximum(m, l[w])
                e = [jnp.exp(x - m) for x in l]
                ssum = e[0]
                for w in range(1, W):
                    ssum = ssum + e[w]
                inv = 1.0 / ssum
                P[hh, j] = [x * inv for x in e]
        PP[jp] = P

    def att_v(jp):
        js, P = JP[jp], PP[jp]
        for j in js:
            O[j] = [None] * (2 * DH)
        dep = None
        for hh, jj in [(h, js) for h in range(2)]:
            if dep is not None:
                for j in jj:
                    P[hh, j] = [jnp.where(never, dep, x) for x in P[hh, j]]
            for d in range(DH):
                r = slice(16 * d + 8 * hh, 16 * d + 8 * hh + 8)
                for j in jj:
                    acc = None
                    for w in range(W):
                        t = P[hh, j][w] * KV[1][j + 14 - 2 * w][r]
                        acc = t if acc is None else acc + t
                    O[j][2 * d + hh] = acc
                    if d == DH - 1:
                        dep = acc

    def att_o(jp):
        rhs = jnp.concatenate([jnp.concatenate(O[j] + [jnp.zeros((64, 128), F32)], axis=0) for j in JP[jp]], axis=1)
        res = _dot(wot[...], gate(rhs), NN)
        for i, j in enumerate(JP[jp]):
            rt = jnp.concatenate([res[:, 128 * i:128 * i + 128], jnp.zeros((64, 128), F32)], axis=0)
            for k in range(4):
                ost[j % 2][k, pl.ds(OP * (j // 2), 128), :] = rt[128 * k:128 * k + 128].T

    def o_rows(par, k, s):
        return ost[par][k, pl.ds(s, 8, stride=OP), :]

    def o_unperm(par):
        for k in range(3):
            for s in range(128):
                oa[k, pl.ds(NJ * s + par, 8, stride=2), :] = o_rows(par, k, s)

    def o_mixed():
        for s in range(128):
            for par in range(2):
                rows = pl.ds(NJ * s + par, 8, stride=2)
                if NJ * s < 512 * NPRE:
                    obuf[0, rows, :] = jnp.where(lo, o_rows(par, 3, s), obuf[0, rows, :])
                else:
                    a3[rows, :] = o_rows(par, 3, s)

    o_a = [pltpu.make_async_copy(oa.at[k], out_h.at[:, pl.ds(128 * k, 128)], osem) for k in range(3)]
    o_b = [[pltpu.make_async_copy(obuf.at[k, pl.ds(_row0(c), 8 * SEGS[c % 2])],
                                  out_h.at[pl.ds(_row0(c), 8 * SEGS[c % 2]), pl.ds(128 * (k + 3), 128)],
                                  osem) for k in range(4)] for c in range(NC)]

    NPRE = 2
    ssm_t(0)
    wait(c_b[0])
    start(c_bx[1], c_bx[2], c_bx[3])
    prep_b(0)
    ssm_in(0, range(2))
    wait(c_b[1], c_bx[1])
    start(*c_c, c_w)
    prep_b(1)
    ssm_t(1)
    ssm_in(0, range(2, 7))
    ssm_in(1, range(2))
    wait(c_bx[2], c_bx[3])
    ssm_in(1, range(2, 7))
    axv[0:16, 0:128] = U[1, 5][0:16].astype(BF16)
    start(c_ax)
    ssm_scan(0)
    ssm_t(2)
    ssm_t(3)
    ssm_in(2, range(7))
    wait(*c_c, c_w)
    w_t(384, 3 * D)
    prep_c()
    ssm_in(3, range(2))
    ssm_scan(1)
    ssm_in(3, range(2, 7))
    cj0 = [(i, j) for i in range(2) for j in range(SEGS[i])]
    h0 = [jnp.concatenate([Hs[c][j] for c, j in cj0[16 * t:16 * t + 16]], axis=0) for t in range(3)]
    y0 = _dot(ccat[...], h0[0], NT)
    ym = _dot(ccat[...], h0[1], NT)
    y1 = _dot(ccat[:, 0:256], h0[2][:, 0:256], NT)
    y1 = jnp.concatenate([jnp.where(never, 0.0, y1[r:r + 8]) for r in range(0, D, 8)], axis=0)
    wait(c_ax)
    start(c_wo, *c_bx[4:])
    y1 = y1 + _dot(ccat[:, 256:], h0[2][:, 256:], NT)
    for t, y in enumerate((y0, ym, y1)):
        y_post(0, cj0[16 * t:16 * t + 16], jnp.concatenate([jnp.zeros((64, 128), F32), y], axis=0), range(4))
    x_t()
    ssm_out(0, range(3, 4))
    ssm_scan(2)
    for j in range(0, NJ, 2):
        att_kv(j)
    ssm_scan(3)
    w_t(0, 384)
    start(*o_b[0][1:], *o_b[1][1:])
    wait(c_wo, *c_bx[4:6])
    for g in range(2):
        KV[g][NJ - 4] = pltpu.roll(KV[g][NJ + 12], 1, 1)
    wo_prep()
    att_kv(1, (1,))
    att_q(0)
    att_q(2)
    att_kv(1, (0,))
    att_q(4)
    att_q(6)
    att_l(0)
    att_v(0)
    att_kv(3, (0,))
    att_kv(3, (1,))
    att_kv(5, (0,))
    att_kv(5, (1,))
    att_q(8)
    att_q(10)
    att_l(1)
    att_v(1)
    att_kv(7, (0,))
    att_kv(7, (1,))
    att_kv(9, (0,))
    att_kv(9, (1,))
    att_q(12)
    att_q(14)
    att_l(2)
    att_v(2)
    att_kv(11, (0,))
    att_kv(11, (1,))
    att_o(0)
    att_kv(13, (0,))
    att_kv(13, (1,))
    att_q(1)
    att_q(3)
    att_l(3)
    att_v(3)
    att_kv(15, (0,))
    att_kv(15, (1,))
    att_o(1)
    ssm_t(4)
    ssm_t(5)
    att_q(5)
    att_q(7)
    ssm_out(1, [0])
    att_l(4)
    att_v(4)
    att_o(2)
    att_q(9)
    att_q(11)
    ssm_out(1, [1])
    push(*o_b[2][1:])
    att_l(5)
    att_v(5)
    att_o(3)
    o_unperm(0)
    att_q(13)
    att_q(15)
    ssm_out(1, [2])
    att_l(6)
    att_v(6)
    att_o(4)
    ssm_out(1, [3])
    push(*o_b[3][1:])
    att_l(7)
    att_v(7)
    att_o(5)
    att_o(6)
    att_o(7)
    ssm_in(4, [0])
    ssm_in(4, [1])
    ssm_in(4, [2])
    ssm_in(4, [3])
    o_unperm(1)
    o_mixed()
    start(*o_a, o_b[0][0], o_b[1][0], o_b[2][0], o_b[3][0])
    wait(*c_bx[6:])
    ssm_t(6)
    ssm_t(7)
    ssm_in(4, range(4, 7))
    ssm_in(5)
    ssm_scan(4)
    ssm_in(6)
    ssm_scan(5)
    ssm_out(2, range(2))
    push(*o_b[4])
    ssm_in(7)
    ssm_out(2, range(2, 3))
    ssm_scan(6)
    ssm_out(2, range(3, 4))
    push(*o_b[5])
    ssm_scan(7)
    ssm_last(3)
    pltpu.make_async_copy(out_h, out_h, osem).wait()


@jax.jit
def pallas_concat_heads__sliding_local_dilated__ssm_conv_s5__prompt_kernel(
    A_x, A_wqkv, A_wo, B_x, B_Lambda_re, B_Lambda_im, B_B_re, B_B_im, B_C_re, B_C_im,
    B_log_dt, B_Dskip,
):
    hbm = pl.BlockSpec(memory_space=pltpu.HBM)
    out = pl.pallas_call(
        _kernel,
        out_shape=jax.ShapeDtypeStruct((S, 2 * D), F32),
        grid=(1,),
        in_specs=[hbm] * 12,
        out_specs=hbm,
        scratch_shapes=[
            pltpu.VMEM((D, S), BF16),
            pltpu.VMEM((D, 3 * D), BF16),
            pltpu.VMEM((D, D), BF16),
            pltpu.VMEM((NC, D, T), BF16),
            pltpu.VMEM((2, D, D), BF16),
            pltpu.VMEM((2, D, D), BF16),
            *[pltpu.VMEM((D,), BF16)] * 4,
            pltpu.VMEM((8, 512), F32),
            pltpu.VMEM((896, 512), F32),
            pltpu.VMEM((D, 896), F32),
            *[pltpu.VMEM((4, 512, 128), F32)] * 4,
            pltpu.VMEM((4, 3 * D, 128), F32),
            pltpu.VMEM((4, D, 128), F32),
            pltpu.VMEM((D, 512), F32),
            pltpu.VMEM((4, 128 * XP, 128), F32),
            pltpu.VMEM((5, S, 128), F32),
            pltpu.VMEM((S, 128), F32),
            pltpu.VMEM((3, S, 128), F32),
            *[pltpu.VMEM((4, 8 * OP, 128), F32)] * 2,
            pltpu.SemaphoreType.DMA((11 + NC,)),
            pltpu.SemaphoreType.DMA(()),
        ],
        compiler_params=pltpu.CompilerParams(vmem_limit_bytes=100 * 1024 * 1024),
    )(A_x[0].T, A_wqkv, A_wo, B_x[0].T, B_Lambda_re, B_Lambda_im,
      B_B_re, B_B_im, B_C_re, B_C_im, B_log_dt, B_Dskip)
    return out.reshape(1, S, 2 * D)
```

```python
import functools

import jax
import jax.numpy as jnp
from jax import lax
import jax.experimental.pallas as pl
import jax.experimental.pallas.tpu as pltpu

S, D, H, DH, W = 2048, 448, 16, 28, 8
NJ = 16
T = 256
NC = S // T
SEGS = (28, 36)
XP = 20
KG, DJ = ((0,), (1,), (2,), (3,)), 8
OP = 132
PIECES = (((0, 1), (0, 1, 2, 3), (0, 1)), ((2,), (0, 1, 2, 3), (0, 1)), ((3,), (0, 1), (0,)), ((3,), (2, 3), (1,)))
GV = 7
PD = 4
F32, BF16 = jnp.float32, jnp.bfloat16
NN = (((1,), (0,)), ((), ()))
NT = (((1,), (1,)), ((), ()))
JP = [(0, 2), (4, 6), (8, 10), (12, 14), (1, 3), (5, 7), (9, 11), (13, 15)]


_dot = functools.partial(lax.dot_general, preferred_element_type=F32)


def _row0(c):
    return 512 * (c // 2) + 8 * SEGS[0] * (c % 2)


def _cmul(ar, ai, br, bi):
    return ar * br - ai * bi, ar * bi + ai * br


def _kernel(ax_h, wqkv_h, wo_h, bx_h, lre_h, lim_h, bre_h, bim_h, cre_h, cim_h, ldt_h, dsk_h,
            out_h,
            axv, wv, wov, bxv, bv, cv, pv0, pv1, pv2, pv3, prm, bcat, ccat, xb0, xb1, xb2, xb3,
            wt32, wo32, wot, xa32, obuf, a3, oa, ost0, ost1, isem, osem):
    ost = (ost0, ost1)
    xb32 = (xb0, xb1, xb2, xb3)

    def cp(i, src, dst):
        return pltpu.make_async_copy(src, dst, isem.at[i])
    c_par = [cp(0, lre_h, pv0), cp(1, lim_h, pv1), cp(2, ldt_h, pv2), cp(3, dsk_h, pv3)]
    c_b = [cp(4, bre_h, bv.at[0]), cp(5, bim_h, bv.at[1])]
    c_c = [cp(6, cre_h, cv.at[0]), cp(7, cim_h, cv.at[1])]
    c_bx = [cp(8 + c, bx_h.at[:, pl.ds(c * T, T)], bxv.at[c]) for c in range(NC)]
    c_w, c_ax, c_wo = cp(8 + NC, wqkv_h, wv), cp(9 + NC, ax_h, axv), cp(10 + NC, wo_h, wov)

    def start(*cs):
        for c in cs:
            c.start()

    def wait(*cs):
        for c in cs:
            c.wait()
    start(*c_par, c_bx[0], c_b[0], c_b[1])

    wait(*c_par, c_bx[0])
    prm[...] = jnp.zeros(prm.shape, F32)
    for i in range(4):
        prm[i:i + 1, 0:D] = (pv0, pv1, pv2, pv3)[i][...].astype(F32).reshape(1, D)
    lane5 = lax.broadcasted_iota(jnp.int32, (8, 512), 1)
    lre = jnp.where(lane5 < D, jnp.broadcast_to(prm[0:1, :], (8, 512)), -1.0)
    lim = jnp.broadcast_to(prm[1:2, :], (8, 512))
    dt = jnp.exp(jnp.broadcast_to(prm[2:3, :], (8, 512))).astype(BF16).astype(F32)
    never = dt[:, 0:128] < 0.0
    zr, zi = dt * lre, dt * lim
    mag = jnp.exp(zr)
    lr, li = mag * jnp.cos(zi), mag * jnp.sin(zi)
    den = lre * lre + lim * lim
    nr, ni = lr - 1.0, li
    cr = 2.0 * (nr * lre + ni * lim) / den
    ci = 2.0 * (ni * lre - nr * lim) / den
    lane1 = lax.broadcasted_iota(jnp.int32, (8, 128), 1)
    sub = lax.broadcasted_iota(jnp.int32, (8, 128), 0)
    lo = lane1 < 64

    def tiles(r, i):
        r3, i3 = r[:, 384:], i[:, 384:]
        rr = jnp.where(lo, r3, pltpu.roll(r3, 64, 1))
        ii = jnp.where(lo, -i3, pltpu.roll(i3, 64, 1))
        return ([r[:, 128 * k:128 * k + 128] for k in range(3)] + [rr],
                [i[:, 128 * k:128 * k + 128] for k in range(3)] + [ii])
    lam = tiles(lr, li)
    sq = [(lr, li)]
    for _ in range(5):
        sq.append(_cmul(*sq[-1], *sq[-1]))
    pws = []
    for base in (_cmul(*_cmul(*sq[4], *sq[3]), *sq[2]), _cmul(*sq[5], *sq[2])):
        pw = []
        for _ in range(3):
            pw.append(tiles(*base))
            base = _cmul(*base, *base)
        pws.append(pw)
    dsk = pltpu.roll(jnp.broadcast_to(prm[3:4, :], (8, 512)), 64, 1)

    def cstep(m, k, a, b):
        if k < 3:
            return m[0][k] * a - m[1][k] * b, m[0][k] * b + m[1][k] * a
        return m[0][k] * a + m[1][k] * b, m[0][k] * b - m[1][k] * a

    pend = []
    z0 = pl.program_id(0)

    def push(*cs):
        start(*cs)
        obuf[4, 0:8, :] = dsk[:, 128:256]
        pend.append([PD, obuf[4, pl.ds(pl.multiple_of(z0 * 8, 8), 8), :]])

    def gate(rhs, t=None):
        if pend and t is None:
            pend[0][0] -= 1
            if pend[0][0] == 0:
                t = pend.pop(0)[1]
        if t is not None:
            parts = []
            for r in range(0, rhs.shape[0], 128):
                last = rhs[r + 120:r + 128]
                last = jnp.concatenate([jnp.where(never, t, last[:, c:c + 128])
                                        for c in range(0, rhs.shape[1], 128)], axis=1)
                parts += [rhs[r:r + 120], last]
            rhs = jnp.concatenate(parts, axis=0)
        return rhs

    def prep_b(i):
        for r in range(0, D, 64):
            v = jnp.concatenate([jnp.zeros((64, 64), F32), bv[i, r:r + 64, :].astype(F32)], axis=1)
            r2 = 384 * i + r if r < 384 else 768 + 64 * i
            bcat[r2:r2 + 64, :] = v

    ctok = []

    def prep_c():
        toks = []
        nci = -ci[0:1, :D]
        for r in range(0, D, 32):
            c_re = cv[0, r:r + 32, :].astype(F32)
            c_im = cv[1, r:r + 32, :].astype(F32)
            c2r = c_re * cr[0:1, :D] - c_im * ci[0:1, :D]
            c2i = c_re * nci - c_im * cr[0:1, :D]
            ccat[r:r + 32, 0:384] = c2r[:, 0:384]
            ccat[r:r + 32, 384:768] = c2i[:, 0:384]
            c3 = jnp.concatenate([c2r[:, 384:448], c2i[:, 384:448]], axis=1)
            ccat[r:r + 32, 768:896] = c3
            toks += [v[i:i + 8, c:c + 128] for v in (c2r[:, 0:384], c2i[:, 0:384], c3)
                     for i in range(0, 32, 8) for c in range(0, v.shape[1], 128)]
        ctok.append(functools.reduce(jnp.maximum, toks))

    def ssm_t(c):
        for k in range(4):
            if k == 0:
                xt = jnp.concatenate([jnp.zeros((64, T), F32), bxv[c, 0:64, :].astype(F32)], axis=0)
            else:
                xt = bxv[c, 128 * k - 64:128 * k + 64, :].astype(F32)
            xb32[c // 2][k, T * (c % 2):T * (c % 2) + T, :] = xt.T

    def xs(c, k, j):
        return xb32[c // 2][k, pl.ds(_row0(c) % 512 + j, 8, stride=SEGS[c % 2]), :]

    U, Hs = {}, {}

    def ssm_in(c, ns=range(7)):
        for n in ns:
            xl = jnp.concatenate([jnp.concatenate([xs(c, k, j) for k in range(4)], axis=1)
                                  for j in range(SEGS[c % 2])], axis=0)
            U[c, n] = _dot(xl, gate(bcat[128 * n:128 * n + 128, :], ctok[0] if c == 3 and n >= 3 else None), NT)

    carry = [(jnp.zeros((8, 128), F32),) * 2] * 4

    def ssm_scan(c):
        SEG, pw = SEGS[c % 2], pws[c % 2]
        sw = pltpu.roll(U[c, 6], 64, 1)

        def u(j, k):
            if k < 3:
                return U[c, k][8 * j:8 * j + 8], U[c, k + 3][8 * j:8 * j + 8]
            return U[c, 6][8 * j:8 * j + 8], sw[8 * j:8 * j + 8]
        h, hs, dep = [None] * 4, {}, None
        for ks in KG:
            for k in ks:
                h[k] = u(0, k)
                if dep is not None:
                    h[k] = tuple(jnp.where(never, dep, v) for v in h[k])
            for j in range(1, SEG):
                for k in ks:
                    a, b = cstep(lam, k, *h[k])
                    ua, ub = u(j, k)
                    h[k] = (a + ua, b + ub)
            for k in ks:
                z = [jnp.where(sub == 0, carry[k][i], pltpu.roll(h[k][i], 1, 0)) for i in range(2)]
                for n in range(3):
                    sh = 1 << n
                    a, b = cstep(pw[n], k, *[jnp.where(sub >= sh, pltpu.roll(v, sh, 0), 0.0) for v in z])
                    z = [z[0] + a, z[1] + b]
                h[k] = tuple(z)
            for j in range(SEG):
                for k in ks:
                    a, b = cstep(lam, k, *h[k])
                    ua, ub = u(j, k)
                    h[k] = hs[j, k] = (a + ua, b + ub)
                if j == SEG * DJ // 8 - 1:
                    dep = h[ks[-1]][0]
        Hs[c] = [jnp.concatenate([hs[j, 0][0], hs[j, 1][0], hs[j, 2][0], hs[j, 0][1], hs[j, 1][1], hs[j, 2][1],
                                  hs[j, 3][0]], axis=1) for j in range(SEG)]
        carry[:] = [tuple(jnp.broadcast_to(v[7:8], (8, 128)) for v in h[k]) for k in range(4)]

    Y = {}

    def ssm_out(p, ts=range(4), between=lambda: None, tok=None):
        cj = [(2 * p + i, j) for i in range(2) for j in range(SEGS[i])]
        yts = [_dot(ccat[...], gate(jnp.concatenate([Hs[c][j] for c, j in cj[16 * t:16 * t + 16]], axis=0), tok), NT)
               for t in ts]
        Y.update({(p, t): y for t, y in zip(ts, yts)})
        between()
        for t, yt in zip(ts, yts):
            blk = cj[16 * t:16 * t + 16]
            y_post(p, blk, jnp.concatenate([jnp.zeros((64, 128), F32), yt], axis=0), range(4))

    def y_post(p, blk, yt, ks):
        for n, k in enumerate(ks):
            y = yt[128 * n:128 * n + 128].T
            for i, (c, j) in enumerate(blk):
                rows = pl.ds(_row0(c) + j, 8, stride=SEGS[c % 2])
                v = y[8 * i:8 * i + 8] + xs(c, k, j) * dsk[:, 128 * k:128 * k + 128]
                if k == 0 and p >= NPRE:
                    v = jnp.where(lo, a3[rows, :], v)
                obuf[k, rows, :] = v

    def ssm_last(p):
        cj = [(2 * p + i, j) for i in range(2) for j in range(SEGS[i])]
        for ks, ts, cs in PIECES:
            hh = jnp.concatenate([Hs[c][j] for c, j in cj[16 * ts[0]:16 * ts[-1] + 16]], axis=0)
            yt = _dot(ccat[max(128 * ks[0] - 64, 0):128 * ks[-1] + 64, :], gate(hh), NT)
            if ks[0] == 0:
                yt = jnp.concatenate([jnp.zeros((64, yt.shape[1]), F32), yt], axis=0)
            for n, t in enumerate(ts):
                y_post(p, cj[16 * t:16 * t + 16], yt[:, 128 * n:128 * n + 128], ks)
            start(*[o_b[2 * p + c][k] for c in cs for k in ks])

    def w_t(c0, c1):
        for k in range(4):
            n = min(128, D - 128 * k)
            blk = wv[128 * k:128 * k + n, c0:c1].astype(F32)
            if n < 128:
                blk = jnp.concatenate([blk, jnp.zeros((128 - n, c1 - c0), F32)], axis=0)
            wt32[k, c0:c1, :] = blk.T

    def w_rows(g):
        return jnp.concatenate(
            [jnp.concatenate([wt32[k, pl.ds(g * D + hh * 224 + d, 8, stride=DH), :] for k in range(4)], axis=1)
             for d in range(DH) for hh in range(2)], axis=0)

    def w_perm(g):
        for d in range(DH):
            v = [jnp.concatenate([wt32[k, pl.ds(g * D + hh * 224 + d, 8, stride=DH), :]
                                  for k in range(4)], axis=1) for hh in range(2)]
            wtp[g * D + 16 * d:g * D + 16 * d + 16, :] = jnp.concatenate(v, axis=0)

    def x_t():
        for k in range(4):
            n = min(128, D - 128 * k)
            for t in range(4):
                blk = axv[128 * k:128 * k + n, 512 * t:512 * t + 512].astype(F32)
                if n < 128:
                    blk = jnp.concatenate([blk, jnp.zeros((128 - n, 512), F32)], axis=0)
                bt = blk.T
                for g in range(32):
                    r = XP * (32 * t + g)
                    xa32[k, r:r + 16, :] = bt[16 * g:16 * g + 16]

    def wo_prep():
        wo = jnp.concatenate([wov[...].astype(F32), jnp.zeros((D, 64), F32)], axis=1)
        for k in range(4):
            wo32[k] = wo[:, 128 * k:128 * k + 128]
        for k in range(4):
            v = [wo32[k, pl.ds(hh * 224 + d, 8, stride=DH), :] for d in range(DH) for hh in range(2)]
            v = jnp.concatenate(v + [jnp.zeros((64, 128), F32)], axis=0).T
            n = min(128, D - 128 * k)
            wot[128 * k:128 * k + n, :] = v[:n]

    def xa(j):
        return jnp.concatenate([xa32[k, pl.ds(j, 128, stride=XP), :] for k in range(4)], axis=1)

    KV, Q, O = ({}, {}), {}, {}

    def att_kv(j, gs=(0, 1)):
        for g in gs:
            r = _dot(w_rows(g + 1), gate(xa(j)), NT)
            KV[g][j + 14] = r
            if j >= 2 and j != NJ - 2:
                KV[g][j - 2] = pltpu.roll(r, 1, 1)

    def att_q(*js, t=None):
        for j in js:
            Q[j] = _dot(w_rows(0), gate(xa(j), t), NT)

    scale = DH ** -0.5

    PP = {}

    def att_l(jp):
        js = JP[jp]
        es = range(js[0], js[1] + 15, 2)
        P = {}
        for hh in range(2):
            lg = {}
            for d in range(DH):
                r = slice(16 * d + 8 * hh, 16 * d + 8 * hh + 8)
                for j in js:
                    for w in range(W):
                        t = Q[j][r] * KV[0][j + 14 - 2 * w][r]
                        lg[j, w] = t if d == 0 else lg[j, w] + t
            for j in js:
                l = [lg[j, w] * scale for w in range(W)]
                l = [jnp.where(lane1 == 0, -1e9, l[w]) if j < 2 * w else l[w] for w in range(W)]
                m = l[0]
                for w in range(1, W):
                    m = jnp.maximum(m, l[w])
                e = [jnp.exp(x - m) for x in l]
                ssum = e[0]
                for w in range(1, W):
                    ssum = ssum + e[w]
                inv = 1.0 / ssum
                P[hh, j] = [x * inv for x in e]
        PP[jp] = P

    def att_v(jp, pace=None):
        js, P = JP[jp], PP[jp]
        for j in js:
            O[j] = [None] * (2 * DH)
        dep = None
        for hh, jj in [(h, js) for h in range(2)]:
            if dep is not None:
                for j in jj:
                    P[hh, j] = [jnp.where(never, dep, x) for x in P[hh, j]]
            for d in range(DH):
                r = slice(16 * d + 8 * hh, 16 * d + 8 * hh + 8)
                if pace is not None and d % GV == 0:
                    row = (D * (hh * DH + d) // (2 * DH)) // 8 * 8
                    for j in jj:
                        P[hh, j] = [jnp.where(never, pace[row:row + 8], x) for x in P[hh, j]]
                for j in jj:
                    acc = None
                    for w in range(W):
                        t = P[hh, j][w] * KV[1][j + 14 - 2 * w][r]
                        acc = t if acc is None else acc + t
                    O[j][2 * d + hh] = acc
                    if d == DH - 1:
                        dep = acc

    ores = {}

    def att_o(jp):
        rhs = jnp.concatenate([jnp.concatenate(O[j] + [jnp.zeros((64, 128), F32)], axis=0) for j in JP[jp]], axis=1)
        res = _dot(wot[...], gate(rhs), NN)
        ores[jp] = jnp.concatenate([res[16 * i:16 * i + 8, 128 * h:128 * h + 128] for h in range(2) for i in range(DH)], axis=0)
        for i, j in enumerate(JP[jp]):
            rt = jnp.concatenate([res[:, 128 * i:128 * i + 128], jnp.zeros((64, 128), F32)], axis=0)
            for k in range(4):
                ost[j % 2][k, pl.ds(OP * (j // 2), 128), :] = rt[128 * k:128 * k + 128].T

    def o_rows(par, k, s):
        return ost[par][k, pl.ds(s, 8, stride=OP), :]

    def o_unperm(par):
        for k in range(3):
            for s in range(128):
                oa[k, pl.ds(NJ * s + par, 8, stride=2), :] = o_rows(par, k, s)

    def o_mixed(early):
        for s in range(128):
            for par in range(2):
                if early != (par == 0 and not 512 <= NJ * s < 512 * NPRE):
                    continue
                rows = pl.ds(NJ * s + par, 8, stride=2)
                if NJ * s < 512 * NPRE:
                    obuf[0, rows, :] = jnp.where(lo, o_rows(par, 3, s), obuf[0, rows, :])
                else:
                    a3[rows, :] = o_rows(par, 3, s)

    o_a = [pltpu.make_async_copy(oa.at[k], out_h.at[:, pl.ds(128 * k, 128)], osem) for k in range(3)]
    o_b = [[pltpu.make_async_copy(obuf.at[k, pl.ds(_row0(c), 8 * SEGS[c % 2])],
                                  out_h.at[pl.ds(_row0(c), 8 * SEGS[c % 2]), pl.ds(128 * (k + 3), 128)],
                                  osem) for k in range(4)] for c in range(NC)]

    NPRE = 2
    ssm_t(0)
    wait(c_b[0])
    start(c_bx[1], c_bx[2], c_bx[3])
    prep_b(0)
    ssm_in(0, range(2))
    wait(c_b[1], c_bx[1])
    start(*c_c, c_w)
    prep_b(1)
    ssm_t(1)
    ssm_in(0, range(2, 7))
    ssm_in(1, range(2))
    wait(c_bx[2], c_bx[3])
    ssm_in(1, range(2, 7))
    axv[0:16, 0:128] = U[1, 5][0:16].astype(BF16)
    start(c_ax)
    ssm_scan(0)
    ssm_t(2)
    ssm_t(3)
    ssm_in(2, range(7))
    wait(*c_c, c_w)
    w_t(384, 3 * D)
    prep_c()
    ssm_in(3, range(2))
    ssm_scan(1)
    ssm_in(3, range(2, 7))
    cj0 = [(i, j) for i in range(2) for j in range(SEGS[i])]
    h0 = [jnp.concatenate([Hs[c][j] for c, j in cj0[16 * t:16 * t + 16]], axis=0) for t in range(3)]
    y0 = _dot(ccat[...], h0[0], NT)
    ym = _dot(ccat[...], h0[1], NT)
    y1 = _dot(ccat[:, 0:256], h0[2][:, 0:256], NT)
    y1 = jnp.concatenate([jnp.where(never, 0.0, y1[r:r + 8]) for r in range(0, D, 8)], axis=0)
    wait(c_ax)
    start(c_wo, *c_bx[4:])
    y1 = y1 + _dot(ccat[:, 256:], h0[2][:, 256:], NT)
    for t, y in enumerate((y0, ym, y1)):
        y_post(0, cj0[16 * t:16 * t + 16], jnp.concatenate([jnp.zeros((64, 128), F32), y], axis=0), range(4))
    x_t()
    ssm_out(0, range(3, 4))
    ssm_scan(2)
    for j in range(0, NJ, 2):
        att_kv(j)
    ssm_scan(3)
    w_t(0, 384)
    start(*o_b[0][1:], *o_b[1][1:])
    wait(c_wo, *c_bx[4:6])
    for g in range(2):
        KV[g][NJ - 4] = pltpu.roll(KV[g][NJ + 12], 1, 1)
    wo_prep()
    att_kv(1, (1,))
    att_q(0)
    att_q(2)
    att_kv(1, (0,))
    att_q(4)
    att_q(6)
    att_l(0)
    att_v(0)
    att_kv(3, (0,))
    att_kv(3, (1,))
    att_kv(5, (0,))
    att_kv(5, (1,))
    att_q(8)
    att_kv(7, (0,))
    att_q(10)
    att_l(1)
    att_v(1)
    att_kv(7, (1,))
    att_kv(9, (0,))
    att_kv(9, (1,))
    att_q(12)
    att_q(14)
    att_l(2)
    att_v(2)
    att_kv(11, (0,))
    att_kv(11, (1,))
    att_kv(13, (1,))
    att_o(0)
    att_kv(13, (0,))
    att_l(3)
    att_v(3)
    att_kv(15, (0,))
    att_kv(15, (1,))
    att_o(1)
    ssm_t(4)
    ssm_t(5)
    att_q(1, 3, t=KV[0][NJ - 1 + 14][120:120 + 8])
    att_l(4)
    ssm_out(1, [0], tok=None)
    att_o(2)
    att_v(4, ores[2])
    att_q(5, 7, t=Y[1, 0][120:120 + 8])
    att_l(5)
    ssm_out(1, [1], tok=None)
    att_o(3)
    att_v(5, ores[3])
    o_unperm(0)
    push(*o_b[2][1:])
    o_mixed(True)
    att_q(9, 11, t=Y[1, 1][120:120 + 8])
    att_l(6)
    ssm_out(1, [2], tok=None)
    att_o(4)
    att_v(6, ores[4])
    att_q(13, 15, t=Y[1, 2][120:120 + 8])
    att_l(7)
    ssm_out(1, [3], tok=None)
    push(*o_b[3][1:])
    att_o(5)
    att_v(7, ores[5])
    att_o(6)
    att_o(7)
    ssm_in(4, [0])
    ssm_in(4, [1])
    ssm_in(4, [2])
    ssm_in(4, [3, 4, 5])
    o_unperm(1)
    o_mixed(False)
    start(*o_a, o_b[0][0], o_b[1][0], o_b[2][0], o_b[3][0])
    wait(*c_bx[6:])
    ssm_t(6)
    ssm_t(7)
    ssm_in(4, range(6, 7))
    ssm_in(5)
    ssm_scan(4)
    ssm_in(6)
    ssm_scan(5)
    ssm_out(2, range(2))
    push(*o_b[4])
    ssm_in(7)
    ssm_out(2, range(2, 3))
    ssm_scan(6)
    ssm_out(2, range(3, 4))
    push(*o_b[5])
    ssm_scan(7)
    ssm_last(3)
    pltpu.make_async_copy(out_h, out_h, osem).wait()


@jax.jit
def pallas_concat_heads__sliding_local_dilated__ssm_conv_s5__prompt_kernel(
    A_x, A_wqkv, A_wo, B_x, B_Lambda_re, B_Lambda_im, B_B_re, B_B_im, B_C_re, B_C_im,
    B_log_dt, B_Dskip,
):
    hbm = pl.BlockSpec(memory_space=pltpu.HBM)
    out = pl.pallas_call(
        _kernel,
        out_shape=jax.ShapeDtypeStruct((S, 2 * D), F32),
        grid=(1,),
        in_specs=[hbm] * 12,
        out_specs=hbm,
        scratch_shapes=[
            pltpu.VMEM((D, S), BF16),
            pltpu.VMEM((D, 3 * D), BF16),
            pltpu.VMEM((D, D), BF16),
            pltpu.VMEM((NC, D, T), BF16),
            pltpu.VMEM((2, D, D), BF16),
            pltpu.VMEM((2, D, D), BF16),
            *[pltpu.VMEM((D,), BF16)] * 4,
            pltpu.VMEM((8, 512), F32),
            pltpu.VMEM((896, 512), F32),
            pltpu.VMEM((D, 896), F32),
            *[pltpu.VMEM((4, 512, 128), F32)] * 4,
            pltpu.VMEM((4, 3 * D, 128), F32),
            pltpu.VMEM((4, D, 128), F32),
            pltpu.VMEM((D, 512), F32),
            pltpu.VMEM((4, 128 * XP, 128), F32),
            pltpu.VMEM((5, S, 128), F32),
            pltpu.VMEM((S, 128), F32),
            pltpu.VMEM((3, S, 128), F32),
            *[pltpu.VMEM((4, 8 * OP, 128), F32)] * 2,
            pltpu.SemaphoreType.DMA((11 + NC,)),
            pltpu.SemaphoreType.DMA(()),
        ],
        compiler_params=pltpu.CompilerParams(vmem_limit_bytes=100 * 1024 * 1024),
    )(A_x[0].T, A_wqkv, A_wo, B_x[0].T, B_Lambda_re, B_Lambda_im,
      B_B_re, B_B_im, B_C_re, B_C_im, B_log_dt, B_Dskip)
    return out.reshape(1, S, 2 * D)
```
